```python
import jax
import jax.numpy as jnp

def _softmax(x, axis=-1):
    return jax.nn.softmax(x, axis=axis)

def _gelu(x):
    return jax.nn.gelu(x, approximate=True)

def _silu(x):
    return jax.nn.silu(x)

def _sigmoid(x):
    return jax.nn.sigmoid(x)

def _layernorm(x, axis=-1, eps=1e-05):
    m = jnp.mean(x, axis=axis, keepdims=True)
    v = jnp.var(x, axis=axis, keepdims=True)
    return (x - m) / jnp.sqrt(v + eps)

def _scatter_add(tgt, idx, src, axis=0):
    return tgt.at[idx].add(src)

def _segment_sum(src, seg, n):
    return jax.ops.segment_sum(src, seg, n)

class _Rng:

    def __init__(self, key):
        self._k = key

    def _next(self):
        self._k, sub = jax.random.split(self._k)
        return sub

    def normal(self, shape):
        return jax.random.normal(self._next(), shape, dtype=jnp.bfloat16)

    def randint(self, lo, hi, shape):
        return jax.random.randint(self._next(), shape, lo, hi, dtype=jnp.int32)

    def uniform(self, shape, lo=0.0, hi=1.0):
        return jax.random.uniform(self._next(), shape, jnp.bfloat16, lo, hi)

    def permutation(self, n):
        return jax.random.permutation(self._next(), n)
kernel_name = 'interleave_layers__memory_aug_infini_attn__sliding_local_dilated__prompt'

def setup_inputs():
    _rng = _Rng(jax.random.key(int.from_bytes(__import__("os").urandom(4), "little")))
    _w = lambda a: (lambda t: t.astype(jnp.bfloat16) if jnp.issubdtype(t.dtype, jnp.floating) else t)(jnp.asarray(a))

    def _A_setup():
        B, S, D, H = (1, 2048, 1024, 32)
        N = 4
        L = max(1, S // N)
        sc = D ** (-0.5)
        return {'x': _w((lambda *s: _rng.normal(s) * 0.05)(B, N * L, D)), 'wq': _w((lambda *s: _rng.normal(s) * 0.05)(D, D) * sc), 'wk': _w((lambda *s: _rng.normal(s) * 0.05)(D, D) * sc), 'wv': _w((lambda *s: _rng.normal(s) * 0.05)(D, D) * sc), 'wo': _w((lambda *s: _rng.normal(s) * 0.05)(D, D) * sc), 'beta': _w((lambda *s: _rng.normal(s) * 0.05)(H))}
    _A_in = _A_setup()

    def _B_setup():
        B, S, D = (1, 2048, 1024)
        return {'x': _w((lambda *s: _rng.normal(s) * 0.05)(B, S, D)), 'wqkv': _w((lambda *s: _rng.normal(s) * 0.05)(D, 3 * D)), 'wo': _w((lambda *s: _rng.normal(s) * 0.05)(D, D))}
    _B_in = _B_setup()
    return {'A_x': _A_in['x'], 'A_wq': _A_in['wq'], 'A_wk': _A_in['wk'], 'A_wv': _A_in['wv'], 'A_wo': _A_in['wo'], 'A_beta': _A_in['beta'], 'B_x': _B_in['x'], 'B_wqkv': _B_in['wqkv'], 'B_wo': _B_in['wo']}

def reference(A_x, A_wq, A_wk, A_wv, A_wo, A_beta, B_x, B_wqkv, B_wo):

    def _A_ref(x, wq, wk, wv, wo, beta):
        B, S, D = x.shape
        H = 32
        Dh = D // H
        N = 4
        L = S // N
        q = (lambda x, *d: x.transpose(*d))((x @ wq).reshape(B, S, H, Dh), 0, 2, 1, 3).reshape(B, H, N, L, Dh)
        k = (lambda x, *d: x.transpose(*d))((x @ wk).reshape(B, S, H, Dh), 0, 2, 1, 3).reshape(B, H, N, L, Dh)
        v = (lambda x, *d: x.transpose(*d))((x @ wv).reshape(B, S, H, Dh), 0, 2, 1, 3).reshape(B, H, N, L, Dh)
        phi = lambda t: jnp.where(t > 0, t + 1.0, jnp.exp(t))
        scale = Dh ** (-0.5)
        ar = jnp.arange(L)
        mask = (lambda x, dt: x.astype(dt))(ar[:, None] < ar[None, :], x.dtype) * -1000000000.0
        g = _sigmoid(beta).reshape(1, H, 1, 1)
        M = jnp.einsum('bhd,bhe->bhde', q[:, :, 0, 0, :] * 0.0, q[:, :, 0, 0, :] * 0.0)
        z = q[:, :, 0, 0, :] * 0.0
        outs = []
        for s in range(N):
            qs, ks, vs = (q[:, :, s].copy(), k[:, :, s].copy(), v[:, :, s].copy())
            logits = jnp.einsum('bhqd,bhkd->bhqk', qs, ks) * scale + mask
            p = _softmax(logits, axis=-1)
            a_dot = jnp.einsum('bhqk,bhkd->bhqd', p, vs)
            pq = phi(qs)
            num = jnp.einsum('bhld,bhde->bhle', pq, M)
            den = jnp.einsum('bhld,bhd->bhl', pq, z)[..., None] + 1e-06
            a_mem = num / den
            o = g * a_mem + (1.0 - g) * a_dot
            outs.append(o)
            pk = phi(ks)
            M = M + jnp.einsum('bhld,bhle->bhde', pk, vs)
            z = z + jnp.einsum('bhld->bhd', pk)
        o = (lambda x, *d: x.transpose(*d))(jnp.stack(outs, 2).reshape(B, H, S, Dh), 0, 2, 1, 3).reshape(B, S, D)
        return o @ wo

    def _B_ref(x, wqkv, wo):
        B, S, D = x.shape
        H = 32
        Dh = D // H
        W, dil = (8, 2)
        qkv = (lambda x, *d: x.transpose(*d))((x @ wqkv).reshape(B, S, 3, H, Dh), 2, 0, 3, 1, 4)
        q, k, v = (qkv[0], qkv[1], qkv[2])
        scale = Dh ** (-0.5)
        pos = jnp.arange(S)
        off = jnp.arange(W) * dil
        idx = pos[:, None] - off[None, :]
        mask = idx >= 0
        idx_c = jnp.where(mask, idx, 0).reshape(-1)
        kg = k[:, :, idx_c, :].reshape(B, H, S, W, Dh)
        vg = v[:, :, idx_c, :].reshape(B, H, S, W, Dh)
        logits = jnp.einsum('bhsd,bhswd->bhsw', q, kg) * scale
        logits = jnp.where(mask[None, None, :, :], logits, -1000000000.0)
        attn = _softmax(logits, axis=-1)
        o = jnp.einsum('bhsw,bhswd->bhsd', attn, vg)
        return (lambda x, *d: x.transpose(*d))(o, 0, 2, 1, 3).reshape(B, S, D) @ wo
    x = A_x
    x = x + _A_ref(_layernorm(x, axis=-1), A_wq, A_wk, A_wv, A_wo, A_beta)
    x = x + _B_ref(_layernorm(x, axis=-1), B_wqkv, B_wo)
    x = x + _A_ref(_layernorm(x, axis=-1), A_wq, A_wk, A_wv, A_wo, A_beta)
    x = x + _B_ref(_layernorm(x, axis=-1), B_wqkv, B_wo)
    return x
```

```python
import math

import jax
import jax.numpy as jnp
from jax import lax
from jax.experimental import pallas as pl
from jax.experimental.pallas import tpu as pltpu

S = 2048
D = 1024
H = 32
DH = 32
SEG = 512
WIN, DIL = 8, 2
HALO = 16
SUB = 128
HS = SUB // 2
NSUB = S // SUB
LOG2E = math.log2(math.e)
QK_SCALE = DH ** -0.5 * LOG2E
PV_LAG = 5

f32 = jnp.float32
bf16 = jnp.bfloat16
u32 = jnp.uint32

AQ, AK, AV, AO, BQ, BK, BV, BO = range(8)


def _mm(a, b):
    return lax.dot_general(a, b, (((1,), (0,)), ((), ())), preferred_element_type=f32)


def _ld16(ref, lead, r0, n):
    return pltpu.bitcast(ref.bitcast(u32)[(*lead, pl.ds(r0, n // 2), slice(None))], bf16)


def _left_operands(a11, a12, a21, a22):
    return (a11 + a22, a21 + a22, a11, a22, a11 + a12, a21 - a11, a12 - a22)


def _right_operands(b11, b12, b21, b22):
    return (b11 + b22, b11, b12 - b22, b21 - b11, b22, b11 + b12, b21 + b22)


def _strassen(prod, emit):
    m1, m4 = prod(0), prod(3)
    c11 = m1 + m4
    m2 = prod(1)
    emit(1, 0, m2 + m4)
    c22 = (m1 - m2) + prod(5)
    m3 = prod(2)
    emit(1, 1, c22 + m3)
    m5 = prod(4)
    emit(0, 1, m3 + m5)
    emit(0, 0, (c11 - m5) + prod(6))


def _layernorm(x):
    d = x - jnp.sum(x, axis=-1, keepdims=True) * (1.0 / D)
    v = jnp.sum(d * d, axis=-1, keepdims=True) * (1.0 / D)
    return d * lax.rsqrt(v + 1e-5)


def _phi(t):
    return jnp.where(t > 0, t + 1.0, jnp.exp(t))


def _tile(x, c):
    return x[:, 128 * c:128 * (c + 1)]


def _kernel(x_hbm, wq_hbm, wk_hbm, wv_hbm, wo_hbm, beta_ref, bqkv_hbm, bo_hbm, out_hbm,
            xbuf, raw_q, raw_k, raw_v, raw_o, raw_bqkv, raw_bo,
            w_aq, w_ak, w_av, w_ao, w_bq, w_bk, w_bv, w_bo,
            xn, vt, obuf, gate, perm_c, perm_r,
            p1_q, p1_pq, p1_k, p1_pk, p1_s,
            p2_x, p2_l, p2_q, p2_k, p2_v, p2_p,
            x_sem, w_sem, o_sem):
    wts = (w_aq, w_ak, w_av, w_ao, w_bq, w_bk, w_bv, w_bo)
    lane = lax.broadcasted_iota(jnp.int32, (128, 128), 1)
    row = lax.broadcasted_iota(jnp.int32, (128, 128), 0)
    lane8 = lax.broadcasted_iota(jnp.int32, (8, 128), 1)
    row8 = lax.broadcasted_iota(jnp.int32, (8, 128), 0)

    x_edges = (0, SUB, SUB + SEG, SUB + 2 * SEG, SUB + 3 * SEG, S)

    def x_copy(i):
        rows = pl.ds(x_edges[i], x_edges[i + 1] - x_edges[i])
        return pltpu.make_async_copy(x_hbm.at[rows], xbuf.at[rows], x_sem.at[i])

    w_pairs = ((wv_hbm, raw_v), (wk_hbm, raw_k), (wq_hbm, raw_q), (wo_hbm, raw_o),
               (bqkv_hbm, raw_bqkv), (bo_hbm, raw_bo))

    def w_copy(i):
        return pltpu.make_async_copy(w_pairs[i][0], w_pairs[i][1], w_sem.at[i])

    def out_copy(c):
        rows = pl.ds(pl.multiple_of(c * 2 * SUB, 2 * SUB), 2 * SUB)
        return pltpu.make_async_copy(xbuf.at[rows], out_hbm.at[rows], o_sem.at[c])

    x_copy(0).start()
    w_copy(0).start()
    x_copy(1).start()
    x_copy(2).start()
    w_copy(1).start()
    x_copy(3).start()
    w_copy(2).start()
    x_copy(4).start()
    for i in range(3, 6):
        w_copy(i).start()

    hr = lax.broadcasted_iota(jnp.int32, (H, H), 0)
    hc = lax.broadcasted_iota(jnp.int32, (H, H), 1)
    sig = 1.0 / (1.0 + jnp.exp(-beta_ref[...].astype(f32)))
    gate[...] = jnp.broadcast_to(
        jnp.sum(jnp.where(hr == hc, sig, 0.0), axis=1, keepdims=True), (H, 128))

    def put_weight(m, r0, top, bot):
        n = top.shape[0]
        for t in range(4):
            ops = _right_operands(_tile(top, t), _tile(top, t + 4), _tile(bot, t), _tile(bot, t + 4))
            for i in range(7):
                wts[m][i, t, pl.ds(r0, n), :] = ops[i].astype(bf16)

    def raw_rows(raw, r0, n, c0=0):
        return raw[pl.ds(r0, n), c0:c0 + D].astype(f32)

    def prep_plain(m, raw, it, n):
        r0 = pl.multiple_of(it * n, n)
        put_weight(m, r0, raw_rows(raw, r0, n), raw_rows(raw, pl.multiple_of(r0 + D // 2, n), n))

    def regroup(buf, slot):
        return jnp.concatenate(
            [buf[slot, pl.ds(d, H, stride=DH + 1), :] for d in range(DH)], axis=0)

    def prep_cols(m, it, zero):
        r0 = pl.multiple_of(it * 128, 128)
        halves = []
        for hf in range(2):
            slot = 2 * (m - BQ) + hf
            wt = raw_rows(raw_bqkv, pl.multiple_of(r0 + hf * (D // 2), 128), 128, (m - BQ) * D).T
            for h in range(H):
                perm_c[slot][0, pl.ds(h * (DH + 1), DH), :] = wt[h * DH:(h + 1) * DH]
            halves.append(regroup(perm_c[slot], zero).T)
        put_weight(m, r0, *halves)

    def prep_rows(it, zero):
        cols = []
        for hf in range(2):
            c0 = pl.multiple_of(it * 128 + hf * (D // 2), 128)
            w = raw_bo[:, pl.ds(c0, 128)].astype(f32)
            for h in range(H):
                perm_r[hf][0, pl.ds(h * (DH + 1), DH), :] = w[h * DH:(h + 1) * DH]
            cols.append(regroup(perm_r[hf], zero))
        hd = D // 2
        ops = _right_operands(cols[0][:hd], cols[1][:hd], cols[0][hd:], cols[1][hd:])
        for i in range(7):
            w_bo[i, it, :, :] = ops[i].astype(bf16)

    def put_left(buf, r0, top, bot):
        for k in range(4):
            ops = _left_operands(top(k), top(k + 4), bot(k), bot(k + 4))
            for i in range(7):
                buf[i, k, pl.ds(r0, ops[i].shape[0]), :] = ops[i].astype(bf16)

    def project(buf, zero, r0, n, m, t, emit):
        def prod(i):
            lhs = jnp.concatenate([_ld16(buf, (i + zero, k), r0, n) for k in range(4)], axis=1)
            return _mm(lhs, _ld16(wts[m], (i, t), 0, D // 2))
        _strassen(prod, emit)

    def norm_unit(src_unit, dst_unit):
        for r in range(0, HS, 16):
            top = _layernorm(xbuf[pl.ds(pl.multiple_of(src_unit * SUB + r, 16), 16), :].astype(f32))
            bot = _layernorm(xbuf[pl.ds(pl.multiple_of(src_unit * SUB + HS + r, 16), 16), :].astype(f32))
            put_left(xn, pl.multiple_of(dst_unit * HS + r, 16),
                     lambda c: _tile(top, c), lambda c: _tile(bot, c))

    def phase0(layer, c):
        for i in range(4):
            @pl.when(jnp.logical_and(layer == 0, c == i))
            def _():
                x_copy(i + 1).wait()
        for u in range(4):
            unit = c * 4 + u
            got = {}

            def emit(rh, ch, val):
                got[rh, ch] = val
            for t in range(4):
                project(xn, 0, pl.multiple_of(unit * (HS // 2), HS // 2), HS, AV, t, emit)
                for ch in range(2):
                    v = jnp.concatenate([got[0, ch], got[1, ch]], axis=0)
                    vt[t + 4 * ch, unit, :, :] = v.T.astype(bf16)
            norm_unit(unit + 1 if u < 3 else jnp.minimum(unit + 1, NSUB - 1), unit + 1)

    def phase1(t):
        zero = t >> 4
        st = {}

        def proj(m, s, half):
            got = {}

            def emit(rh, ch, val):
                got[rh, ch] = val
            project(xn, 0, (s * 4 + half * 2) * (HS // 2), 2 * HS, m, t, emit)
            for ch in range(2):
                slot = 2 * s + ch
                for u in range(2):
                    blk = 2 * half + u
                    y = jnp.concatenate([got[0, ch][HS * u:HS * (u + 1)],
                                         got[1, ch][HS * u:HS * (u + 1)]], axis=0)
                    if m == AK:
                        p1_k[slot][blk, :, :] = y.astype(bf16)
                        if s < 3:
                            pk = _phi(y)
                            p1_pk[slot][blk, :, :] = pk.astype(bf16)
                            z = jnp.sum(pk.reshape(16, 8, 128), axis=0)
                            st['dz', slot] = z if blk == 0 else st['dz', slot] + z
                    else:
                        y = y.T
                        p1_q[slot][blk, :, :] = (y * QK_SCALE).astype(bf16)
                        if s > 0:
                            p1_pq[slot - 2][blk, :, :] = _phi(y).astype(bf16)

        def scores(n, s, ch, i, kb):
            slot = 2 * s + ch
            k = _ld16(p1_k[slot], (kb + zero,), 0, 128)
            for j in range(4):
                q = _ld16(p1_q[slot], (i + zero,), 16 * j, DH)
                parts = [jnp.zeros((DH * j, 128), bf16)] * (j > 0) + [q]
                parts += [jnp.zeros((DH * (3 - j), 128), bf16)] * (j < 3)
                sc = _mm(k, jnp.concatenate(parts, axis=0))
                if kb == i:
                    sc = jnp.where(row <= lane, sc, -1e30)
                p1_s[n % len(p1_s)][4 * kb + j, :, :] = sc
                mx = jnp.max(sc.reshape(16, 8, 128), axis=0)
                if kb > 0:
                    mx = jnp.maximum(mx, st['m', n, j])
                if kb == i:
                    mx = jnp.max(mx, axis=0, keepdims=True)
                st['m', n, j] = mx

        def values(n, s, ch, i, kb):
            g = t + 4 * ch
            outs = []
            for j in range(4):
                p = jnp.exp2(p1_s[n % len(p1_s)][4 * kb + j + zero, :, :] - st['m', n, j])
                l = jnp.sum(p.reshape(16, 8, 128), axis=0)
                o = _mm(_ld16(vt, (g, 4 * s + kb), 16 * j, DH), p)
                if kb > 0:
                    l = l + st['l', n, j]
                    o = o + st['o', n, j]
                st['l', n, j], st['o', n, j] = l, o
                if kb == i:
                    gj = gate[pl.ds(4 * g + j, 1), :]
                    o = o * ((1.0 - gj) / jnp.sum(l, axis=0, keepdims=True))
                    if s > 0:
                        nd = _tile(st['nd', s, ch], i)
                        o = o + nd[DH * j:DH * (j + 1)] * (gj / (nd[128 + j:129 + j] + 1e-6))
                    outs.append(o)
            if kb == i:
                obuf[g, pl.ds(SEG * s + 128 * i, 128), :] = jnp.concatenate(outs, axis=0).T

        def mem_read(s, ch):
            mt, z = st['M', ch]
            z = jnp.sum(z, axis=0, keepdims=True)
            lhs = jnp.concatenate([jnp.where((lane >> 5) == (row >> 5), mt, 0.0),
                                   jnp.where((lane8 >> 5) == row8, z, 0.0),
                                   jnp.zeros((8, 128), f32)], axis=0).astype(bf16)
            pq = jnp.concatenate(
                [_ld16(p1_pq[2 * s + ch - 2], (b + zero,), 0, 128) for b in range(4)], axis=1)
            st['nd', s, ch] = _mm(lhs, pq)

        def mem_update(s, ch):
            slot = 2 * s + ch
            v = jnp.concatenate(
                [_ld16(vt, (t + 4 * ch, 4 * s + b), 0, 128) for b in range(4)], axis=1)
            pk = jnp.concatenate(
                [_ld16(p1_pk[slot], (b + zero,), 0, 128) for b in range(4)], axis=0)
            mt, z = _mm(v, pk), st['dz', slot]
            if s > 0:
                mt, z = mt + st['M', ch][0], z + st['M', ch][1]
            st['M', ch] = (mt, z)

        tiles = []
        for s in range(4):
            for ch in range(2):
                for i in (3, 2, 1, 0):
                    n = (2 * s + ch) * 4 + (3 - i)
                    tiles += [(n, s, ch, i, kb) for kb in range(i + 1)]
        side = {
            1: lambda: prep_plain(AO, raw_o, t, 128),
            11: lambda: prep_cols(BK, t, zero),
            21: lambda: prep_cols(BQ, t, zero),
            31: lambda: prep_cols(BV, t, zero),
            41: lambda: prep_rows(t, zero),
        }
        for m, half in ((AQ, 1), (AK, 0), (AK, 1), (AQ, 0)):
            proj(m, 0, half)
        for a in range(len(tiles) + PV_LAG):
            s, pos = divmod(a, 20)
            if s < 3 and pos % 5 == 0:
                m, half = ((AQ, 1), (AK, 0), (AK, 1), (AQ, 0))[pos // 5]
                proj(m, s + 1, half)
            if a in side:
                side[a]()
            if a < len(tiles):
                scores(*tiles[a])
            if a >= PV_LAG:
                n, s, ch, i, kb = tiles[a - PV_LAG]
                if i == 3 and kb == 0 and s > 0:
                    mem_read(s, ch)
                values(n, s, ch, i, kb)
                if i == 2 and kb == 0 and s < 3:
                    mem_update(s, ch)

    def phase2(layer, c):
        zero = c >> 4
        base = [pl.multiple_of((2 * c + u) * SUB, SUB) for u in range(2)]

        def rows(u, r, n):
            return pl.ds(pl.multiple_of(base[u] + r, 16), n)

        def infini_out(u):
            put_left(p2_l[u], 0, lambda g: obuf[g, rows(u, 0, HS), :],
                     lambda g: obuf[g, rows(u, HS, HS), :])
            for t in range(4):
                def emit(rh, ch, val):
                    g = t + 4 * ch
                    x = xbuf[rows(u, rh * HS, HS), 128 * g:128 * (g + 1)].astype(f32)
                    p2_x[u][g, pl.ds(rh * HS, HS), :] = x + val
                project(p2_l[u], zero, 0, HS, AO, t, emit)

        def norm(u):
            for r in range(0, HS, 16):
                top, bot = (
                    _layernorm(jnp.concatenate(
                        [p2_x[u][g + zero, pl.ds(rh * HS + r, 16), :] for g in range(8)], axis=1))
                    for rh in range(2))
                put_left(p2_l[2 + u], r, lambda g: _tile(top, g), lambda g: _tile(bot, g))

        def local_proj(u, m, dst, off):
            for t in range(4):
                def emit(rh, ch, val):
                    dst[u][t + 4 * ch, pl.ds(off + rh * HS, HS), :] = val
                    if off and rh == 1 and u == 0:
                        dst[1][t + 4 * ch, pl.ds(0, HALO), :] = val[HS - HALO:]
                project(p2_l[2 + u], zero, 0, HS, m, t, emit)

        def probs(u):
            for r in range(0, SUB, 16):
                lg = [None] * WIN
                for g in range(8):
                    q = p2_q[u][g + zero, pl.ds(r, 16), :]
                    for w in range(WIN):
                        qk = q * p2_k[u][g + zero, pl.ds(HALO + r - DIL * w, 16), :]
                        lg[w] = qk if g == 0 else lg[w] + qk
                for w in range(WIN):
                    a = lg[w] + pltpu.roll(lg[w], 64, 1)
                    a = (a + pltpu.roll(a, 32, 1)) * QK_SCALE
                    if u == 0 and r == 0 and w > 0:
                        pos = base[0] + lax.broadcasted_iota(jnp.int32, (16, 128), 0)
                        a = jnp.where(pos >= DIL * w, a, -1e9 * LOG2E)
                    lg[w] = a
                mx = lg[0]
                for w in range(1, WIN):
                    mx = jnp.maximum(mx, lg[w])
                ex = [jnp.exp2(a - mx) for a in lg]
                den = ex[0]
                for w in range(1, WIN):
                    den = den + ex[w]
                inv = 1.0 / den
                for w in range(WIN):
                    p2_p[u][w, pl.ds(r, 16), :] = ex[w] * inv

        def mix(u):
            for r in range(0, HS, 16):
                p = [[p2_p[u][w + zero, pl.ds(rh * HS + r, 16), :] for w in range(WIN)]
                     for rh in range(2)]

                def out(rh, g):
                    acc = None
                    for w in range(WIN):
                        pv = p[rh][w] * p2_v[u][g + zero, pl.ds(HALO + rh * HS + r - DIL * w, 16), :]
                        acc = pv if w == 0 else acc + pv
                    return acc
                put_left(p2_l[4 + u], r, lambda g: out(0, g), lambda g: out(1, g))

        def local_out(u):
            for t in range(4):
                def emit(rh, ch, val):
                    g = t + 4 * ch
                    y = p2_x[u][g + zero, pl.ds(rh * HS, HS), :] + val
                    xbuf[rows(u, rh * HS, HS), 128 * g:128 * (g + 1)] = y.astype(bf16)
                project(p2_l[4 + u], zero, 0, HS, BO, t, emit)

        infini_out(0)
        infini_out(1)
        norm(0)
        local_proj(0, BK, p2_k, HALO)
        norm(1)
        local_proj(0, BQ, p2_q, 0)
        local_proj(1, BK, p2_k, HALO)
        probs(0)
        local_proj(1, BQ, p2_q, 0)
        local_proj(0, BV, p2_v, HALO)
        probs(1)
        local_proj(1, BV, p2_v, HALO)
        mix(0)
        local_out(0)
        mix(1)
        local_out(1)
        for buf in (p2_k, p2_v):
            for g in range(8):
                buf[0][g, pl.ds(0, HALO), :] = buf[1][g + zero, pl.ds(SUB, HALO), :]

        @pl.when(layer == 1)
        def _():
            out_copy(c).start()

    x_copy(0).wait()

    def layer_pair(layer, carry):
        norm_unit(0, 0)

        @pl.when(layer == 0)
        def _():
            w_copy(0).wait()
            lax.fori_loop(0, 8, lambda i, _: prep_plain(AV, raw_v, i, 64), None)

        lax.fori_loop(0, 4, lambda c, _: phase0(layer, c), None)

        @pl.when(layer == 0)
        def _():
            w_copy(1).wait()
            lax.fori_loop(0, 8, lambda i, _: prep_plain(AK, raw_k, i, 64), None)
            w_copy(2).wait()
            lax.fori_loop(0, 8, lambda i, _: prep_plain(AQ, raw_q, i, 64), None)
            for i in range(3, 6):
                w_copy(i).wait()

        lax.fori_loop(0, 4, lambda t, _: phase1(t), None)

        for buf in (p2_k, p2_v):
            buf[0][:, pl.ds(0, HALO), :] = jnp.zeros((8, HALO, 128), f32)
        lax.fori_loop(0, NSUB // 2, lambda c, _: phase2(layer, c), None)
        return carry

    lax.fori_loop(0, 2, layer_pair, None)
    for c in range(NSUB // 2):
        out_copy(c).wait()


@jax.jit
def pallas_interleave_layers__memory_aug_infini_attn__sliding_local_dilated__prompt_kernel(
    A_x: jax.Array,
    A_wq: jax.Array,
    A_wk: jax.Array,
    A_wv: jax.Array,
    A_wo: jax.Array,
    A_beta: jax.Array,
    B_x: jax.Array,
    B_wqkv: jax.Array,
    B_wo: jax.Array,
):
    del B_x
    vmem = pltpu.VMEM
    hbm = pl.BlockSpec(memory_space=pl.ANY)
    scratch = [
        vmem((S, D), bf16),
        *[vmem((D, D), bf16)] * 4, vmem((D, 3 * D), bf16), vmem((D, D), bf16),
        *[vmem((7, 4, D // 2, 128), bf16)] * 8,
        vmem((7, 4, (NSUB + 1) * HS, 128), bf16),
        vmem((8, NSUB, 128, 128), bf16),
        vmem((8, S, 128), f32),
        vmem((H, 128), f32),
        [vmem((2, H * (DH + 1), 128), f32)] * 6,
        [vmem((2, H * (DH + 1), 128), f32)] * 2,
        [vmem((4, 128, 128), bf16)] * 8,
        [vmem((4, 128, 128), bf16)] * 6,
        [vmem((4, 128, 128), bf16)] * 8,
        [vmem((4, 128, 128), bf16)] * 6,
        [vmem((16, 128, 128), f32)] * 8,
        [vmem((8, SUB, 128), f32)] * 2,
        [vmem((7, 4, HS, 128), bf16)] * 6,
        [vmem((8, SUB, 128), f32)] * 2,
        [vmem((8, HALO + SUB, 128), f32)] * 2,
        [vmem((8, HALO + SUB, 128), f32)] * 2,
        [vmem((WIN, SUB, 128), f32)] * 2,
        pltpu.SemaphoreType.DMA((5,)),
        pltpu.SemaphoreType.DMA((6,)),
        pltpu.SemaphoreType.DMA((NSUB // 2,)),
    ]
    out = pl.pallas_call(
        _kernel,
        out_shape=jax.ShapeDtypeStruct((S, D), bf16),
        in_specs=[hbm, hbm, hbm, hbm, hbm, pl.BlockSpec(memory_space=pltpu.VMEM), hbm, hbm],
        out_specs=hbm,
        scratch_shapes=scratch,
        compiler_params=pltpu.CompilerParams(vmem_limit_bytes=112 * 1024 * 1024),
        name="interleaved_layers",
    )(A_x.reshape(S, D), A_wq, A_wk, A_wv, A_wo, A_beta.reshape(1, H), B_wqkv, B_wo)
    return out.reshape(1, S, D)
```

```python
import math
from functools import partial

import jax
import jax.numpy as jnp
from jax import lax
from jax.experimental import pallas as pl
from jax.experimental.pallas import tpu as pltpu

S = 2048
D = 1024
H = 32
DH = 32
SEG = 512
WIN, DIL = 8, 2
HALO = 16
SUB = 128
HS = SUB // 2
NSUB = S // SUB
LOG2E = math.log2(math.e)
QK_SCALE = DH ** -0.5 * LOG2E
PV_LAG = 5

f32 = jnp.float32
bf16 = jnp.bfloat16
u32 = jnp.uint32

AQ, AK, AV, AO, BQ, BK, BV, BO = range(8)


def _mm(a, b):
    return lax.dot_general(a, b, (((1,), (0,)), ((), ())), preferred_element_type=f32)


def _ld16(ref, lead, r0, n):
    return pltpu.bitcast(ref.bitcast(u32)[(*lead, pl.ds(r0, n // 2), slice(None))], bf16)


def _left_operands(a11, a12, a21, a22):
    return (a11 + a22, a21 + a22, a11, a22, a11 + a12, a21 - a11, a12 - a22)


def _right_operands(b11, b12, b21, b22):
    return (b11 + b22, b11, b12 - b22, b21 - b11, b22, b11 + b12, b21 + b22)


def _strassen(prod, emit, park, zero):
    m1 = prod(0)
    rows = pl.ds(0, m1.shape[0])
    yield m1
    m4 = prod(3)
    park[0][0, rows, :] = m1 + m4
    yield m4
    m2 = prod(1)
    emit(1, 0, m2 + m4)
    park[1][0, rows, :] = m1 - m2
    yield m2
    m6 = prod(5)
    yield m6
    m3 = prod(2)
    emit(1, 1, park[1][zero, rows, :] + (m6 + m3))
    yield m3
    m5 = prod(4)
    emit(0, 1, m3 + m5)
    yield m5
    m7 = prod(6)
    emit(0, 0, park[0][zero, rows, :] + (m7 - m5))
    yield m7


def _tree(op, xs):
    while len(xs) > 1:
        xs = [op(xs[i], xs[i + 1]) for i in range(0, len(xs), 2)]
    return xs[0]


def _chain(*gens):
    for g in gens:
        yield from g


def _take(gen, n):
    for _ in range(n):
        yield next(gen)


def fence(buf, tick, slot=0):
    if tick is not None:
        buf[buf.shape[0] - 1 - slot, pl.ds(0, 8), :] = tick[tick.shape[0] - 8:]


def _interleave(mxu, jobs):
    jobs = sorted(jobs, key=lambda j: j[0])
    n, prods = 0, []
    for i, prod in enumerate(mxu):
        prods.append(prod)
        while n < len(jobs) and jobs[n][0] < i + 1:
            r = 8 * int(max(jobs[n][0] - i, 0) * (prod.shape[0] // 8))
            jobs[n][1](prod[r:r + 8])
            n += 1
    assert n == len(jobs)
    return prods


def _spread(fns, first, last):
    return [(first + (last - first) * i / len(fns), fn) for i, fn in enumerate(fns)]


def _layernorm(x):
    d = x - jnp.sum(x, axis=-1, keepdims=True) * (1.0 / D)
    v = jnp.sum(d * d, axis=-1, keepdims=True) * (1.0 / D)
    return d * lax.rsqrt(v + 1e-5)


def _phi(t):
    return jnp.where(t > 0, t + 1.0, jnp.exp(t))


def _tile(x, c):
    return x[:, 128 * c:128 * (c + 1)]


def _kernel(x_hbm, wq_hbm, wk_hbm, wv_hbm, wo_hbm, beta_ref, bqkv_hbm, bo_hbm, out_hbm,
            xbuf, raw_q, raw_k, raw_v, raw_o, raw_bqkv, raw_bo,
            w_aq, w_ak, w_av, w_ao, w_bq, w_bk, w_bv, w_bo,
            xn, vbuf, obuf, gate, causal, perm_c, perm_r,
            p1_q, p1_pq, p1_k, p1_pk, p1_v, p1_f, p1_m, p1_mt, p1_o, p1_x, p1_s,
            p2_t, p2_x, p2_l, p2_q, p2_k, p2_v, p2_p, p2_a, stat, park,
            x_sem, w_sem, o_sem):
    wts = (w_aq, w_ak, w_av, w_ao, w_bq, w_bk, w_bv, w_bo)
    lane = lax.broadcasted_iota(jnp.int32, (128, 128), 1)
    row = lax.broadcasted_iota(jnp.int32, (128, 128), 0)
    lane8 = lax.broadcasted_iota(jnp.int32, (8, 128), 1)
    row8 = lax.broadcasted_iota(jnp.int32, (8, 128), 0)

    x_edges = (0, SUB, SUB + SEG, SUB + 2 * SEG, SUB + 3 * SEG, S)

    def x_copy(i):
        rows = pl.ds(x_edges[i], x_edges[i + 1] - x_edges[i])
        return pltpu.make_async_copy(x_hbm.at[rows], xbuf.at[rows], x_sem.at[i])

    w_pairs = ((wv_hbm, raw_v), (wk_hbm, raw_k), (wq_hbm, raw_q), (wo_hbm, raw_o),
               (bqkv_hbm, raw_bqkv), (bo_hbm, raw_bo))

    def w_copy(i):
        return pltpu.make_async_copy(w_pairs[i][0], w_pairs[i][1].at[pl.ds(0, D)], w_sem.at[i])

    def out_copy(c):
        rows = pl.ds(pl.multiple_of(c * 2 * SUB, 2 * SUB), 2 * SUB)
        return pltpu.make_async_copy(xbuf.at[rows], out_hbm.at[rows], o_sem.at[c])

    x_copy(0).start()
    w_copy(0).start()
    x_copy(1).start()
    x_copy(2).start()
    w_copy(1).start()
    x_copy(3).start()
    w_copy(2).start()
    x_copy(4).start()
    for i in range(3, 6):
        w_copy(i).start()

    hr = lax.broadcasted_iota(jnp.int32, (8, H), 0)
    hc = lax.broadcasted_iota(jnp.int32, (8, H), 1)
    sig = 1.0 / (1.0 + jnp.exp(-beta_ref[...].astype(f32)))
    for g in range(8):
        gate[g] = jnp.broadcast_to(
            jnp.sum(jnp.where(hr + 4 * g == hc, sig, 0.0), axis=1, keepdims=True), (8, 128))
    causal[0] = jnp.where(row <= lane, 0.0, -1e9 * LOG2E)

    def put_weight(m, r0, top, bot):
        n = top.shape[0]
        for t in range(4):
            ops = _right_operands(_tile(top, t), _tile(top, t + 4), _tile(bot, t), _tile(bot, t + 4))
            for i in range(7):
                wts[m][i, t, pl.ds(r0, n), :] = ops[i].astype(bf16)

    def raw_rows(raw, r0, n, c0=0):
        return raw[pl.ds(r0, n), c0:c0 + D].astype(f32)

    def prep_plain(m, raw, it, n):
        r0 = pl.multiple_of(it * n, n)
        put_weight(m, r0, raw_rows(raw, r0, n), raw_rows(raw, pl.multiple_of(r0 + D // 2, n), n))

    def fence16(buf, tick):
        if tick is not None:
            buf[pl.ds(buf.shape[0] - 16, 16), 0:128] = jnp.concatenate([tick, tick], axis=0).astype(bf16)

    turns = []

    def turn_tick(tick):
        if len(turns) < 3:
            return tick
        return pltpu.bitcast(pltpu.bitcast(tick, u32) | turns[-3], f32)

    def turned_(x):
        y = x.T
        turns.append(pltpu.bitcast(y[:16 if y.dtype == bf16 else 8], u32))
        return y

    def put_right(m, t, rows, quads):
        for i, op in enumerate(_right_operands(*quads)):
            wts[m][i, t, rows, :] = op.astype(bf16)

    def plain_jobs(m, raw, it):
        def job(r, t, tick):
            fence16(raw, tick)
            r0 = pl.multiple_of(it * 128 + r, 16)
            put_right(m, t, pl.ds(r0, 16),
                      [raw[pl.ds(pl.multiple_of(r0 + rh * (D // 2), 16), 16),
                           128 * (t + 4 * ch):128 * (t + 4 * ch + 1)].astype(f32)
                       for rh in range(2) for ch in range(2)])
        return [partial(job, r, t) for r in range(0, 128, 16) for t in range(4)]

    def regroup(buf, slot, c):
        return jnp.concatenate(
            [buf[slot, pl.ds(d, H, stride=DH + 1), :] for d in range(4 * c, 4 * c + 4)], axis=0)

    def cols_jobs(m, it, zero):
        turned, back = perm_c[m - BQ]

        def turn(c, tick):
            fence16(raw_bqkv, turn_tick(tick))
            c0 = (m - BQ) * D + 128 * c
            w = turned_(pltpu.pack_elementwise(
                [raw_bqkv[pl.ds(pl.multiple_of(it * 128 + rh * (D // 2), 128), 128), c0:c0 + 128].astype(f32)
                 for rh in range(2)], packed_dtype=bf16))
            for j in range(4):
                turned[0, pl.ds((4 * c + j) * (DH + 1), DH), :] = w[j * DH:(j + 1) * DH]

        def unturn(c, tick):
            fence(turned, pltpu.bitcast(turn_tick(tick), u32))
            back[c] = turned_(regroup(turned, zero, c))

        def job(r, t, tick):
            fence(back, pltpu.bitcast(tick, u32))
            w = [back[t + 4 * ch + zero, pl.ds(r, 16), :] for ch in range(2)]
            put_right(m, t, pl.ds(pl.multiple_of(it * 128 + r, 16), 16),
                      [pltpu.unpack_elementwise(w[ch], index=rh, packed_dtype=bf16, unpacked_dtype=f32)
                       for rh in range(2) for ch in range(2)])
        return ([partial(turn, c) for c in range(8)], [partial(unturn, c) for c in range(8)],
                [partial(job, r, t) for r in range(0, 128, 16) for t in range(4)])

    def rows_jobs(it, zero):
        def spread_heads(h, tick):
            fence16(raw_bo, tick)
            perm_r[0, pl.ds(h * (DH + 1), DH), :] = pltpu.pack_elementwise(
                [raw_bo[pl.ds(h * DH, DH), pl.ds(pl.multiple_of(it * 128 + ch * (D // 2), 128), 128)].astype(f32)
                 for ch in range(2)], packed_dtype=bf16)

        def job(d, h0, tick):
            fence(perm_r, pltpu.bitcast(tick, u32))
            w = [perm_r[zero, pl.ds(h0 * (DH + 1) + d + rh * (DH // 2), 16, stride=DH + 1), :]
                 for rh in range(2)]
            put_right(BO, it, pl.ds(d * H + h0, 16),
                      [pltpu.unpack_elementwise(w[rh], index=ch, packed_dtype=bf16, unpacked_dtype=f32)
                       for rh in range(2) for ch in range(2)])
        return [partial(spread_heads, h) for h in range(H)], [partial(job, d, h0) for d in range(DH // 2) for h0 in (0, 16)]

    def put_left(buf, r0, top, bot, ks=range(4)):
        for k in ks:
            ops = _left_operands(top(k), top(k + 4), bot(k), bot(k + 4))
            for i in range(7):
                buf[i, k, pl.ds(r0, ops[i].shape[0]), :] = ops[i].astype(bf16)
        return ops[6]

    def project(*args):
        for _ in project_steps(*args):
            pass

    def project_steps(buf, zero, r0, n, m, t, emit):
        def prod(i):
            lhs = jnp.concatenate([_ld16(buf, (i + zero, k), r0, n) for k in range(4)], axis=1)
            return _mm(lhs, _ld16(wts[m], (i, t), 0, D // 2))
        return _strassen(prod, emit, park, zero)

    def pin(buf, spare, zero):
        def job(tick):
            v = buf.bitcast(u32)[zero, 0, pl.ds(0, 8), :] | pltpu.bitcast(tick, u32)
            fence(spare, pltpu.bitcast(pltpu.roll(v, 1, 1), f32))
        return job

    def norm_jobs(src, hold, st, zero, dsts, t0, t1):
        nr = 16

        def mean_job(r, tick):
            hold(tick)
            tot = _tree(jnp.add, [src(g, r, nr) for g in range(8)])
            mean = jnp.sum(tot, axis=-1, keepdims=True) * (1.0 / D)
            st[0][0, pl.ds(r, nr), :] = jnp.broadcast_to(mean, (nr, 128))

        def var_job(r, tick):
            hold(tick)
            mean = st[0][zero, pl.ds(r, nr), :]
            dev = [src(g, r, nr) - mean for g in range(8)]
            var = jnp.sum(_tree(jnp.add, [d * d for d in dev]), axis=-1, keepdims=True) * (1.0 / D)
            st[1][0, pl.ds(r, nr), :] = jnp.broadcast_to(lax.rsqrt(var + 1e-5), (nr, 128))

        def out_job(r, k, tick):
            hold(tick)
            mean = [st[0][zero, pl.ds(rh * HS + r, 16), :] for rh in range(2)]
            rstd = [st[1][zero, pl.ds(rh * HS + r, 16), :] for rh in range(2)]
            ops = _left_operands(*[(src(k + 4 * ch, rh * HS + r, 16) - mean[rh]) * rstd[rh]
                                   for rh in range(2) for ch in range(2)])
            for i in range(7):
                for buf, r0 in dsts:
                    buf[i, k, pl.ds(r0 + r if isinstance(r0, int) else pl.multiple_of(r0 + r, 16), 16), :] = ops[i].astype(bf16)

        at = lambda f: t0 + (t1 - t0) * f / 39
        return (_spread([partial(mean_job, r) for r in range(0, SUB, nr)], at(0), at(8))
                + _spread([partial(var_job, r) for r in range(0, SUB, nr)], at(11), at(19))
                + _spread([partial(out_job, r, k) for r in range(0, HS, 16) for k in range(4)],
                          at(23), at(39)))

    def norm_unit(src_unit, dst_unit, slot, zero, t0, t1):
        def src(g, r, n):
            r0 = src_unit * SUB + r
            r0 = r0 if isinstance(r0, int) else pl.multiple_of(r0, 16)
            return xbuf[pl.ds(r0, n), 128 * g:128 * (g + 1)].astype(f32)
        return norm_jobs(src, partial(fence16, xbuf), stat[slot], zero,
                         [(xn, dst_unit * HS), (p2_l[slot], 0)], t0, t1)

    def phase0(layer, c):
        zero = c >> 4
        for i in range(4):
            @pl.when(jnp.logical_and(layer == 0, c == i))
            def _():
                x_copy(i + 1).wait()

        def values(u):
            for t in range(4):
                def emit(rh, ch, val):
                    vbuf[t + 4 * ch, c * 4 + u, pl.ds(rh * HS, HS), :] = val.astype(bf16)
                yield from project_steps(p2_l[u], zero, 0, HS, AV, t, emit)

        jobs = []
        for u in range(4):
            nxt = c * 4 + u + 1
            jobs += norm_unit(nxt if u < 3 else jnp.minimum(nxt, NSUB - 1), nxt, (u + 1) % 4, zero,
                              *((0, 21), (22, 49), (50, 77), (78, 106))[u])
        _interleave(_chain(*[values(u) for u in range(4)]), jobs)

    def phase1(t):
        zero = t >> 4
        st = {}
        hist = []
        turns.clear()
        todo = []

        def turn_q(s, ch, blk, tick):
            fence(p1_f[blk // 2], turn_tick(tick))
            y = turned_(p1_f[blk // 2][2 * ch + blk % 2 + zero])
            p1_q[2 * s + ch][blk] = (y * QK_SCALE).astype(bf16)
            if s > 0:
                p1_pq[2 * s + ch - 2][blk] = _phi(y).astype(bf16)

        def turn_v(s, blk, tick):
            tick = turn_tick(tick)
            vbuf[8, 0, pl.ds(0, 16), :] = jnp.concatenate([tick, tick], axis=0).astype(bf16)
            y = turned_(jnp.concatenate([vbuf[t + 4 * ch, 4 * s + blk] for ch in range(2)], axis=1))
            for ch in range(2):
                p1_v[2 * s + ch][blk] = y[128 * ch:128 * (ch + 1)]

        def proj(m, s, half, extra):
            def emit(rh, ch, val):
                slot = 2 * s + ch
                for u in range(2):
                    blk = 2 * half + u
                    y = val[HS * u:HS * (u + 1)]
                    rows = pl.ds(rh * HS, HS)
                    if m == AQ:
                        p1_f[half][2 * ch + u, rows, :] = y
                        continue
                    p1_k[slot][blk, rows, :] = y.astype(bf16)
                    if s < 3:
                        pk = _phi(y)
                        p1_pk[slot][blk, rows, :] = pk.astype(bf16)
                        z = jnp.sum(pk.reshape(HS // 8, 8, 128), axis=0)
                        st['dz', slot] = z + st['dz', slot] if ('dz', slot) in st else z
            jobs = _spread(todo + [partial(turn_v, s, 2 * half + (m == AK))], 0, 6) + _spread(extra, 0, 6)
            todo.clear()
            hist.extend(_interleave(
                project_steps(xn, zero, (s * 4 + half * 2) * (HS // 2), 2 * HS, m, t, emit), jobs))
            if m == AQ:
                todo.extend(partial(turn_q, s, ch, 2 * half + u) for ch in range(2) for u in (1, 0))

        def scores(a, n, s, ch, i, kb):
            slot = 2 * s + ch
            k = _ld16(p1_k[slot], (kb + zero,), 0, 128)
            for j in range(4):
                q = _ld16(p1_q[slot], (i + zero,), 16 * j, DH)
                parts = [jnp.zeros((DH * j, 128), bf16)] * (j > 0) + [q]
                parts += [jnp.zeros((DH * (3 - j), 128), bf16)] * (j < 3)
                sc = _mm(k, jnp.concatenate(parts, axis=0))
                if kb == i:
                    sc = sc + causal[zero]
                p1_s[a % len(p1_s)][j] = sc
                mx = jnp.max(sc.reshape(16, 8, 128), axis=0)
                if kb > 0:
                    mx = jnp.maximum(mx, st['m', n, j])
                if kb == i:
                    p1_x[n % len(p1_x)][j] = jnp.broadcast_to(jnp.max(mx, axis=0, keepdims=True), (8, 128))
                st['m', n, j] = mx
            return sc

        def values(a, n, s, ch, i, kb, prev):
            g = t + 4 * ch
            buf = p1_s[a % len(p1_s)]
            NT_ = 8
            acc = p1_o[n % len(p1_o)]
            mx = [p1_x[n % len(p1_x)][j + zero] for j in range(4)]
            l = [st.get(('l', n, j)) for j in range(4)]
            p = [[None] * 16 for _ in range(4)]
            for b in reversed(range(16)):
                if (b + 1) % (16 // NT_) == 0:
                    r = 128 + (15 - b) * 96 // 128 * 8
                    if prev[r // 128] is not None:
                        fence(buf, prev[r // 128][r % 128:r % 128 + 8])
                for j in range(4):
                    p[j][b] = jnp.exp2(buf[j + zero, pl.ds(8 * b, 8), :] - mx[j])
                    l[j] = p[j][b] if l[j] is None else l[j] + p[j][b]
            if kb == i:
                tot = [jnp.sum(x, axis=0, keepdims=True) for x in l]
                tot = jnp.where(row8 < 2, jnp.where(row8 == 0, tot[0], tot[1]),
                                jnp.where(row8 == 2, tot[2], tot[3]))
                scale = (1.0 - gate[g]) / tot
            for j in range(4):
                st['l', n, j] = l[j]
                head = pl.ds(DH * j, DH)
                o = _mm(_ld16(p1_v[2 * s + ch], (kb + zero,), 16 * j, DH),
                        jnp.concatenate(p[j], axis=0))
                if kb > 0:
                    o = o + acc[j][zero]
                if kb == i:
                    o = o * scale[j:j + 1]
                    if s > 0:
                        o = o + p1_m[ch][i + zero, head, :]
                    obuf[g, pl.ds(SEG * s + 128 * i + DH * j, DH), :] = o
                else:
                    acc[j][0] = o

        def mem_read(s, ch):
            z = jnp.sum(st['z', ch], axis=0, keepdims=True)
            lhs = jnp.concatenate([jnp.where((lane8 >> 5) == row8, z, 0.0),
                                   jnp.zeros((8, 128), f32),
                                   jnp.where((lane >> 5) == (row >> 5), p1_mt[ch][zero], 0.0)],
                                  axis=0).astype(bf16)
            for b in range(4):
                nd = _mm(lhs, _ld16(p1_pq[2 * s + ch - 2], (b + zero,), 0, 128))
                inv = gate[t + 4 * ch] / (nd[0:8] + 1e-6)
                for j in range(4):
                    p1_m[ch][b, pl.ds(DH * j, DH), :] = nd[16 + DH * j:16 + DH * (j + 1)] * inv[j:j + 1]
            hist.append(nd[16:])

        def mem_update(s, ch):
            slot = 2 * s + ch
            v = jnp.concatenate([_ld16(p1_v[slot], (b + zero,), 0, 128) for b in range(4)], axis=1)
            pk = jnp.concatenate([_ld16(p1_pk[slot], (b + zero,), 0, 128) for b in range(4)], axis=0)
            mt, z = _mm(v, pk), st['dz', slot]
            hist.append(mt)
            if s > 0:
                mt, z = mt + p1_mt[ch][zero], z + st['z', ch]
            p1_mt[ch][0] = mt
            st['z', ch] = z

        tiles = []
        for s in range(4):
            for ch in range(2):
                for i in (3, 2, 1, 0):
                    n = (2 * s + ch) * 4 + (3 - i)
                    tiles += [(n, s, ch, i, kb) for kb in range(i + 1)]
        cq, ck, cv = (cols_jobs(m, t, zero) for m in (BQ, BK, BV))
        pa, (ra, rb) = plain_jobs(AO, raw_o, t), rows_jobs(t, zero)
        halves = lambda x: (x[:len(x) // 2], x[len(x) // 2:])
        side = [cq[0], pa, halves(ck[0])[0], halves(ck[0])[1] + halves(cv[0])[0],
                cq[1], ra, halves(cv[0])[1], halves(ck[1])[0],
                halves(ck[1])[1] + halves(cq[2])[0], halves(cq[2])[1], halves(cv[1])[0], halves(cv[1])[1],
                ck[2], halves(rb)[0], halves(rb)[1], cv[2]]
        blocks = ((AQ, 1), (AQ, 0), (AK, 0), (AK, 1))
        for m, half in blocks:
            proj(m, 0, half, side.pop(0))
        LAG = PV_LAG
        done = 0
        for a in range(len(tiles) + 2):
            s, pos = divmod(a, 20)
            if s < 3 and pos % 5 == 0:
                m, half = blocks[pos // 5]
                proj(m, s + 1, half, side.pop(0))
            upto = max(a + 1 - LAG, {76: 73, 77: 74, 78: 76, 79: 77, 80: 79, 81: 80}.get(a, 0))
            for b in range(done, upto):
                n, s, ch, i, kb = tiles[b]
                if i == 3 and kb == 0 and s > 0:
                    mem_read(s, ch)
                if i == 2 and kb == 1 and s < 3:
                    mem_update(s, ch)
            prev = hist[-2:]
            hist.append(scores(a, *tiles[a]) if a < len(tiles) else None)
            for b in range(done, upto):
                values(b, *tiles[b], prev if b == done else [None, None])
            done = max(done, upto)

    def out_jobs(unit, u, zero, t0, t1):
        def turn(g, tick):
            fence(obuf, tick)
            p2_t[u][g] = obuf[g, pl.ds(pl.multiple_of(unit * SUB, SUB), SUB), :].T

        def operands(r, k, tick):
            fence(p2_t[u], tick)
            put_left(p2_l[u], r, lambda g: p2_t[u][g + zero, pl.ds(r, 16), :],
                     lambda g: p2_t[u][g + zero, pl.ds(HS + r, 16), :], (k,))
        tm = t0 + (t1 - t0) * 0.4
        return (_spread([partial(turn, g) for g in range(8)], t0, tm)
                + _spread([partial(operands, r, k) for r in range(0, HS, 16) for k in range(4)], tm + 4, t1))

    def phase2(layer, c):
        zero = c >> 4
        base = [pl.multiple_of((2 * c + u) * SUB, SUB) for u in range(2)]

        def rows(u, r, n):
            return pl.ds(pl.multiple_of(base[u] + r, 16), n)

        def infini_out(u):
            for t in range(4):
                def emit(rh, ch, val):
                    g = t + 4 * ch
                    x = xbuf[rows(u, rh * HS, HS), 128 * g:128 * (g + 1)].astype(f32)
                    p2_x[u][g, pl.ds(rh * HS, HS), :] = x + val
                yield from project_steps(p2_l[u], zero, 0, HS, AO, t, emit)

        def norm(u, t0, t1):
            return norm_jobs(lambda g, r, n: p2_x[u][g + zero, pl.ds(r, n), :], partial(fence, p2_x[u]),
                             stat[u], zero, [(p2_l[2 + u], 0)], t0, t1)

        def local_proj(u, m, dst, off):
            for t in range(4):
                def emit(rh, ch, val):
                    dst[u][t + 4 * ch, pl.ds(off + rh * HS, HS), :] = val
                    if off and rh == 1 and u == 0:
                        dst[1][t + 4 * ch, pl.ds(0, HALO), :] = val[HS - HALO:]
                yield from project_steps(p2_l[2 + u], zero, 0, HS, m, t, emit)

        def attend(u, t0, t1, t2, t3):
            NW = 2

            def logits(b, w0, tick):
                for buf in (p2_q[u], p2_k[u]):
                    fence(buf, tick)
                lg = {}
                for g in range(8):
                    q = p2_q[u][g + zero, pl.ds(8 * b, 8), :]
                    for w in range(w0, w0 + NW):
                        qk = q * p2_k[u][g + zero, pl.ds(HALO + 8 * b - DIL * w, 8), :]
                        lg[w] = qk if g == 0 else lg[w] + qk
                for w in range(w0, w0 + NW):
                    a = lg[w]
                    a = (a + pltpu.roll(a, 64, 1)) + (pltpu.roll(a, 32, 1) + pltpu.roll(a, 96, 1))
                    a = a * QK_SCALE
                    if u == 0 and 8 * b < DIL * w:
                        a = jnp.where(base[0] + 8 * b + row8 >= DIL * w, a, -1e9 * LOG2E)
                    p2_a[u][b][1][w] = a

            def softmax(b, tick):
                fence(p2_a[u][b][1], tick)
                lg = [p2_a[u][b][1][w + zero] for w in range(WIN)]
                mx = _tree(jnp.maximum, lg)
                ex = [jnp.exp2(a - mx) for a in lg]
                inv = 1.0 / _tree(jnp.add, ex)
                for w in range(WIN):
                    p2_a[u][b][2][w] = ex[w] * inv

            def mix(b, g0, tick):
                for buf in (p2_v[u], p2_a[u][b][2]):
                    fence(buf, tick)
                acc = {}
                for w in range(WIN):
                    p = p2_a[u][b][2][w + zero]
                    for g in range(g0, g0 + NW):
                        pv = p * p2_v[u][g + zero, pl.ds(HALO + 8 * b - DIL * w, 8), :]
                        acc[g] = pv if w == 0 else acc[g] + pv
                for g in range(g0, g0 + NW):
                    p2_p[u][g, pl.ds(8 * b, 8), :] = acc[g]

            def operands(r, k, tick):
                fence(p2_p[u], tick)
                put_left(p2_l[4 + u], r, lambda g: p2_p[u][g + zero, pl.ds(r, 16), :],
                         lambda g: p2_p[u][g + zero, pl.ds(HS + r, 16), :], (k,))

            order = [rh * 8 + 2 * j + i for j in range(4) for rh in range(2) for i in range(2)]
            step = (t1 - t0) / 16
            lag = step + 3
            mstep = (t3 - t2) / 4
            return (_spread([partial(logits, b, w) for b in order for w in range(0, WIN, NW)], t0, t1)
                    + _spread([partial(softmax, b) for b in order],
                              t0 + lag + step * NW / 16, t1 + lag + step * NW / 16)
                    + _spread([partial(mix, b, g) for b in order for g in range(0, 8, NW)], t2, t3)
                    + [(t2 + mstep * (j + 1) + 0.5 * k, partial(operands, 16 * j, k))
                       for j in range(4) for k in range(4)])

        def local_out(u):
            for t in range(4):
                def emit(rh, ch, val):
                    g = t + 4 * ch
                    y = p2_x[u][g + zero, pl.ds(rh * HS, HS), :] + val
                    xbuf[rows(u, rh * HS, HS), 128 * g:128 * (g + 1)] = y.astype(bf16)
                yield from project_steps(p2_l[4 + u], zero, 0, HS, BO, t, emit)

        _interleave(
            _chain(infini_out(0), infini_out(1),
                   local_proj(0, BK, p2_k, HALO), local_proj(0, BQ, p2_q, 0), local_proj(0, BV, p2_v, HALO),
                   local_proj(1, BK, p2_k, HALO), local_proj(1, BQ, p2_q, 0), local_proj(1, BV, p2_v, HALO),
                   local_out(0), local_out(1)),
            out_jobs(2 * c + 1, 1, zero, 0, 22) + out_jobs(jnp.minimum(2 * c + 2, NSUB - 1), 0, zero, 252, 277)
            + norm(0, 28, 49) + norm(1, 70, 112)
            + attend(0, 112, 152, 156, 194) + attend(1, 196, 222.0, 224, 246.0))
        for buf in (p2_k, p2_v):
            for g in range(8):
                buf[0][g, pl.ds(0, HALO), :] = buf[1][g + zero, pl.ds(SUB, HALO), :]

        @pl.when(layer == 1)
        def _():
            out_copy(c).start()

    x_copy(0).wait()

    def layer_pair(layer, carry):
        for _, job in norm_unit(0, 0, 0, layer >> 4, 0, 1):
            job(None)

        @pl.when(layer == 0)
        def _():
            w_copy(0).wait()
            lax.fori_loop(0, 8, lambda i, _: prep_plain(AV, raw_v, i, 64), None)

        lax.fori_loop(0, 4, lambda c, _: phase0(layer, c), None)

        @pl.when(layer == 0)
        def _():
            w_copy(1).wait()
            lax.fori_loop(0, 8, lambda i, _: prep_plain(AK, raw_k, i, 64), None)
            w_copy(2).wait()
            lax.fori_loop(0, 8, lambda i, _: prep_plain(AQ, raw_q, i, 64), None)
            for i in range(3, 6):
                w_copy(i).wait()

        lax.fori_loop(0, 4, lambda t, _: phase1(t), None)

        for _, job in out_jobs(layer >> 4, 0, layer >> 4, 0, 22):
            job(None)
        for buf in (p2_k, p2_v):
            buf[0][0:8, pl.ds(0, HALO), :] = jnp.zeros((8, HALO, 128), f32)
        lax.fori_loop(0, NSUB // 2, lambda c, _: phase2(layer, c), None)
        return carry

    lax.fori_loop(0, 2, layer_pair, None)
    for c in range(NSUB // 2):
        out_copy(c).wait()


@jax.jit
def pallas_interleave_layers__memory_aug_infini_attn__sliding_local_dilated__prompt_kernel(
    A_x: jax.Array,
    A_wq: jax.Array,
    A_wk: jax.Array,
    A_wv: jax.Array,
    A_wo: jax.Array,
    A_beta: jax.Array,
    B_x: jax.Array,
    B_wqkv: jax.Array,
    B_wo: jax.Array,
):
    del B_x
    vmem = pltpu.VMEM
    hbm = pl.BlockSpec(memory_space=pl.ANY)
    scratch = [
        vmem((S + 16, D), bf16),
        *[vmem((D + 16, D), bf16)] * 4, vmem((D + 16, 3 * D), bf16), vmem((D + 16, D), bf16),
        *[vmem((7, 4, D // 2, 128), bf16)] * 8,
        vmem((7, 4, (NSUB + 1) * HS, 128), bf16),
        vmem((9, NSUB, 128, 128), bf16),
        vmem((9, S, 128), f32),
        vmem((8, 8, 128), f32),
        vmem((2, 128, 128), f32),
        [[vmem((2, H * (DH + 1), 128), u32), vmem((9, 128, 128), u32)]] * 3,
        vmem((2, H * (DH + 1), 128), u32),
        [vmem((4, 128, 128), bf16)] * 8,
        [vmem((4, 128, 128), bf16)] * 6,
        [vmem((4, 128, 128), bf16)] * 8,
        [vmem((4, 128, 128), bf16)] * 6,
        [vmem((4, 128, 128), bf16)] * 8,
        [vmem((5, 128, 128), f32)] * 2,
        [vmem((4, 128, 128), f32)] * 2,
        [vmem((2, 128, 128), f32)] * 2,
        [[vmem((2, DH, 128), f32)] * 4] * 4,
        [vmem((4, 8, 128), f32)] * 8,
        [vmem((5, 128, 128), f32)] * 10,
        [vmem((10, SUB, 128), f32)] * 2,
        [vmem((10, SUB, 128), f32)] * 2,
        [vmem((8, 4, HS, 128), bf16)] * 6,
        [vmem((10, SUB, 128), f32)] * 2,
        [vmem((10, HALO + SUB, 128), f32)] * 2,
        [vmem((10, HALO + SUB, 128), f32)] * 2,
        [vmem((WIN + 2, SUB, 128), f32)] * 2,
        [[[vmem((WIN + 2, 8, 128), f32)] * 3] * 16] * 2,
        [[vmem((2, SUB, 128), f32)] * 2] * 4,
        [vmem((2, SUB, 128), f32)] * 2,
        pltpu.SemaphoreType.DMA((5,)),
        pltpu.SemaphoreType.DMA((6,)),
        pltpu.SemaphoreType.DMA((NSUB // 2,)),
    ]
    out = pl.pallas_call(
        _kernel,
        out_shape=jax.ShapeDtypeStruct((S, D), bf16),
        in_specs=[hbm, hbm, hbm, hbm, hbm, pl.BlockSpec(memory_space=pltpu.VMEM), hbm, hbm],
        out_specs=hbm,
        scratch_shapes=scratch,
        compiler_params=pltpu.CompilerParams(vmem_limit_bytes=112 * 1024 * 1024, flags={"XLA_TPU_FORCE_LP_LLO_SCHEDULER": True}),
        name="interleaved_layers",
    )(A_x.reshape(S, D), A_wq, A_wk, A_wv, A_wo, A_beta.reshape(1, H), B_wqkv, B_wo)
    return out.reshape(1, S, D)
```

```python
import math
from functools import partial

import jax
import jax.numpy as jnp
import numpy as np
from jax import lax
from jax.experimental import pallas as pl
from jax.experimental.pallas import tpu as pltpu

S = 2048
D = 1024
H = 32
DH = 32
SEG = 512
WIN, DIL = 8, 2
HALO = 16
SUB = 128
HS = SUB // 2
NSUB = S // SUB
LOG2E = math.log2(math.e)
QK_SCALE = DH ** -0.5 * LOG2E
PV_LAG = 5

f32 = jnp.float32
bf16 = jnp.bfloat16
u32 = jnp.uint32

AQ, AK, AV, AO, BQ, BK, BV, BO = range(8)


def _mm(a, b):
    return lax.dot_general(a, b, (((1,), (0,)), ((), ())), preferred_element_type=f32)


def _ld16(ref, lead, r0, n):
    return pltpu.bitcast(ref.bitcast(u32)[(*lead, pl.ds(r0, n // 2), slice(None))], bf16)


def _left_operands(a11, a12, a21, a22):
    return (a11 + a22, a21 + a22, a11, a22, a11 + a12, a21 - a11, a12 - a22)


def _right_operands(b11, b12, b21, b22):
    return (b11 + b22, b11, b12 - b22, b21 - b11, b22, b11 + b12, b21 + b22)


def _strassen(prod, emit, park, zero):
    m1 = prod(0)
    rows = pl.ds(0, m1.shape[0])
    yield m1
    m4 = prod(3)
    park[0][0, rows, :] = m1 + m4
    yield m4
    m2 = prod(1)
    emit(1, 0, m2 + m4)
    park[1][0, rows, :] = m1 - m2
    yield m2
    m6 = prod(5)
    yield m6
    m3 = prod(2)
    emit(1, 1, park[1][zero, rows, :] + (m6 + m3))
    yield m3
    m5 = prod(4)
    emit(0, 1, m3 + m5)
    yield m5
    m7 = prod(6)
    emit(0, 0, park[0][zero, rows, :] + (m7 - m5))
    yield m7


def _strassen_lean(prod, emit, park, zero):
    m = prod(0)
    park[0][0] = m
    yield m
    m = prod(3)
    park[1][0] = park[0][zero] + m
    park[2][0] = m
    yield m
    m = prod(1)
    emit(1, 0, park[2][zero] + m)
    park[3][0] = park[0][zero] - m
    yield m
    m = prod(5)
    park[4][0] = park[3][zero] + m
    yield m
    m = prod(2)
    emit(1, 1, park[4][zero] + m)
    park[5][0] = m
    yield m
    m = prod(4)
    emit(0, 1, park[5][zero] + m)
    park[6][0] = park[1][zero] - m
    yield m
    m = prod(6)
    emit(0, 0, park[6][zero] + m)
    yield m


def _tree(op, xs):
    while len(xs) > 1:
        xs = [op(xs[i], xs[i + 1]) for i in range(0, len(xs), 2)]
    return xs[0]


def _chain(*gens):
    for g in gens:
        yield from g


def _take(gen, n):
    for _ in range(n):
        yield next(gen)


def fence(buf, tick, slot=0):
    if tick is not None:
        buf[buf.shape[0] - 1 - slot, pl.ds(0, 8), :] = tick[tick.shape[0] - 8:]


def _paced(mxu, jobs):
    jobs = sorted(jobs, key=lambda j: j[0])
    n = 0
    for i, prod in enumerate(mxu):
        while n < len(jobs) and jobs[n][0] < i + 1:
            r = 8 * int(max(jobs[n][0] - i, 0) * (prod.shape[0] // 8))
            jobs[n][1](prod[r:r + 8])
            n += 1
        yield prod
    assert n == len(jobs)


def _interleave(mxu, jobs):
    for _ in _paced(mxu, jobs):
        pass


def _spread(fns, first, last):
    return [(first + (last - first) * i / len(fns), fn) for i, fn in enumerate(fns)]


def _layernorm(x):
    d = x - jnp.sum(x, axis=-1, keepdims=True) * (1.0 / D)
    v = jnp.sum(d * d, axis=-1, keepdims=True) * (1.0 / D)
    return d * lax.rsqrt(v + 1e-5)


def _pair(lo, hi):
    return (pltpu.bitcast(lo.astype(f32), u32) >> 16) | pltpu.bitcast(hi.astype(f32), u32)


def _unpair(w, i):
    return pltpu.bitcast(w & np.uint32(0xFFFF0000) if i else w << 16, f32)


def _swap_odd_heads(lo, hi):
    odd = (lax.broadcasted_iota(jnp.int32, lo.shape, 1) & DH) != 0
    return jnp.where(odd, hi, lo), jnp.where(odd, lo, hi)


def _phi(t):
    return jnp.where(t > 0, t + 1.0, jnp.exp(t))


def _tile(x, c):
    return x[:, 128 * c:128 * (c + 1)]


def _kernel(x_hbm, wq_hbm, wk_hbm, wv_hbm, wo_hbm, beta_ref, bqkv_hbm, bo_hbm, out_hbm,
            xbuf, raw_q, raw_k, raw_v, raw_o, raw_bqkv, raw_bo,
            w_aq, w_ak, w_av, w_ao, w_bq, w_bk, w_bv, w_bo,
            xn, vbuf, obuf, gate, causal, perm_c, perm_r,
            p0_l, p1_q, p1_pq, p1_k, p1_pk, p1_v, p1_f, p1_m, p1_mt, p1_x, p1_l, p1_p, p1_s,
            p2_t, p2_x, p2_l, p2_q, p2_k, p2_v, p2_p, p2_a, stat, park,
            x_sem, w_sem, o_sem):
    wts = (w_aq, w_ak, w_av, w_ao, w_bq, w_bk, w_bv, w_bo)
    lane = lax.broadcasted_iota(jnp.int32, (128, 128), 1)
    row = lax.broadcasted_iota(jnp.int32, (128, 128), 0)
    lane8 = lax.broadcasted_iota(jnp.int32, (8, 128), 1)
    row8 = lax.broadcasted_iota(jnp.int32, (8, 128), 0)

    x_edges = (0, SUB, SUB + SEG, SUB + 2 * SEG, SUB + 3 * SEG, S)

    def x_copy(i):
        rows = pl.ds(x_edges[i], x_edges[i + 1] - x_edges[i])
        return pltpu.make_async_copy(x_hbm.at[rows], xbuf.at[rows], x_sem.at[i])

    w_pairs = ((wv_hbm, raw_v), (wk_hbm, raw_k), (wq_hbm, raw_q), (wo_hbm, raw_o), (bo_hbm, raw_bo))

    def w_copy(i):
        return pltpu.make_async_copy(w_pairs[i][0], w_pairs[i][1].at[pl.ds(0, D)], w_sem.at[i])

    def bqkv_copies(t):
        rows = [pl.ds(pl.multiple_of(t * 128 + rh * (D // 2), 128), 128) for rh in range(2)]
        return [pltpu.make_async_copy(bqkv_hbm.at[r], raw_bqkv.at[r], w_sem.at[5 + rh])
                for rh, r in enumerate(rows)]

    def out_copy(c):
        rows = pl.ds(pl.multiple_of(c * 2 * SUB, 2 * SUB), 2 * SUB)
        return pltpu.make_async_copy(xbuf.at[rows], out_hbm.at[rows], o_sem.at[c])

    x_copy(0).start()
    w_copy(0).start()

    hr = lax.broadcasted_iota(jnp.int32, (8, H), 0)
    hc = lax.broadcasted_iota(jnp.int32, (8, H), 1)
    sig = 1.0 / (1.0 + jnp.exp(-beta_ref[...].astype(f32)))
    for g in range(8):
        gate[g] = jnp.broadcast_to(
            jnp.sum(jnp.where(hr + 4 * g == hc, sig, 0.0), axis=1, keepdims=True), (8, 128))
    for i, query in enumerate((lane, lane ^ 64, lane | 64)):
        causal[i] = jnp.where(row <= query, 0.0, -1e9 * LOG2E)

    def put_weight(m, r0, top, bot):
        n = top.shape[0]
        for t in range(4):
            ops = _right_operands(_tile(top, t), _tile(top, t + 4), _tile(bot, t), _tile(bot, t + 4))
            for i in range(7):
                wts[m][i, t, pl.ds(r0, n), :] = ops[i].astype(bf16)

    def raw_rows(raw, r0, n, c0=0):
        return raw[pl.ds(r0, n), c0:c0 + D].astype(f32)

    def prep_plain(m, raw, it, n):
        r0 = pl.multiple_of(it * n, n)
        put_weight(m, r0, raw_rows(raw, r0, n), raw_rows(raw, pl.multiple_of(r0 + D // 2, n), n))

    def fence16(buf, tick):
        if tick is not None:
            buf[pl.ds(buf.shape[0] - 16, 16), 0:128] = jnp.concatenate([tick, tick], axis=0).astype(bf16)

    turns = []

    def turn_tick(tick):
        if len(turns) < 3:
            return tick
        return pltpu.bitcast(pltpu.bitcast(tick, u32) | turns[-3], f32)

    def turned_(x):
        y = x.T
        turns.append(pltpu.bitcast(y[:16 if y.dtype == bf16 else 8], u32))
        return y

    def put_right(m, t, rows, quads):
        for i, op in enumerate(_right_operands(*quads)):
            wts[m][i, t, rows, :] = op.astype(bf16)

    def plain_jobs(m, raw, it):
        def job(r, t, tick):
            fence16(raw, tick)
            r0 = pl.multiple_of(it * 128 + r, 16)
            put_right(m, t, pl.ds(r0, 16),
                      [raw[pl.ds(pl.multiple_of(r0 + rh * (D // 2), 16), 16),
                           128 * (t + 4 * ch):128 * (t + 4 * ch + 1)].astype(f32)
                       for rh in range(2) for ch in range(2)])
        return [partial(job, r, t) for r in range(0, 128, 16) for t in range(4)]

    def regroup(buf, slot, c):
        return jnp.concatenate(
            [buf[slot, pl.ds(d, H, stride=DH + 1), :] for d in range(4 * c, 4 * c + 4)], axis=0)

    def cols_jobs(m, it, zero):
        turned, back = perm_c[m - BQ]

        def turn(c, tick):
            fence16(raw_bqkv, turn_tick(tick))
            c0 = (m - BQ) * D + 128 * c
            w = turned_(_pair(
                *[raw_bqkv[pl.ds(pl.multiple_of(it * 128 + rh * (D // 2), 128), 128), c0:c0 + 128]
                  for rh in range(2)]))
            for j in range(4):
                turned[0, pl.ds((4 * c + j) * (DH + 1), DH), :] = w[j * DH:(j + 1) * DH]

        def unturn(c, tick):
            fence(turned, pltpu.bitcast(turn_tick(tick), u32))
            back[c] = turned_(regroup(turned, zero, c))

        def job(r, t, tick):
            fence(back, pltpu.bitcast(tick, u32))
            w = [back[t + 4 * ch + zero, pl.ds(r, 16), :] for ch in range(2)]
            put_right(m, t, pl.ds(pl.multiple_of(it * 128 + r, 16), 16),
                      [_unpair(w[ch], rh) for rh in range(2) for ch in range(2)])
        return ([partial(turn, c) for c in range(8)], [partial(unturn, c) for c in range(8)],
                [partial(job, r, t) for r in range(0, 128, 16) for t in range(4)])

    def rows_jobs(it, zero):
        def spread_heads(h, tick):
            fence16(raw_bo, tick)
            perm_r[0, pl.ds(h * (DH + 1), DH), :] = _pair(
                *[raw_bo[pl.ds(h * DH, DH), pl.ds(pl.multiple_of(it * 128 + ch * (D // 2), 128), 128)]
                  for ch in range(2)])

        def job(d, h0, tick):
            fence(perm_r, pltpu.bitcast(tick, u32))
            w = [perm_r[zero, pl.ds(h0 * (DH + 1) + d + rh * (DH // 2), 16, stride=DH + 1), :]
                 for rh in range(2)]
            put_right(BO, it, pl.ds(d * H + h0, 16),
                      [_unpair(w[rh], ch) for rh in range(2) for ch in range(2)])
        return [partial(spread_heads, h) for h in range(H)], [partial(job, d, h0) for d in range(DH // 2) for h0 in (0, 16)]

    def put_left(buf, r0, top, bot, ks=range(4)):
        for k in ks:
            ops = _left_operands(top(k), top(k + 4), bot(k), bot(k + 4))
            for i in range(7):
                buf[i, k, pl.ds(r0, ops[i].shape[0]), :] = ops[i].astype(bf16)
        return ops[6]

    def project(*args):
        for _ in project_steps(*args):
            pass

    def project_steps(buf, zero, r0, n, m, t, emit):
        def prod(i):
            lhs = jnp.concatenate([_ld16(buf, (i + zero, k), r0, n) for k in range(4)], axis=1)
            return _mm(lhs, _ld16(wts[m], (i, t), 0, D // 2))
        return (_strassen_lean if n == SUB and 1 else _strassen)(prod, emit, park, zero)

    def norm_jobs(src, hold, st, zero, dsts, t0, t1):
        def row_mean(parts):
            tot = parts[0]
            for x in parts[1:]:
                tot = tot + x
            return jnp.sum(tot, axis=-1, keepdims=True) * (1.0 / D)

        def mean_job(r, tick):
            hold(tick)
            st[0][0, pl.ds(r, 16), :] = jnp.broadcast_to(
                row_mean([src(g, r, 16) for g in range(8)]), (16, 128))

        def var_job(r, tick):
            fence(st[0], tick)
            mean = st[0][zero, pl.ds(r, 8), :]
            dev = [src(g, r, 8) - mean for g in range(8)]
            st[1][0, pl.ds(r, 8), :] = jnp.broadcast_to(
                lax.rsqrt(row_mean([d * d for d in dev]) + 1e-5), (8, 128))

        def out_job(r, k, which, tick):
            hold(tick)
            fence(st[0], tick)
            fence(st[1], tick)
            mean = [st[0][zero, pl.ds(rh * HS + r, 16), :] for rh in range(2)]
            rstd = [st[1][zero, pl.ds(rh * HS + r, 16), :] for rh in range(2)]
            ops = _left_operands(*[(src(k + 4 * ch, rh * HS + r, 16) - mean[rh]) * rstd[rh]
                                   for rh in range(2) for ch in range(2)])
            for i in which:
                for buf, r0 in dsts:
                    buf[i, k, pl.ds(r0 + r if isinstance(r0, int) else pl.multiple_of(r0 + r, 16), 16), :] = ops[i].astype(bf16)

        work = t1 - t0 - 4
        return (_spread([partial(mean_job, r) for r in range(0, SUB, 16)], t0, t0 + 0.15 * work)
                + _spread([partial(var_job, r) for r in range(0, SUB, 8)],
                          t0 + 2 + 0.15 * work, t0 + 2 + 0.45 * work)
                + _spread([partial(out_job, r, k, which) for r in range(0, HS, 16) for k in range(4)
                           for which in (((2, 4, 6), (0, 1, 3, 5)) if 1 else (range(7),))],
                          t0 + 4 + 0.45 * work, t1))

    def norm_unit(src_unit, dst_unit, slot, zero, t0, t1):
        def src(g, r, n):
            r0 = src_unit * SUB + r
            r0 = pl.multiple_of(r0, 8)
            return xbuf[pl.ds(r0, n), 128 * g:128 * (g + 1)].astype(f32)
        return norm_jobs(src, partial(fence16, xbuf), stat[slot], zero,
                         [(xn, dst_unit * HS), (p0_l[slot], 0)], t0, t1)

    def phase0(layer, c):
        zero = c >> 4
        for i in range(4):
            @pl.when(jnp.logical_and(layer == 0, c == i))
            def _():
                x_copy(i + 1).wait()
                for j in ((2, 3, 4), (), (), ())[i]:
                    x_copy(j).start()
                for j in ((), (1, 2), (3, 4), ())[i]:
                    w_copy(j).start()
                if i == 2:
                    for cp in bqkv_copies(zero):
                        cp.start()

        def values(u):
            for t in range(4):
                def emit(rh, ch, val):
                    vbuf[t + 4 * ch, c * 4 + u, pl.ds(rh * HS, HS), :] = val.astype(bf16)
                yield from project_steps(p0_l[u], zero, 0, HS, AV, t, emit)

        jobs = []
        for u in range(4):
            nxt = c * 4 + u + 1
            jobs += norm_unit(nxt if u < 3 else jnp.minimum(nxt, NSUB - 1), nxt, (u + 1) % 4, zero,
                              *((0, 24), (24, 52), (52, 80), (80, 110))[u])
        _interleave(_chain(*[values(u) for u in range(4)]), jobs)

    def phase1(layer, t):
        zero = t >> 4

        @pl.when(layer == 0)
        def _():
            for cp in bqkv_copies(t):
                cp.wait()

            @pl.when(t < 3)
            def _():
                for cp in bqkv_copies(t + 1):
                    cp.start()

        st = {}
        never = row8 < zero
        turns.clear()
        todo = []

        def turn_q(s, ch, blk, tick):
            fence(p1_f[blk // 2], turn_tick(tick))
            y = p1_f[blk // 2][2 * ch + blk % 2 + zero]
            y = turned_(jnp.concatenate(_swap_odd_heads(y[:HS], y[HS:]), axis=0))
            p1_q[2 * s + ch][blk][0] = (y * QK_SCALE).astype(bf16)
            if s > 0:
                p1_pq[2 * s + ch - 2][blk][0] = _phi(y).astype(bf16)

        def turn_v(s, blk, tick):
            tick = turn_tick(tick)
            vbuf[8, 0, pl.ds(0, 16), :] = jnp.concatenate([tick, tick], axis=0).astype(bf16)
            y = turned_(jnp.concatenate([vbuf[t + 4 * ch, 4 * s + blk] for ch in range(2)], axis=1))
            for ch in range(2):
                p1_v[2 * s + ch][blk][0] = y[128 * ch:128 * (ch + 1)]

        def proj(m, s, half, extra):
            def emit(rh, ch, val):
                slot = 2 * s + ch
                for u in range(2):
                    blk = 2 * half + u
                    y = val[HS * u:HS * (u + 1)]
                    rows = pl.ds(rh * HS, HS)
                    if m == AQ:
                        p1_f[half][2 * ch + u, rows, :] = y
                        continue
                    p1_k[slot][blk][0, rows, :] = y.astype(bf16)
                    if s < 3:
                        pk = _phi(y)
                        p1_pk[slot][blk][0, rows, :] = pk.astype(bf16)
                        z = jnp.sum(pk.reshape(HS // 8, 8, 128), axis=0)
                        st['dz', slot] = z + st['dz', slot] if ('dz', slot) in st else z
            jobs = (_spread(todo + [partial(turn_v, s, 2 * half + (m == AK))], 0, 4)
                    + _spread(extra, 0, 7))
            todo.clear()
            yield from _paced(
                project_steps(xn, zero, (s * 4 + half * 2) * (HS // 2), 2 * HS, m, t, emit), jobs)
            if m == AQ:
                todo.extend(partial(turn_q, s, ch, 2 * half + u) for ch in range(2) for u in (1, 0))

        def scores(a, n, s, ch, i, kb):
            slot = 2 * s + ch
            buf = p1_s[a % len(p1_s)]
            qbuf = p1_q[slot][i].bitcast(u32)

            def queries(first, parts):
                pad = (first, 4 - first - len(parts))
                parts = ([jnp.zeros((16 * pad[0], 128), u32)] * (pad[0] > 0) + parts
                         + [jnp.zeros((16 * pad[1], 128), u32)] * (pad[1] > 0))
                return pltpu.bitcast(jnp.concatenate(parts, axis=0), bf16)

            nk = HS if kb == i else 128
            k = _ld16(p1_k[slot][kb], (zero,), 0, nk)
            mx = []
            for j in range(4):
                sc = _mm(k, queries(j, [qbuf[zero, pl.ds(16 * j, 16), :]]))
                if kb == i:
                    sc = sc + causal[j % 2 + zero, pl.ds(0, HS), :]
                buf[j, pl.ds(0, nk), :] = sc
                m = jnp.max(sc.reshape(nk // 8, 8, 128), axis=0)
                mx.append(jnp.maximum(m, st['m', n, j]) if kb > 0 else m)
                st['m', n, j] = mx[j]
            if kb < i:
                return sc
            upper = lax.broadcasted_iota(jnp.int32, (16, 128), 1) >= HS
            for j in (0, 2):
                m = None
                for r in (HS, HS + 32):
                    at = zero if r == HS else t >> 5
                    q = [jnp.where(upper, qbuf[at, pl.ds(16 * j, 16), :], 0),
                         jnp.where(upper, 0, qbuf[at, pl.ds(16 * j + 16, 16), :])]
                    up = _mm(_ld16(p1_k[slot][kb], (zero,), r // 2, 32), queries(j, q))
                    up = up + causal[2 + zero, pl.ds(r, 32), :]
                    buf[j, pl.ds(r, 32), :] = up
                    mu = jnp.max(up.reshape(4, 8, 128), axis=0)
                    m = mu if m is None else jnp.maximum(m, mu)
                tops = []
                for jj, own in ((j, lane8 >= HS), (j + 1, lane8 < HS)):
                    top = jnp.where(own, jnp.maximum(mx[jj], m), mx[jj])
                    tops.append(jnp.broadcast_to(jnp.max(top, axis=0, keepdims=True), (8, 128)))
                    p1_x[n % len(p1_x)][jj] = tops[-1]
                p1_x[n % len(p1_x)][4 + j // 2] = jnp.where(lane8 >= HS, tops[0], tops[1])
            return jnp.concatenate([sc, up], axis=0)

        def probs(a, n, s, ch, i, kb, rows):
            buf, out = p1_s[a % len(p1_s)], p1_p[a % len(p1_p)]
            nr = 32
            runs = [(j, 0, HS if kb == i else 128) for j in range(4)]
            if kb == i:
                runs += [(j, HS, 128) for j in (0, 2)]
            count, c = sum(hi - lo for _, lo, hi in runs) // nr, 0
            for j, lo, hi in runs:
                top, l = p1_x[n % len(p1_x)][(4 + j // 2 if lo else j) + zero], None
                for r in range(lo, hi, nr):
                    m = jnp.where(never, rows[c * len(rows) // count], top) if rows else top
                    c += 1
                    p = jnp.exp2(buf[j + zero, pl.ds(r, nr), :] - jnp.concatenate([m] * (nr // 8), axis=0))
                    for x in range(0, nr, 8):
                        l = p[x:x + 8] if l is None else l + p[x:x + 8]
                    if lo:
                        upper = lax.broadcasted_iota(jnp.int32, (nr, 128), 1) >= HS
                        out[j, pl.ds(r, nr), :] = jnp.where(upper, p, 0.0).astype(bf16)
                        out[j + 1, pl.ds(r, nr), :] = jnp.where(upper, 0.0, p).astype(bf16)
                    else:
                        out[j, pl.ds(r, nr), :] = p.astype(bf16)
                tot = p1_l[n % len(p1_l)]
                if lo:
                    for jj, own in ((j, lane8 >= HS), (j + 1, lane8 < HS)):
                        tot[jj][0] = jnp.broadcast_to(jnp.sum(
                            tot[jj][zero] + jnp.where(own, l, 0.0), axis=0, keepdims=True), (8, 128))
                else:
                    tot[j][0] = l + tot[j][zero] if kb > 0 else l

        def values(a, n, s, ch, i, kb):
            tot = [x[zero] for x in p1_l[n % len(p1_l)]]
            scale = (1.0 - gate[t + 4 * ch]) / jnp.where(
                row8 < 2, jnp.where(row8 == 0, tot[0], tot[1]), jnp.where(row8 == 2, tot[2], tot[3]))
            o, ticks = [None] * 4, []
            for b in range(i + 1):
                for j in range(4):
                    pv = _mm(_ld16(p1_v[2 * s + ch][b], (zero,), 16 * j, DH),
                             _ld16(p1_p[(a - i + b) % len(p1_p)], (j + zero,), 0, 128))
                    o[j] = o[j] + pv if b else pv
                ticks.append(pv)
            for j in range(4):
                y = o[j] * scale[j:j + 1]
                if s > 0:
                    y = y + p1_m[2 * ch + i // 2][i % 2 + zero, pl.ds(DH * j, DH), :]
                obuf[t + 4 * ch, pl.ds(SEG * s + 128 * i + DH * j, DH), :] = y
            return jnp.concatenate(ticks, axis=0)

        def mem_read(s, ch, half):
            z = jnp.sum(st['z', ch], axis=0, keepdims=True)
            lhs = jnp.concatenate([jnp.where((lane8 >> 5) == row8, z, 0.0),
                                   jnp.where((lane >> 5) == (row >> 5), p1_mt[ch][zero], 0.0)], axis=0)
            for b in (2 * half, 2 * half + 1):
                nd = _mm(lhs, _ld16(p1_pq[2 * s + ch - 2][b], (zero,), 0, 128))
                inv = gate[t + 4 * ch] / (nd[0:8] + 1e-6)
                for j in range(4):
                    p1_m[2 * ch + half][b % 2, pl.ds(DH * j, DH), :] = nd[8 + DH * j:8 + DH * (j + 1)] * inv[j:j + 1]
            return nd

        def mem_update(s, ch):
            slot = 2 * s + ch
            v = jnp.concatenate([_ld16(p1_v[slot][b], (zero,), 0, 128) for b in range(4)], axis=1)
            pk = jnp.concatenate([_ld16(p1_pk[slot][b], (zero,), 0, 128) for b in range(4)], axis=0)
            mt, z = _mm(v, pk), st['dz', slot]
            tick = mt
            if s > 0:
                mt, z = mt + p1_mt[ch][zero], z + st['z', ch]
            p1_mt[ch][0] = mt
            st['z', ch] = z
            return tick

        tiles = []
        for s in range(4):
            for half in ((0, 1) if s == 0 else (1, 0)):
                for i in (2 * half + 1, 2 * half):
                    for ch in range(2):
                        n = tiles[-1][0] + 1 if tiles else 0
                        tiles += [(n, s, ch, i, kb) for kb in range(i + 1)]

        def first_turn(ch, tick):
            fence(obuf, turn_tick(tick))
            p2_t[0][ch] = turned_(obuf[t + 4 * ch, pl.ds(0, SUB), :])

        def first_operands(r, tick):
            fence(p2_t[0], tick)
            o = [_swap_odd_heads(*[p2_t[0][ch + zero, pl.ds(rh * HS + r, 16), :] for rh in range(2)])
                 for ch in range(2)]
            ops = _left_operands(o[0][0], o[1][0], o[0][1], o[1][1])
            for i in range(7):
                p2_l[0][i, t, pl.ds(r, 16), :] = ops[i].astype(bf16)

        cq, ck, cv = (cols_jobs(m, t, zero) for m in (BQ, BK, BV))
        pa, (ra, rb) = plain_jobs(AO, raw_o, t), rows_jobs(t, zero)
        halves = lambda x: (x[:len(x) // 2], x[len(x) // 2:])
        side = [cq[0], pa, halves(ck[0])[0], halves(ck[0])[1] + halves(cv[0])[0],
                cq[1], ra, halves(cv[0])[1], halves(ck[1])[0],
                halves(ck[1])[1] + halves(cq[2])[0], halves(cq[2])[1], halves(cv[1])[0], halves(cv[1])[1],
                [partial(first_turn, ch) for ch in range(2)] + halves(rb)[0], ck[2],
                [partial(first_operands, r) for r in range(0, HS, 16)] + halves(rb)[1], cv[2]]
        blocks = [(AQ, 0, 0), (AK, 0, 0), (AQ, 0, 1), (AK, 0, 1)]
        for s in range(1, 4):
            blocks += [(AQ, s, 1), (AK, s, 0), (AK, s, 1), (AQ, s, 0)]
        stream = _chain(*[proj(*blk, jobs) for blk, jobs in zip(blocks, side)])
        issued = exps = done = 0
        ready, owed = [0, 0], []
        for a in range(len(tiles) + 3):
            s, pos = divmod(a, 20)
            hist = []
            if 0 < s < 4 and pos in ((2, 13) if s < 3 else (10, 14)):
                hist.append([mem_read(s, ch, int(pos < 13)) for ch in range(2)][1])
            if s < 3 and pos in (16, 18):
                hist.append(mem_update(s, (pos - 16) // 2))
            due = min(int(24 + 1.4 * a) if a < 59 else 106 + (a - 59), 112)
            hist.extend(next(stream) for _ in range(issued, due))
            issued = due
            if a < len(tiles):
                hist.append(scores(a, *tiles[a]))
            for b in range(done, ready[-2]):
                if tiles[b][3] == tiles[b][4]:
                    owed.append(b)
            done = ready[-2]
            for _ in range({77: 1, 79: 1, 80: 2, 81: 9, 82: 9}.get(a, 0) if a >= 68 else 9):
                if owed:
                    b = owed.pop(0)
                    hist.append(values(b, *tiles[b]))
            if due == 112:
                next(stream, None)
                if todo:
                    todo.pop(0)(hist[0][0:8])
            upto = min(max(a - 3, {77: 75, 78: 76, 79: 78, 80: 80}.get(a, 0)), len(tiles))
            rows = [x[r:r + 8] for x in hist[-4:] for r in range(0, x.shape[0], 8)]
            if a == 80:
                rows = rows[:16]
            for b in range(exps, upto):
                share = len(rows) // (upto - exps)
                probs(b, *tiles[b], rows[(b - exps) * share:(b + 1 - exps) * share])
            exps = max(exps, upto)
            ready.append(exps)
        assert not todo and not owed and done == len(tiles)

    def out_jobs(unit, u, zero, t0, t1):
        def turn(g, tick):
            fence(obuf, tick)
            p2_t[u][g] = obuf[g, pl.ds(pl.multiple_of(unit * SUB, SUB), SUB), :].T

        def operands(r, k, tick):
            fence(p2_t[u], tick)
            o = {g: _swap_odd_heads(*[p2_t[u][g + zero, pl.ds(rh * HS + r, 16), :] for rh in range(2)])
                 for g in (k, k + 4)}
            put_left(p2_l[u], r, lambda g: o[g][0], lambda g: o[g][1], (k,))
        tm = t0 + 6
        return (_spread([partial(turn, g) for g in range(8)], t0, tm)
                + _spread([partial(operands, r, k) for r in range(0, HS, 16) for k in range(4)], tm + 4, t1))

    def phase2(layer, c):
        zero = c >> 4
        base = [pl.multiple_of((2 * c + u) * SUB, SUB) for u in range(2)]

        def rows(u, r, n):
            return pl.ds(pl.multiple_of(base[u] + r, 16), n)

        def infini_out(u):
            for t in range(4):
                def emit(rh, ch, val):
                    g = t + 4 * ch
                    x = xbuf[rows(u, rh * HS, HS), 128 * g:128 * (g + 1)].astype(f32)
                    p2_x[u][g, pl.ds(rh * HS, HS), :] = x + val
                yield from project_steps(p2_l[u], zero, 0, HS, AO, t, emit)

        def norm(u, t0, t1):
            return norm_jobs(lambda g, r, n: p2_x[u][g + zero, pl.ds(r, n), :], partial(fence, p2_x[u]),
                             stat[u], zero, [(p2_l[2 + u], 0)], t0, t1)

        def local_proj(u, m, dst, off):
            for t in range(4):
                def emit(rh, ch, val):
                    dst[u][t + 4 * ch, pl.ds(off + rh * HS, HS), :] = val
                    if off and rh == 1 and u == 0:
                        dst[1][t + 4 * ch, pl.ds(0, HALO), :] = val[HS - HALO:]
                yield from project_steps(p2_l[2 + u], zero, 0, HS, m, t, emit)

        def attend(u, t0, t1, t2, t3):
            held = {}

            def shifted(buf, g, r, w):
                x = buf[g + zero, pl.ds(HALO + r - DIL * w - 8, 24), :]
                return (w, x[8:]), (w + WIN // 2, x[:16])

            def logits(r, w0, g, tick):
                fence(p2_q[u], tick)
                q = p2_q[u][g + zero, pl.ds(r, 16), :]
                for w, k in shifted(p2_k[u], g, r, w0) + shifted(p2_k[u], g, r, w0 + 1):
                    a = held[w] = q * k if g == 0 else held[w] + q * k
                    if g < 7:
                        continue
                    a = (a + pltpu.roll(a, 64, 1)) + (pltpu.roll(a, 32, 1) + pltpu.roll(a, 96, 1))
                    a = a * QK_SCALE
                    if u == 0 and r == 0 and w > 0:
                        pos = base[0] + lax.broadcasted_iota(jnp.int32, (16, 128), 0)
                        a = jnp.where(pos >= DIL * w, a, -1e9 * LOG2E)
                    p2_a[u][r // 16][0][w] = a

            def softmax(r, tick):
                src, dst = p2_a[u][r // 16]
                fence(src, tick)
                lg = [src[w + zero, pl.ds(r % 16, 8), :] for w in range(WIN)]
                mx = lg[0]
                for a in lg[1:]:
                    mx = jnp.maximum(mx, a)
                ex = [jnp.exp2(a - mx) for a in lg]
                den = ex[0]
                for a in ex[1:]:
                    den = den + a
                for w in range(WIN):
                    dst[w, pl.ds(r % 16, 8), :] = ex[w]
                dst[WIN, pl.ds(r % 16, 8), :] = 1.0 / den

            def mix(r, g, tick):
                fence(p2_v[u], tick)
                if g % 2 == 0:
                    fence(p2_a[u][r // 16][1], tick)
                    held['p'] = [p2_a[u][r // 16][1][w + zero] for w in range(WIN + 1)]
                acc = None
                for w0 in range(WIN // 2):
                    for w, v in shifted(p2_v[u], g, r, w0):
                        acc = held['p'][w] * v if acc is None else acc + held['p'][w] * v
                p2_p[u][r % HS // 16][g, pl.ds(r // HS * 16, 16), :] = acc * held['p'][WIN]

            def operands(r, k, tick):
                src = p2_p[u][r // 16]
                fence(src, tick)
                put_left(p2_l[4 + u], r, lambda g: src[g + zero, pl.ds(0, 16), :],
                         lambda g: src[g + zero, pl.ds(16, 16), :], (k,))

            order = [rh * HS + r for r in range(0, HS, 16) for rh in range(2)]
            lag = (t1 - t0) / 8 + 3.06
            step = (t3 - t2) / 4
            return (_spread([partial(logits, r, w, g) for r in order for w in (0, 2) for g in range(8)], t0, t1)
                    + _spread([partial(softmax, r + i) for r in order for i in (0, 8)], t0 + lag, t1 + lag)
                    + _spread([partial(mix, r, g) for r in order for g in range(8)], t2, t3)
                    + [(t2 + step * (j + 1) + (step / 4 if j < 3 else 0.3) * k + 0.2, partial(operands, 16 * j, k))
                       for j in range(4) for k in range(4)])

        def local_out(u):
            for t in range(4):
                def emit(rh, ch, val):
                    g = t + 4 * ch
                    y = p2_x[u][g + zero, pl.ds(rh * HS, HS), :] + val
                    xbuf[rows(u, rh * HS, HS), 128 * g:128 * (g + 1)] = y.astype(bf16)
                yield from project_steps(p2_l[4 + u], zero, 0, HS, BO, t, emit)

        _interleave(
            _chain(infini_out(0), infini_out(1),
                   local_proj(0, BK, p2_k, HALO), local_proj(0, BQ, p2_q, 0), local_proj(0, BV, p2_v, HALO),
                   local_proj(1, BK, p2_k, HALO), local_proj(1, BQ, p2_q, 0), local_proj(1, BV, p2_v, HALO),
                   local_out(0), local_out(1)),
            out_jobs(2 * c + 1, 1, zero, 0, 24) + out_jobs(jnp.minimum(2 * c + 2, NSUB - 1), 0, zero, 250, 279)
            + norm(0, 28, 52) + norm(1, 58, 110)
            + attend(0, 112, 150, 156, 194) + attend(1, 196, 221.0, 224, 247.0))
        for buf in (p2_k, p2_v):
            for g in range(8):
                buf[0][g, pl.ds(0, HALO), :] = buf[1][g + zero, pl.ds(SUB, HALO), :]

        @pl.when(layer == 1)
        def _():
            out_copy(c).start()

    x_copy(0).wait()
    x_copy(1).start()

    def layer_pair(layer, carry):
        def norm_rows(i, _):
            r = pl.multiple_of(i * 32, 32)
            top, bot = (_layernorm(xbuf[pl.ds(r + rh * HS, 32), :].astype(f32)) for rh in range(2))
            for buf in (xn, p0_l[0]):
                put_left(buf, r, lambda g: _tile(top, g), lambda g: _tile(bot, g))
        lax.fori_loop(0, HS // 32, norm_rows, None)

        @pl.when(layer == 0)
        def _():
            w_copy(0).wait()
            lax.fori_loop(0, 8, lambda i, _: prep_plain(AV, raw_v, i, 64), None)

        lax.fori_loop(0, 4, lambda c, _: phase0(layer, c), None)

        @pl.when(layer == 0)
        def _():
            w_copy(1).wait()
            lax.fori_loop(0, 8, lambda i, _: prep_plain(AK, raw_k, i, 64), None)
            w_copy(2).wait()
            lax.fori_loop(0, 8, lambda i, _: prep_plain(AQ, raw_q, i, 64), None)
            for i in range(3, 5):
                w_copy(i).wait()

        lax.fori_loop(0, 4, lambda t, _: phase1(layer, t), None)

        for buf in (p2_k, p2_v):
            buf[0][0:8, pl.ds(0, HALO), :] = jnp.zeros((8, HALO, 128), f32)
        lax.fori_loop(0, NSUB // 2, lambda c, _: phase2(layer, c), None)
        return carry

    lax.fori_loop(0, 2, layer_pair, None)
    for c in range(NSUB // 2):
        out_copy(c).wait()


@jax.jit
def pallas_interleave_layers__memory_aug_infini_attn__sliding_local_dilated__prompt_kernel(
    A_x: jax.Array,
    A_wq: jax.Array,
    A_wk: jax.Array,
    A_wv: jax.Array,
    A_wo: jax.Array,
    A_beta: jax.Array,
    B_x: jax.Array,
    B_wqkv: jax.Array,
    B_wo: jax.Array,
):
    del B_x
    vmem = pltpu.VMEM
    hbm = pl.BlockSpec(memory_space=pl.ANY)
    scratch = [
        vmem((S + 16, D), bf16),
        *[vmem((D + 16, D), bf16)] * 4, vmem((D + 16, 3 * D), bf16), vmem((D + 16, D), bf16),
        *[vmem((7, 4, D // 2, 128), bf16)] * 8,
        vmem((7, 4, (NSUB + 1) * HS, 128), bf16),
        vmem((9, NSUB, 128, 128), bf16),
        vmem((9, S, 128), f32),
        vmem((8, 8, 128), f32),
        vmem((3, 128, 128), f32),
        [[vmem((2, H * (DH + 1), 128), u32), vmem((9, 128, 128), u32)]] * 3,
        vmem((2, H * (DH + 1), 128), u32),
        [vmem((7, 4, HS, 128), bf16)] * 4,
        [[vmem((2, 128, 128), bf16)] * 4] * 8,
        [[vmem((2, 128, 128), bf16)] * 4] * 6,
        [[vmem((2, 128, 128), bf16)] * 4] * 8,
        [[vmem((2, 128, 128), bf16)] * 4] * 6,
        [[vmem((2, 128, 128), bf16)] * 4] * 8,
        [vmem((5, 128, 128), f32)] * 2,
        [vmem((2, 128, 128), f32)] * 4,
        [vmem((2, 128, 128), f32)] * 2,
        [vmem((6, 8, 128), f32)] * 8,
        [[vmem((2, 8, 128), f32)] * 4] * 8,
        [vmem((4, 128, 128), bf16)] * 20,
        [vmem((5, 128, 128), f32)] * 8,
        [vmem((10, SUB, 128), f32)] * 2,
        [vmem((10, SUB, 128), f32)] * 2,
        [vmem((8, 4, HS, 128), bf16)] * 6,
        [vmem((10, SUB, 128), f32)] * 2,
        [vmem((10, HALO + SUB, 128), f32)] * 2,
        [vmem((10, HALO + SUB, 128), f32)] * 2,
        [[vmem((9, 32, 128), f32)] * 4] * 2,
        [[[vmem((WIN + 2, 16, 128), f32)] * 2] * 8] * 2,
        [[vmem((2, SUB, 128), f32)] * 2] * 4,
        [vmem((2, SUB, 128), f32)] * 7,
        pltpu.SemaphoreType.DMA((5,)),
        pltpu.SemaphoreType.DMA((7,)),
        pltpu.SemaphoreType.DMA((NSUB // 2,)),
    ]
    out = pl.pallas_call(
        _kernel,
        out_shape=jax.ShapeDtypeStruct((S, D), bf16),
        in_specs=[hbm, hbm, hbm, hbm, hbm, pl.BlockSpec(memory_space=pltpu.VMEM), hbm, hbm],
        out_specs=hbm,
        scratch_shapes=scratch,
        compiler_params=pltpu.CompilerParams(vmem_limit_bytes=112 * 1024 * 1024, flags={"XLA_TPU_FORCE_LP_LLO_SCHEDULER": True}),
        name="interleaved_layers",
    )(A_x.reshape(S, D), A_wq, A_wk, A_wv, A_wo, A_beta.reshape(1, H), B_wqkv, B_wo)
    return out.reshape(1, S, D)
```

```python
import math
from functools import partial

import jax
import jax.numpy as jnp
import numpy as np
from jax import lax
from jax.experimental import pallas as pl
from jax.experimental.pallas import tpu as pltpu

S = 2048
D = 1024
H = 32
DH = 32
SEG = 512
WIN, DIL = 8, 2
HALO = 16
SUB = 128
HS = SUB // 2
NSUB = S // SUB
LOG2E = math.log2(math.e)
QK_SCALE = DH ** -0.5 * LOG2E
PV_LAG = 5

f32 = jnp.float32
bf16 = jnp.bfloat16
u32 = jnp.uint32

AQ, AK, AV, AO, BQ, BK, BV, BO = range(8)


def _mm(a, b):
    return lax.dot_general(a, b, (((1,), (0,)), ((), ())), preferred_element_type=f32)


def _ld16(ref, lead, r0, n):
    return pltpu.bitcast(ref.bitcast(u32)[(*lead, pl.ds(r0, n // 2), slice(None))], bf16)


def _left_operands(a11, a12, a21, a22):
    return (a11 + a22, a21 + a22, a11, a22, a11 + a12, a21 - a11, a12 - a22)


def _right_operands(b11, b12, b21, b22):
    return (b11 + b22, b11, b12 - b22, b21 - b11, b22, b11 + b12, b21 + b22)


def _strassen(prod, emit, park, zero):
    m1 = prod(0)
    rows = pl.ds(0, m1.shape[0])
    yield m1
    m4 = prod(3)
    park[0][0, rows, :] = m1 + m4
    yield m4
    m2 = prod(1)
    emit(1, 0, m2 + m4)
    park[1][0, rows, :] = m1 - m2
    yield m2
    m6 = prod(5)
    yield m6
    m3 = prod(2)
    emit(1, 1, park[1][zero, rows, :] + (m6 + m3))
    yield m3
    m5 = prod(4)
    emit(0, 1, m3 + m5)
    yield m5
    m7 = prod(6)
    emit(0, 0, park[0][zero, rows, :] + (m7 - m5))
    yield m7


def _strassen_lean(prod, emit, park, zero):
    m = prod(0)
    park[0][0] = m
    yield m
    m = prod(3)
    park[1][0] = park[0][zero] + m
    park[2][0] = m
    yield m
    m = prod(1)
    emit(1, 0, park[2][zero] + m)
    park[3][0] = park[0][zero] - m
    yield m
    m = prod(5)
    park[4][0] = park[3][zero] + m
    yield m
    m = prod(2)
    emit(1, 1, park[4][zero] + m)
    park[5][0] = m
    yield m
    m = prod(4)
    emit(0, 1, park[5][zero] + m)
    park[6][0] = park[1][zero] - m
    yield m
    m = prod(6)
    emit(0, 0, park[6][zero] + m)
    yield m


def _tree(op, xs):
    while len(xs) > 1:
        xs = [op(xs[i], xs[i + 1]) for i in range(0, len(xs), 2)]
    return xs[0]


def _chain(*gens):
    for g in gens:
        yield from g


def _take(gen, n):
    for _ in range(n):
        yield next(gen)


def fence(buf, tick, slot=0):
    if tick is not None:
        buf[buf.shape[0] - 1 - slot, pl.ds(0, 8), :] = tick[tick.shape[0] - 8:]


def _paced(mxu, jobs):
    jobs = sorted(jobs, key=lambda j: j[0])
    n = 0
    for i, prod in enumerate(mxu):
        while n < len(jobs) and jobs[n][0] < i + 1:
            r = 8 * int(max(jobs[n][0] - i, 0) * (prod.shape[0] // 8))
            jobs[n][1](prod[r:r + 8])
            n += 1
        yield prod
    assert n == len(jobs)


def _interleave(mxu, jobs):
    for _ in _paced(mxu, jobs):
        pass


def _spread(fns, first, last):
    return [(first + (last - first) * i / len(fns), fn) for i, fn in enumerate(fns)]


def _layernorm(x):
    d = x - jnp.sum(x, axis=-1, keepdims=True) * (1.0 / D)
    v = jnp.sum(d * d, axis=-1, keepdims=True) * (1.0 / D)
    return d * lax.rsqrt(v + 1e-5)


def _pair(lo, hi):
    return (pltpu.bitcast(lo.astype(f32), u32) >> 16) | pltpu.bitcast(hi.astype(f32), u32)


def _unpair(w, i):
    return pltpu.bitcast(w & np.uint32(0xFFFF0000) if i else w << 16, f32)


def _swap_odd_heads(lo, hi):
    odd = (lax.broadcasted_iota(jnp.int32, lo.shape, 1) & DH) != 0
    return jnp.where(odd, hi, lo), jnp.where(odd, lo, hi)


def _phi(t):
    return jnp.where(t > 0, t + 1.0, jnp.exp(t))


def _tile(x, c):
    return x[:, 128 * c:128 * (c + 1)]


def _kernel(x_hbm, wq_hbm, wk_hbm, wv_hbm, wo_hbm, beta_hbm, bqkv_hbm, bo_hbm, out_hbm,
            xbuf, raw_q, raw_k, raw_v, raw_o, raw_bqkv, raw_bo,
            w_aq, w_ak, w_av, w_ao, w_bq, w_bk, w_bv, w_bo,
            xn, vbuf, obuf, gate, causal, perm_c, perm_r,
            p0_l, p1_q, p1_pq, p1_k, p1_pk, p1_v, p1_f, p1_m, p1_mt, p1_x, p1_l, p1_p, p1_s,
            p2_t, p2_x, p2_l, p2_q, p2_k, p2_v, p2_p, p2_a, stat, park, beta_ref,
            x_sem, w_sem, o_sem):
    wts = (w_aq, w_ak, w_av, w_ao, w_bq, w_bk, w_bv, w_bo)
    lane = lax.broadcasted_iota(jnp.int32, (128, 128), 1)
    row = lax.broadcasted_iota(jnp.int32, (128, 128), 0)
    lane8 = lax.broadcasted_iota(jnp.int32, (8, 128), 1)
    row8 = lax.broadcasted_iota(jnp.int32, (8, 128), 0)

    x_edges = (0, SUB, SUB + SEG, SUB + 2 * SEG, SUB + 3 * SEG, S)

    def x_copy(i):
        rows = pl.ds(x_edges[i], x_edges[i + 1] - x_edges[i])
        return pltpu.make_async_copy(x_hbm.at[rows], xbuf.at[rows], x_sem.at[i])

    w_pairs = ((wv_hbm, raw_v), (wk_hbm, raw_k), (wq_hbm, raw_q), (wo_hbm, raw_o), (bo_hbm, raw_bo))

    def w_copy(i):
        return pltpu.make_async_copy(w_pairs[i][0], w_pairs[i][1].at[pl.ds(0, D)], w_sem.at[i])

    def bqkv_copies(i):
        rows = [pl.ds(128 * i + rh * (D // 2), 128 + 256 * i) for rh in range(2)]
        return [pltpu.make_async_copy(bqkv_hbm.at[r], raw_bqkv.at[r], w_sem.at[5 + 2 * i + rh])
                for rh, r in enumerate(rows)]

    def out_copy(c):
        rows = pl.ds(pl.multiple_of(c * SUB, SUB), SUB)
        return pltpu.make_async_copy(xbuf.at[rows], out_hbm.at[rows], o_sem.at[c])

    beta_copy = pltpu.make_async_copy(beta_hbm, beta_ref, w_sem.at[9])
    x_copy(0).start()
    beta_copy.start()
    w_copy(0).start()
    x_copy(0).wait()
    x_copy(1).start()
    beta_copy.wait()

    hr = lax.broadcasted_iota(jnp.int32, (8, H), 0)
    hc = lax.broadcasted_iota(jnp.int32, (8, H), 1)
    sig = 1.0 / (1.0 + jnp.exp(-beta_ref[...].astype(f32)))
    for g in range(8):
        gate[g] = jnp.broadcast_to(
            jnp.sum(jnp.where(hr + 4 * g == hc, sig, 0.0), axis=1, keepdims=True), (8, 128))
    for i, query in enumerate((lane, lane ^ 64, lane | 64)):
        causal[i] = jnp.where(row <= query, 0.0, -1e9 * LOG2E)

    def put_weight(m, r0, top, bot):
        n = top.shape[0]
        for t in range(4):
            ops = _right_operands(_tile(top, t), _tile(top, t + 4), _tile(bot, t), _tile(bot, t + 4))
            for i in range(7):
                wts[m][i, t, pl.ds(r0, n), :] = ops[i].astype(bf16)

    def raw_rows(raw, r0, n, c0=0):
        return raw[pl.ds(r0, n), c0:c0 + D].astype(f32)

    def prep_plain(m, raw, it, n):
        r0 = pl.multiple_of(it * n, n)
        put_weight(m, r0, raw_rows(raw, r0, n), raw_rows(raw, pl.multiple_of(r0 + D // 2, n), n))

    def fence16(buf, tick):
        if tick is not None:
            buf[pl.ds(buf.shape[0] - 16, 16), 0:128] = jnp.concatenate([tick, tick], axis=0).astype(bf16)

    turns = []

    def turn_tick(tick):
        if len(turns) < 3:
            return tick
        return pltpu.bitcast(pltpu.bitcast(tick, u32) | turns[-3], f32)

    def turned_(x):
        y = x.T
        turns.append(pltpu.bitcast(y[:16 if y.dtype == bf16 else 8], u32))
        return y

    def put_right(dst, t, r, quads):
        for i, op in enumerate(_right_operands(*quads)):
            dst[i, t, pl.ds(r, 16), :] = op.astype(bf16)

    def band(ref, it, rh=0):
        rows = pl.ds(pl.multiple_of(it * 128 + rh * (D // 2), 128), 128)
        return ref.at[(slice(None),) * (len(ref.shape) - 2) + (rows,)]

    def plain_jobs(m, raw, it):
        def job(r, t, tick):
            fence16(raw, tick)
            put_right(band(wts[m], it), t, r,
                      [band(raw, it, rh)[pl.ds(r, 16), pl.ds(128 * (t + 4 * ch), 128)].astype(f32)
                       for rh in range(2) for ch in range(2)])
        return [partial(job, r, t) for r in range(0, 128, 16) for t in range(4)]

    def regroup(buf, slot, c):
        return jnp.concatenate(
            [buf[slot, pl.ds(d, H, stride=DH + 1), :] for d in range(4 * c, 4 * c + 4)], axis=0)

    def cols_jobs(m, it, zero):
        turned, back = perm_c[m - BQ]

        def turn(c, tick):
            fence16(raw_bqkv, turn_tick(tick))
            c0 = (m - BQ) * D + 128 * c
            w = turned_(_pair(
                *[raw_bqkv[pl.ds(pl.multiple_of(it * 128 + rh * (D // 2), 128), 128), c0:c0 + 128]
                  for rh in range(2)]))
            for j in range(4):
                turned[0, pl.ds((4 * c + j) * (DH + 1), DH), :] = w[j * DH:(j + 1) * DH]

        def unturn(c, tick):
            fence(turned, pltpu.bitcast(turn_tick(tick), u32))
            back[c] = turned_(regroup(turned, zero, c))

        def job(r, t, tick):
            fence(back, pltpu.bitcast(tick, u32))
            w = [back[t + 4 * ch + zero, pl.ds(r, 16), :] for ch in range(2)]
            put_right(band(wts[m], it), t, r,
                      [_unpair(w[ch], rh) for rh in range(2) for ch in range(2)])
        return ([partial(turn, c) for c in range(8)], [partial(unturn, c) for c in range(8)],
                [partial(job, r, t) for r in range(0, 128, 16) for t in range(4)])

    def rows_jobs(it, zero):
        def spread_heads(h, tick):
            fence16(raw_bo, tick)
            perm_r[0, pl.ds(h * (DH + 1), DH), :] = _pair(
                *[raw_bo[pl.ds(h * DH, DH), pl.ds(pl.multiple_of(it * 128 + ch * (D // 2), 128), 128)]
                  for ch in range(2)])

        def job(d, h0, tick):
            fence(perm_r, pltpu.bitcast(tick, u32))
            w = [perm_r[zero, pl.ds(h0 * (DH + 1) + d + rh * (DH // 2), 16, stride=DH + 1), :]
                 for rh in range(2)]
            put_right(w_bo, it, d * H + h0,
                      [_unpair(w[rh], ch) for rh in range(2) for ch in range(2)])
        return [partial(spread_heads, h) for h in range(H)], [partial(job, d, h0) for d in range(DH // 2) for h0 in (0, 16)]

    def put_left(buf, r0, top, bot, ks=range(4)):
        for k in ks:
            ops = _left_operands(top(k), top(k + 4), bot(k), bot(k + 4))
            for i in range(7):
                buf[i, k, pl.ds(r0, ops[i].shape[0]), :] = ops[i].astype(bf16)
        return ops[6]

    def project(*args):
        for _ in project_steps(*args):
            pass

    def project_steps(buf, zero, r0, n, m, t, emit):
        def prod(i):
            lhs = jnp.concatenate([_ld16(buf, (i + zero, k), r0, n) for k in range(4)], axis=1)
            return _mm(lhs, _ld16(wts[m], (i, t), 0, D // 2))
        return (_strassen_lean if n == SUB and 1 else _strassen)(prod, emit, park, zero)

    def norm_jobs(src, hold, st, zero, dsts, t0, t1):
        def row_mean(parts):
            tot = parts[0]
            for x in parts[1:]:
                tot = tot + x
            return jnp.sum(tot, axis=-1, keepdims=True) * (1.0 / D)

        def mean_job(r, tick):
            hold(tick)
            st[0][0, pl.ds(r, 16), :] = jnp.broadcast_to(
                row_mean([src(g, r, 16) for g in range(8)]), (16, 128))

        def var_job(r, tick):
            fence(st[0], tick)
            mean = st[0][zero, pl.ds(r, 8), :]
            dev = [src(g, r, 8) - mean for g in range(8)]
            st[1][0, pl.ds(r, 8), :] = jnp.broadcast_to(
                lax.rsqrt(row_mean([d * d for d in dev]) + 1e-5), (8, 128))

        def out_job(r, k, which, tick):
            hold(tick)
            fence(st[0], tick)
            fence(st[1], tick)
            mean = [st[0][zero, pl.ds(rh * HS + r, 16), :] for rh in range(2)]
            rstd = [st[1][zero, pl.ds(rh * HS + r, 16), :] for rh in range(2)]
            ops = _left_operands(*[(src(k + 4 * ch, rh * HS + r, 16) - mean[rh]) * rstd[rh]
                                   for rh in range(2) for ch in range(2)])
            for i in which:
                for buf in dsts:
                    buf[i, k, pl.ds(r, 16), :] = ops[i].astype(bf16)

        work = t1 - t0 - 4
        return (_spread([partial(mean_job, r) for r in range(0, SUB, 16)], t0, t0 + 0.15 * work)
                + _spread([partial(var_job, r) for r in range(0, SUB, 8)],
                          t0 + 2 + 0.15 * work, t0 + 2 + 0.45 * work)
                + _spread([partial(out_job, r, k, which) for r in range(0, HS, 16) for k in range(4)
                           for which in (((2, 4, 6), (0, 1, 3, 5)) if 1 else (range(7),))],
                          t0 + 4 + 0.45 * work, t1))

    def norm_unit(src_unit, dst_unit, slot, zero, t0, t1):
        x = xbuf.at[pl.ds(pl.multiple_of(src_unit * SUB, SUB), SUB)]
        return norm_jobs(lambda g, r, n: x[pl.ds(r, n), pl.ds(128 * g, 128)].astype(f32),
                         partial(fence16, xbuf), stat[slot], zero,
                         [xn.at[:, :, pl.ds(pl.multiple_of(dst_unit * HS, HS), HS)], p0_l[slot]], t0, t1)

    def phase0(layer, c):
        zero = c >> 4
        for i in range(4):
            @pl.when(jnp.logical_and(layer == 0, c == i))
            def _():
                x_copy(i + 1).wait()
                for j in ((2, 3, 4), (), (), ())[i]:
                    x_copy(j).start()
                for j in ((), (1, 2), (3, 4), ())[i]:
                    w_copy(j).start()
                if i == 2:
                    for cp in bqkv_copies(0):
                        cp.start()

        def values(u):
            for t in range(4):
                def emit(rh, ch, val):
                    vbuf[t + 4 * ch, c * 4 + u, pl.ds(rh * HS, HS), :] = val.astype(bf16)
                yield from project_steps(p0_l[u], zero, 0, HS, AV, t, emit)

        jobs = []
        for u in range(4):
            nxt = c * 4 + u + 1
            jobs += norm_unit(nxt if u < 3 else jnp.minimum(nxt, NSUB - 1), nxt, (u + 1) % 4, zero,
                              *((0, 24), (24, 52), (52, 80), (80, 110))[u])
        _interleave(_chain(*[values(u) for u in range(4)]), jobs)

    def phase1(layer, t):
        zero = t >> 4

        @pl.when(jnp.logical_and(layer == 0, t == 1))
        def _():
            for cp in bqkv_copies(1):
                cp.wait()

        st = {}
        never = row8 < zero
        turns.clear()
        todo = []

        def turn_q(s, ch, blk, tick):
            fence(p1_f[blk // 2], turn_tick(tick))
            y = p1_f[blk // 2][2 * ch + blk % 2 + zero]
            y = turned_(jnp.concatenate(_swap_odd_heads(y[:HS], y[HS:]), axis=0))
            p1_q[2 * s + ch][blk][0] = (y * QK_SCALE).astype(bf16)
            if s > 0:
                p1_pq[2 * s + ch - 2][blk][0] = _phi(y).astype(bf16)

        def turn_v(s, blk, tick):
            tick = turn_tick(tick)
            vbuf[8, 0, pl.ds(0, 16), :] = jnp.concatenate([tick, tick], axis=0).astype(bf16)
            y = turned_(jnp.concatenate([vbuf[t + 4 * ch, 4 * s + blk] for ch in range(2)], axis=1))
            for ch in range(2):
                p1_v[2 * s + ch][blk][0] = y[128 * ch:128 * (ch + 1)]

        def proj(m, s, half, extra):
            def emit(rh, ch, val):
                slot = 2 * s + ch
                for u in range(2):
                    blk = 2 * half + u
                    y = val[HS * u:HS * (u + 1)]
                    rows = pl.ds(rh * HS, HS)
                    if m == AQ:
                        p1_f[half][2 * ch + u, rows, :] = y
                        continue
                    p1_k[slot][blk][0, rows, :] = y.astype(bf16)
                    if s < 3:
                        pk = _phi(y)
                        p1_pk[slot][blk][0, rows, :] = pk.astype(bf16)
                        z = jnp.sum(pk.reshape(HS // 8, 8, 128), axis=0)
                        st['dz', slot] = z + st['dz', slot] if ('dz', slot) in st else z
            jobs = (_spread(todo + [partial(turn_v, s, 2 * half + (m == AK))], 0, 4)
                    + _spread(extra, 0, 7))
            todo.clear()
            yield from _paced(
                project_steps(xn, zero, (s * 4 + half * 2) * (HS // 2), 2 * HS, m, t, emit), jobs)
            if m == AQ:
                todo.extend(partial(turn_q, s, ch, 2 * half + u) for ch in range(2) for u in (1, 0))

        def scores(a, n, s, ch, i, kb):
            slot = 2 * s + ch
            buf = p1_s[a % len(p1_s)]
            qbuf = p1_q[slot][i].bitcast(u32)

            def queries(first, parts):
                pad = (first, 4 - first - len(parts))
                parts = ([jnp.zeros((16 * pad[0], 128), u32)] * (pad[0] > 0) + parts
                         + [jnp.zeros((16 * pad[1], 128), u32)] * (pad[1] > 0))
                return pltpu.bitcast(jnp.concatenate(parts, axis=0), bf16)

            nk = HS if kb == i else 128
            k = _ld16(p1_k[slot][kb], (zero,), 0, nk)
            mx = []
            for j in range(4):
                sc = _mm(k, queries(j, [qbuf[zero, pl.ds(16 * j, 16), :]]))
                if kb == i:
                    sc = sc + causal[j % 2 + zero, pl.ds(0, HS), :]
                buf[j, pl.ds(0, nk), :] = sc
                m = jnp.max(sc.reshape(nk // 8, 8, 128), axis=0)
                mx.append(jnp.maximum(m, st['m', n, j]) if kb > 0 else m)
                st['m', n, j] = mx[j]
            if kb < i:
                return sc
            upper = lax.broadcasted_iota(jnp.int32, (16, 128), 1) >= HS
            for j in (0, 2):
                m = None
                for r in (HS, HS + 32):
                    at = zero if r == HS else t >> 5
                    q = [jnp.where(upper, qbuf[at, pl.ds(16 * j, 16), :], 0),
                         jnp.where(upper, 0, qbuf[at, pl.ds(16 * j + 16, 16), :])]
                    up = _mm(_ld16(p1_k[slot][kb], (zero,), r // 2, 32), queries(j, q))
                    up = up + causal[2 + zero, pl.ds(r, 32), :]
                    buf[j, pl.ds(r, 32), :] = up
                    mu = jnp.max(up.reshape(4, 8, 128), axis=0)
                    m = mu if m is None else jnp.maximum(m, mu)
                tops = []
                for jj, own in ((j, lane8 >= HS), (j + 1, lane8 < HS)):
                    top = jnp.where(own, jnp.maximum(mx[jj], m), mx[jj])
                    tops.append(jnp.broadcast_to(jnp.max(top, axis=0, keepdims=True), (8, 128)))
                    p1_x[n % len(p1_x)][jj] = tops[-1]
                p1_x[n % len(p1_x)][4 + j // 2] = jnp.where(lane8 >= HS, tops[0], tops[1])
            return jnp.concatenate([sc, up], axis=0)

        def probs(a, n, s, ch, i, kb, rows):
            buf, out = p1_s[a % len(p1_s)], p1_p[a % len(p1_p)]
            nr = 32
            runs = [(j, 0, HS if kb == i else 128) for j in range(4)]
            if kb == i:
                runs += [(j, HS, 128) for j in (0, 2)]
            count, c = sum(hi - lo for _, lo, hi in runs) // nr, 0
            for j, lo, hi in runs:
                top, l = p1_x[n % len(p1_x)][(4 + j // 2 if lo else j) + zero], None
                for r in range(lo, hi, nr):
                    m = jnp.where(never, rows[c * len(rows) // count], top) if rows else top
                    c += 1
                    p = jnp.exp2(buf[j + zero, pl.ds(r, nr), :] - jnp.concatenate([m] * (nr // 8), axis=0))
                    for x in range(0, nr, 8):
                        l = p[x:x + 8] if l is None else l + p[x:x + 8]
                    if lo:
                        upper = lax.broadcasted_iota(jnp.int32, (nr, 128), 1) >= HS
                        out[j, pl.ds(r, nr), :] = jnp.where(upper, p, 0.0).astype(bf16)
                        out[j + 1, pl.ds(r, nr), :] = jnp.where(upper, 0.0, p).astype(bf16)
                    else:
                        out[j, pl.ds(r, nr), :] = p.astype(bf16)
                tot = p1_l[n % len(p1_l)]
                if lo:
                    for jj, own in ((j, lane8 >= HS), (j + 1, lane8 < HS)):
                        tot[jj][0] = jnp.broadcast_to(jnp.sum(
                            tot[jj][zero] + jnp.where(own, l, 0.0), axis=0, keepdims=True), (8, 128))
                else:
                    tot[j][0] = l + tot[j][zero] if kb > 0 else l

        def values(a, n, s, ch, i, kb):
            tot = [x[zero] for x in p1_l[n % len(p1_l)]]
            scale = (1.0 - gate[t + 4 * ch]) / jnp.where(
                row8 < 2, jnp.where(row8 == 0, tot[0], tot[1]), jnp.where(row8 == 2, tot[2], tot[3]))
            o, ticks = [None] * 4, []
            for b in range(i + 1):
                for j in range(4):
                    pv = _mm(_ld16(p1_v[2 * s + ch][b], (zero,), 16 * j, DH),
                             _ld16(p1_p[(a - i + b) % len(p1_p)], (j + zero,), 0, 128))
                    o[j] = o[j] + pv if b else pv
                ticks.append(pv)
            for j in range(4):
                y = o[j] * scale[j:j + 1]
                if s > 0:
                    y = y + p1_m[2 * ch + i // 2][i % 2 + zero, pl.ds(DH * j, DH), :]
                obuf[t + 4 * ch, pl.ds(SEG * s + 128 * i + DH * j, DH), :] = y
            return jnp.concatenate(ticks, axis=0)

        def mem_read(s, ch, half):
            z = jnp.sum(st['z', ch], axis=0, keepdims=True)
            lhs = jnp.concatenate([jnp.where((lane8 >> 5) == row8, z, 0.0),
                                   *[jnp.where((lane[:DH] >> 5) == j, p1_mt[ch][zero, pl.ds(DH * j, DH), :], 0.0)
                                     for j in range(4)]], axis=0)
            for b in (2 * half, 2 * half + 1):
                nd = _mm(lhs, _ld16(p1_pq[2 * s + ch - 2][b], (zero,), 0, 128))
                inv = gate[t + 4 * ch] / (nd[0:8] + 1e-6)
                for j in range(4):
                    p1_m[2 * ch + half][b % 2, pl.ds(DH * j, DH), :] = nd[8 + DH * j:8 + DH * (j + 1)] * inv[j:j + 1]
            return nd

        def mem_update(s, ch):
            slot = 2 * s + ch
            v = jnp.concatenate([_ld16(p1_v[slot][b], (zero,), 0, 128) for b in range(4)], axis=1)
            pk = jnp.concatenate([_ld16(p1_pk[slot][b], (zero,), 0, 128) for b in range(4)], axis=0)
            mt, z = _mm(v, pk), st['dz', slot]
            tick = mt
            if s > 0:
                mt, z = mt + p1_mt[ch][zero], z + st['z', ch]
            p1_mt[ch][0] = mt
            st['z', ch] = z
            return tick

        tiles = []
        for s in range(4):
            for half in ((0, 1) if s == 0 else (1, 0)):
                for i in (2 * half + 1, 2 * half):
                    for ch in range(2):
                        n = tiles[-1][0] + 1 if tiles else 0
                        tiles += [(n, s, ch, i, kb) for kb in range(i + 1)]

        def first_turn(ch, tick):
            fence(obuf, turn_tick(tick))
            p2_t[0][ch] = turned_(obuf[t + 4 * ch, pl.ds(0, SUB), :])

        def first_operands(r, tick):
            fence(p2_t[0], tick)
            o = [_swap_odd_heads(*[p2_t[0][ch + zero, pl.ds(rh * HS + r, 16), :] for rh in range(2)])
                 for ch in range(2)]
            ops = _left_operands(o[0][0], o[1][0], o[0][1], o[1][1])
            for i in range(7):
                p2_l[0][i, t, pl.ds(r, 16), :] = ops[i].astype(bf16)

        cq, ck, cv = (cols_jobs(m, t, zero) for m in (BQ, BK, BV))
        pa, (ra, rb) = plain_jobs(AO, raw_o, t), rows_jobs(t, zero)
        halves = lambda x: (x[:len(x) // 2], x[len(x) // 2:])
        side = [cq[0], pa, halves(ck[0])[0], halves(ck[0])[1] + halves(cv[0])[0],
                cq[1], ra, halves(cv[0])[1], halves(ck[1])[0],
                halves(ck[1])[1] + halves(cq[2])[0], halves(cq[2])[1], halves(cv[1])[0], halves(cv[1])[1],
                [partial(first_turn, ch) for ch in range(2)] + halves(rb)[0], ck[2],
                [partial(first_operands, r) for r in range(0, HS, 16)] + halves(rb)[1], cv[2]]
        blocks = [(AQ, 0, 0), (AK, 0, 0), (AQ, 0, 1), (AK, 0, 1)]
        for s in range(1, 4):
            blocks += [(AQ, s, 1), (AK, s, 0), (AK, s, 1), (AQ, s, 0)]
        stream = _chain(*[proj(*blk, jobs) for blk, jobs in zip(blocks, side)])
        issued = exps = done = 0
        ready, owed = [0, 0], []
        for a in range(len(tiles) + 3):
            s, pos = divmod(a, 20)
            hist = []
            if 0 < s < 4 and pos in ((2, 13) if s < 3 else (10, 14)):
                hist.append([mem_read(s, ch, int(pos < 13)) for ch in range(2)][1])
            if s < 3 and pos in (16, 18):
                hist.append(mem_update(s, (pos - 16) // 2))
            due = min(int(24 + 1.4 * a) if a < 59 else 106 + (a - 59), 112)
            hist.extend(next(stream) for _ in range(issued, due))
            issued = due
            if a < len(tiles):
                hist.append(scores(a, *tiles[a]))
            for b in range(done, ready[-2]):
                if tiles[b][3] == tiles[b][4]:
                    owed.append(b)
            done = ready[-2]
            for _ in range({77: 1, 79: 1, 80: 2, 81: 9, 82: 9}.get(a, 0) if a >= 68 else 9):
                if owed:
                    b = owed.pop(0)
                    hist.append(values(b, *tiles[b]))
            if due == 112:
                next(stream, None)
                if todo:
                    todo.pop(0)(hist[0][0:8])
            upto = min(max(a - 3, {77: 75, 78: 76, 79: 78, 80: 80}.get(a, 0)), len(tiles))
            rows = [x[r:r + 8] for x in hist[-4:] for r in range(0, x.shape[0], 8)]
            if a == 80:
                rows = rows[:16]
            for b in range(exps, upto):
                share = len(rows) // (upto - exps)
                probs(b, *tiles[b], rows[(b - exps) * share:(b + 1 - exps) * share])
            exps = max(exps, upto)
            ready.append(exps)
        assert not todo and not owed and done == len(tiles)

    def out_jobs(unit, u, zero, t0, t1):
        def turn(g, tick):
            fence(obuf, tick)
            p2_t[u][g] = obuf[g, pl.ds(pl.multiple_of(unit * SUB, SUB), SUB), :].T

        def operands(r, k, tick):
            fence(p2_t[u], tick)
            o = {g: _swap_odd_heads(*[p2_t[u][g + zero, pl.ds(rh * HS + r, 16), :] for rh in range(2)])
                 for g in (k, k + 4)}
            put_left(p2_l[u], r, lambda g: o[g][0], lambda g: o[g][1], (k,))
        tm = t0 + 6
        return (_spread([partial(turn, g) for g in range(8)], t0, tm)
                + _spread([partial(operands, r, k) for r in range(0, HS, 16) for k in range(4)], tm + 4, t1))

    def phase2(layer, c):
        zero = c >> 4
        base = [pl.multiple_of((2 * c + u) * SUB, SUB) for u in range(2)]

        def rows(u, r, n):
            return pl.ds(pl.multiple_of(base[u] + r, 16), n)

        def infini_out(u):
            for t in range(4):
                def emit(rh, ch, val):
                    g = t + 4 * ch
                    x = xbuf[rows(u, rh * HS, HS), 128 * g:128 * (g + 1)].astype(f32)
                    p2_x[u][g, pl.ds(rh * HS, HS), :] = x + val
                yield from project_steps(p2_l[u], zero, 0, HS, AO, t, emit)

        def norm(u, t0, t1):
            return norm_jobs(lambda g, r, n: p2_x[u][g + zero, pl.ds(r, n), :], partial(fence, p2_x[u]),
                             stat[u], zero, [p2_l[2 + u]], t0, t1)

        def local_proj(u, m, dst, off):
            for t in range(4):
                def emit(rh, ch, val):
                    dst[u][t + 4 * ch, pl.ds(off + rh * HS, HS), :] = val
                    if off and rh == 1 and u == 0:
                        dst[1][t + 4 * ch, pl.ds(0, HALO), :] = val[HS - HALO:]
                yield from project_steps(p2_l[2 + u], zero, 0, HS, m, t, emit)

        def attend(u, t0, t1, t2, t3):
            held = {}

            def shifted(buf, g, r, w):
                x = buf[g + zero, pl.ds(HALO + r - DIL * w - 8, 24), :]
                return (w, x[8:]), (w + WIN // 2, x[:16])

            def logits(r, w0, g, tick):
                fence(p2_q[u], tick)
                q = p2_q[u][g + zero, pl.ds(r, 16), :]
                for w, k in shifted(p2_k[u], g, r, w0) + shifted(p2_k[u], g, r, w0 + 1):
                    a = held[w] = q * k if g == 0 else held[w] + q * k
                    if g < 7:
                        continue
                    a = (a + pltpu.roll(a, 64, 1)) + (pltpu.roll(a, 32, 1) + pltpu.roll(a, 96, 1))
                    a = a * QK_SCALE
                    if u == 0 and r == 0 and w > 0:
                        pos = base[0] + lax.broadcasted_iota(jnp.int32, (16, 128), 0)
                        a = jnp.where(pos >= DIL * w, a, -1e9 * LOG2E)
                    p2_a[u][r // 16][0][w] = a

            def softmax(r, tick):
                src, dst = p2_a[u][r // 16]
                fence(src, tick)
                lg = [src[w + zero, pl.ds(r % 16, 8), :] for w in range(WIN)]
                mx = lg[0]
                for a in lg[1:]:
                    mx = jnp.maximum(mx, a)
                ex = [jnp.exp2(a - mx) for a in lg]
                den = ex[0]
                for a in ex[1:]:
                    den = den + a
                for w in range(WIN):
                    dst[w, pl.ds(r % 16, 8), :] = ex[w]
                dst[WIN, pl.ds(r % 16, 8), :] = 1.0 / den

            def mix(r, g, tick):
                fence(p2_v[u], tick)
                if g % 2 == 0:
                    fence(p2_a[u][r // 16][1], tick)
                    held['p'] = [p2_a[u][r // 16][1][w + zero] for w in range(WIN + 1)]
                acc = None
                for w0 in range(WIN // 2):
                    for w, v in shifted(p2_v[u], g, r, w0):
                        acc = held['p'][w] * v if acc is None else acc + held['p'][w] * v
                p2_p[u][r % HS // 16][g, pl.ds(r // HS * 16, 16), :] = acc * held['p'][WIN]

            def operands(r, k, tick):
                src = p2_p[u][r // 16]
                fence(src, tick)
                put_left(p2_l[4 + u], r, lambda g: src[g + zero, pl.ds(0, 16), :],
                         lambda g: src[g + zero, pl.ds(16, 16), :], (k,))

            order = [rh * HS + r for r in range(0, HS, 16) for rh in range(2)]
            lag = (t1 - t0) / 8 + 3.06
            step = (t3 - t2) / 4
            return (_spread([partial(logits, r, w, g) for r in order for w in (0, 2) for g in range(8)], t0, t1)
                    + _spread([partial(softmax, r + i) for r in order for i in (0, 8)], t0 + lag, t1 + lag)
                    + _spread([partial(mix, r, g) for r in order for g in range(8)], t2, t3)
                    + [(t2 + step * (j + 1) + (step / 4 if j < 3 else 0.3) * k + 0.2, partial(operands, 16 * j, k))
                       for j in range(4) for k in range(4)])

        def send(u, tick):
            @pl.when(layer == 1)
            def _():
                out_copy(2 * c + u).start()

        def local_out(u):
            for t in range(4):
                def emit(rh, ch, val):
                    g = t + 4 * ch
                    y = p2_x[u][g + zero, pl.ds(rh * HS, HS), :] + val
                    xbuf[rows(u, rh * HS, HS), 128 * g:128 * (g + 1)] = y.astype(bf16)
                yield from project_steps(p2_l[4 + u], zero, 0, HS, BO, t, emit)

        _interleave(
            _chain(infini_out(0), infini_out(1),
                   local_proj(0, BK, p2_k, HALO), local_proj(0, BQ, p2_q, 0), local_proj(0, BV, p2_v, HALO),
                   local_proj(1, BK, p2_k, HALO), local_proj(1, BQ, p2_q, 0), local_proj(1, BV, p2_v, HALO),
                   local_out(0), local_out(1)),
            out_jobs(2 * c + 1, 1, zero, 0, 24) + out_jobs(jnp.minimum(2 * c + 2, NSUB - 1), 0, zero, 250, 279)
            + norm(0, 28, 52) + norm(1, 58, 110) + [(252, partial(send, 0))]
            + attend(0, 112, 150, 156, 194) + attend(1, 196, 221.0, 224, 247.0))
        for buf in (p2_k, p2_v):
            for g in range(8):
                buf[0][g, pl.ds(0, HALO), :] = buf[1][g + zero, pl.ds(SUB, HALO), :]

        send(1, None)

    def layer_pair(layer, carry):
        def norm_rows(i, _):
            r = pl.multiple_of(i * 32, 32)
            top, bot = (_layernorm(xbuf[pl.ds(r + rh * HS, 32), :].astype(f32)) for rh in range(2))
            for buf in (xn, p0_l[0]):
                put_left(buf, r, lambda g: _tile(top, g), lambda g: _tile(bot, g))
        lax.fori_loop(0, HS // 32, norm_rows, None)

        @pl.when(layer == 0)
        def _():
            w_copy(0).wait()
            lax.fori_loop(0, 8, lambda i, _: prep_plain(AV, raw_v, i, 64), None)

        lax.fori_loop(0, 4, lambda c, _: phase0(layer, c), None)

        @pl.when(layer == 0)
        def _():
            w_copy(1).wait()
            lax.fori_loop(0, 8, lambda i, _: prep_plain(AK, raw_k, i, 64), None)
            w_copy(2).wait()
            lax.fori_loop(0, 8, lambda i, _: prep_plain(AQ, raw_q, i, 64), None)
            for cp in [w_copy(3), w_copy(4)] + bqkv_copies(0):
                cp.wait()
            for cp in bqkv_copies(1):
                cp.start()

        lax.fori_loop(0, 4, lambda t, _: phase1(layer, t), None)

        for buf in (p2_k, p2_v):
            buf[0][0:8, pl.ds(0, HALO), :] = jnp.zeros((8, HALO, 128), f32)
        lax.fori_loop(0, NSUB // 2, lambda c, _: phase2(layer, c), None)
        return carry

    lax.fori_loop(0, 2, layer_pair, None)
    for c in range(NSUB):
        out_copy(c).wait()


@jax.jit
def pallas_interleave_layers__memory_aug_infini_attn__sliding_local_dilated__prompt_kernel(
    A_x: jax.Array,
    A_wq: jax.Array,
    A_wk: jax.Array,
    A_wv: jax.Array,
    A_wo: jax.Array,
    A_beta: jax.Array,
    B_x: jax.Array,
    B_wqkv: jax.Array,
    B_wo: jax.Array,
):
    del B_x
    vmem = pltpu.VMEM
    hbm = pl.BlockSpec(memory_space=pl.ANY)
    scratch = [
        vmem((S + 16, D), bf16),
        *[vmem((D + 16, D), bf16)] * 4, vmem((D + 16, 3 * D), bf16), vmem((D + 16, D), bf16),
        *[vmem((7, 4, D // 2, 128), bf16)] * 8,
        vmem((7, 4, (NSUB + 1) * HS, 128), bf16),
        vmem((9, NSUB, 128, 128), bf16),
        vmem((9, S, 128), f32),
        vmem((8, 8, 128), f32),
        vmem((3, 128, 128), f32),
        [[vmem((2, H * (DH + 1), 128), u32), vmem((9, 128, 128), u32)]] * 3,
        vmem((2, H * (DH + 1), 128), u32),
        [vmem((7, 4, HS, 128), bf16)] * 4,
        [[vmem((2, 128, 128), bf16)] * 4] * 8,
        [[vmem((2, 128, 128), bf16)] * 4] * 6,
        [[vmem((2, 128, 128), bf16)] * 4] * 8,
        [[vmem((2, 128, 128), bf16)] * 4] * 6,
        [[vmem((2, 128, 128), bf16)] * 4] * 8,
        [vmem((5, 128, 128), f32)] * 2,
        [vmem((2, 128, 128), f32)] * 4,
        [vmem((2, 128, 128), f32)] * 2,
        [vmem((6, 8, 128), f32)] * 8,
        [[vmem((2, 8, 128), f32)] * 4] * 8,
        [vmem((4, 128, 128), bf16)] * 20,
        [vmem((5, 128, 128), f32)] * 8,
        [vmem((10, SUB, 128), f32)] * 2,
        [vmem((10, SUB, 128), f32)] * 2,
        [vmem((8, 4, HS, 128), bf16)] * 6,
        [vmem((10, SUB, 128), f32)] * 2,
        [vmem((10, HALO + SUB, 128), f32)] * 2,
        [vmem((10, HALO + SUB, 128), f32)] * 2,
        [[vmem((9, 32, 128), f32)] * 4] * 2,
        [[[vmem((WIN + 2, 16, 128), f32)] * 2] * 8] * 2,
        [[vmem((2, SUB, 128), f32)] * 2] * 4,
        [vmem((2, SUB, 128), f32)] * 7,
        vmem((1, H), bf16),
        pltpu.SemaphoreType.DMA((5,)),
        pltpu.SemaphoreType.DMA((10,)),
        pltpu.SemaphoreType.DMA((NSUB,)),
    ]
    out = pl.pallas_call(
        _kernel,
        out_shape=jax.ShapeDtypeStruct((S, D), bf16),
        in_specs=[hbm] * 8,
        out_specs=hbm,
        scratch_shapes=scratch,
        compiler_params=pltpu.CompilerParams(vmem_limit_bytes=112 * 1024 * 1024, flags={"XLA_TPU_FORCE_LP_LLO_SCHEDULER": True}),
        name="interleaved_layers",
    )(A_x.reshape(S, D), A_wq, A_wk, A_wv, A_wo, A_beta.reshape(1, H), B_wqkv, B_wo)
    return out.reshape(1, S, D)
```

```python
import math
from functools import partial, reduce

import jax
import jax.numpy as jnp
import numpy as np
from jax import lax
from jax.experimental import pallas as pl
from jax.experimental.pallas import tpu as pltpu

S = 2048
D = 1024
HALF = D // 2
H = 32
DH = 32
SEG = 512
WIN, DIL = 8, 2
HALO = 16
SUB = 128
HS = SUB // 2
NSUB = S // SUB
LOG2E = math.log2(math.e)
QK_SCALE = DH ** -0.5 * LOG2E
MASKED = -1e9 * LOG2E

f32 = jnp.float32
bf16 = jnp.bfloat16
u32 = jnp.uint32


def _mm(a, b):
    return lax.dot_general(a, b, (((1,), (0,)), ((), ())), preferred_element_type=f32)


def _iota(shape, axis):
    return lax.broadcasted_iota(jnp.int32, shape, axis)


def _words(ref, lead, r, n):
    return ref.bitcast(u32)[(*lead, pl.ds(r // 2, n // 2), slice(None))]


def _ld16(ref, lead, r, n):
    return pltpu.bitcast(_words(ref, lead, r, n), bf16)


def _pair(lo, hi):
    return (pltpu.bitcast(lo.astype(f32), u32) >> 16) | pltpu.bitcast(hi.astype(f32), u32)


def _unpair(w, i):
    return pltpu.bitcast(w & np.uint32(0xFFFF0000) if i else w << 16, f32)


def _phi(t):
    return jnp.where(t > 0, t + 1.0, jnp.exp(t))


def _row_mean(tiles):
    return jnp.sum(reduce(jnp.add, tiles), axis=-1, keepdims=True) * (1.0 / D)


def _swap_odd_heads(lo, hi):
    odd = (_iota(lo.shape, 1) & DH) != 0
    return jnp.where(odd, hi, lo), jnp.where(odd, lo, hi)


def _put_left(dsts, k, r, a11, a12, a21, a22, which=range(7)):
    ops = (a11 + a22, a21 + a22, a11, a22, a11 + a12, a21 - a11, a12 - a22)
    for i in which:
        for dst in dsts:
            dst[i, k, pl.ds(r, a11.shape[0]), :] = ops[i].astype(bf16)


def _put_right(dst, t, r, b11, b12, b21, b22):
    for i, op in enumerate((b11 + b22, b11, b12 - b22, b21 - b11, b22, b11 + b12, b21 + b22)):
        dst[i, t, pl.ds(r, b11.shape[0]), :] = op.astype(bf16)


def _strassen(prod, emit, park, zero):
    m1 = prod(0)
    rows = pl.ds(0, m1.shape[0])
    yield m1
    m4 = prod(3)
    park[0][0, rows, :] = m1 + m4
    yield m4
    m2 = prod(1)
    emit(1, 0, m2 + m4)
    park[1][0, rows, :] = m1 - m2
    yield m2
    m6 = prod(5)
    yield m6
    m3 = prod(2)
    emit(1, 1, park[1][zero, rows, :] + (m6 + m3))
    yield m3
    m5 = prod(4)
    emit(0, 1, m3 + m5)
    yield m5
    m7 = prod(6)
    emit(0, 0, park[0][zero, rows, :] + (m7 - m5))
    yield m7


def _strassen_lean(prod, emit, park, zero):
    m = prod(0)
    park[0][0] = m
    yield m
    m = prod(3)
    park[1][0] = park[0][zero] + m
    park[2][0] = m
    yield m
    m = prod(1)
    emit(1, 0, park[2][zero] + m)
    park[3][0] = park[0][zero] - m
    yield m
    m = prod(5)
    park[4][0] = park[3][zero] + m
    yield m
    m = prod(2)
    emit(1, 1, park[4][zero] + m)
    park[5][0] = m
    yield m
    m = prod(4)
    emit(0, 1, park[5][zero] + m)
    park[6][0] = park[1][zero] - m
    yield m
    m = prod(6)
    emit(0, 0, park[6][zero] + m)
    yield m


def _fence(buf, tick):
    if buf.dtype == bf16:
        spare = (buf.shape[0] - 1, 0) if len(buf.shape) == 4 else (pl.ds(buf.shape[0] - 16, 16),)
        buf[(*spare, *[pl.ds(0, 16)] * (len(spare) - 1), pl.ds(0, 128))] = (
            jnp.concatenate([tick, tick], axis=0).astype(bf16))
    else:
        buf[buf.shape[0] - 1, pl.ds(0, 8), :] = pltpu.bitcast(tick, buf.dtype)


def _spread(jobs, first, last):
    return [(first + (last - first) * i / len(jobs), job) for i, job in enumerate(jobs)]


def _paced(stages, jobs):
    jobs = sorted(jobs, key=lambda j: j[0])
    n = 0
    for i, prod in enumerate(p for stage in stages for p in stage):
        while n < len(jobs) and jobs[n][0] < i + 1:
            r = 8 * int(max(jobs[n][0] - i, 0) * (prod.shape[0] // 8))
            jobs[n][1](prod[r:r + 8])
            n += 1
        yield prod
    assert n == len(jobs)


def _kernel(x_hbm, wq_hbm, wk_hbm, wv_hbm, wo_hbm, beta_hbm, bqkv_hbm, bo_hbm, out_hbm,
            xbuf, raw_vkq, raw_o, raw_bqkv, raw_bo, w_kq, w_v, w_o, w_bq, w_bk, w_bv, w_bo,
            xn, vbuf, obuf, gate, causal, perm_c, perm_r,
            p0_l, p1_q, p1_pq, p1_k, p1_pk, p1_v, p1_f, p1_m, p1_mt, p1_x, p1_l, p1_p, p1_s,
            p2_t, p2_x, p2_l, p2_q, p2_k, p2_v, p2_o, p2_a, stat, park, beta,
            x_sem, v_sem, w_sem, o_sem):
    lane8, row8 = _iota((8, 128), 1), _iota((8, 128), 0)

    x_edges = (0, 2 * SUB, SUB + SEG, SUB + 2 * SEG, SUB + 3 * SEG, S)

    def x_copy(i):
        rows = pl.ds(x_edges[i], x_edges[i + 1] - x_edges[i])
        return pltpu.make_async_copy(x_hbm.at[rows], xbuf.at[rows], x_sem.at[i])

    def wv_copies(i):
        rows = [pl.ds(128 * i + rh * HALF, 128) for rh in range(2)]
        return [pltpu.make_async_copy(wv_hbm.at[r], raw_vkq.at[0, r], v_sem.at[2 * i + rh])
                for rh, r in enumerate(rows)]

    def w_copy(i):
        src = (wk_hbm, wq_hbm, wo_hbm, bo_hbm)[i]
        dst = (raw_vkq.at[1], raw_vkq.at[2], raw_o, raw_bo)[i]
        return pltpu.make_async_copy(src, dst.at[pl.ds(0, D)], w_sem.at[i])

    def bqkv_copies(i):
        rows = [pl.ds(128 * i + rh * HALF, 128 + 256 * i) for rh in range(2)]
        return [pltpu.make_async_copy(bqkv_hbm.at[r], raw_bqkv.at[r], w_sem.at[4 + 2 * i + rh])
                for rh, r in enumerate(rows)]

    def out_copy(unit):
        rows = pl.ds(pl.multiple_of(unit * SUB, SUB), SUB)
        return pltpu.make_async_copy(xbuf.at[rows], out_hbm.at[rows], o_sem.at[unit])

    beta_copy = pltpu.make_async_copy(beta_hbm, beta, w_sem.at[8])
    for cp in [x_copy(0), beta_copy] + wv_copies(0):
        cp.start()
    x_copy(0).wait()
    for cp in wv_copies(1) + wv_copies(2):
        cp.start()
    beta_copy.wait()

    sig = 1.0 / (1.0 + jnp.exp(-beta[...].astype(f32)))
    for g in range(8):
        pick = _iota((8, H), 0) + 4 * g == _iota((8, H), 1)
        gate[g] = jnp.broadcast_to(
            jnp.sum(jnp.where(pick, sig, 0.0), axis=1, keepdims=True), (8, 128))
    lane = _iota((128, 128), 1)
    for i, query in enumerate((lane, lane ^ HS, lane | HS)):
        causal[i] = jnp.where(_iota((128, 128), 0) <= query, 0.0, MASKED)

    def quads(upper, lower, r, n, t):
        return [half[pl.ds(r, n), pl.ds(128 * (t + 4 * ch), 128)].astype(f32)
                for half in (upper, lower) for ch in range(2)]

    def band(ref, start, n):
        rows = pl.ds(pl.multiple_of(start, n), n)
        return ref.at[(slice(None),) * (len(ref.shape) - 2) + (rows,)]

    def project(left, r, n, right, t, emit, zero, first=0):
        def prod(i):
            lhs = jnp.concatenate([_ld16(left, (i + zero, k), r, n) for k in range(4)], axis=1)
            return _mm(lhs, _ld16(right, (first + i, t), 0, HALF))
        return (_strassen_lean if n == SUB else _strassen)(prod, emit, park, zero)

    def norm_jobs(src, src_buf, st, dsts, zero, t0, t1):
        def mean_job(r, tick):
            _fence(src_buf, tick)
            st[0][0, pl.ds(r, 16), :] = jnp.broadcast_to(
                _row_mean([src(g, r, 16) for g in range(8)]), (16, 128))

        def var_job(r, tick):
            _fence(st[0], tick)
            mean = st[0][zero, pl.ds(r, 8), :]
            dev = [src(g, r, 8) - mean for g in range(8)]
            st[1][0, pl.ds(r, 8), :] = jnp.broadcast_to(
                lax.rsqrt(_row_mean([d * d for d in dev]) + 1e-5), (8, 128))

        def out_job(r, k, which, tick):
            for buf in (src_buf, *st):
                _fence(buf, tick)
            mean, rstd = ([b[zero, pl.ds(rh * HS + r, 16), :] for rh in range(2)] for b in st)
            _put_left(dsts, k, r, *[(src(k + 4 * ch, rh * HS + r, 16) - mean[rh]) * rstd[rh]
                                    for rh in range(2) for ch in range(2)], which=which)

        work = t1 - t0 - 4
        return (_spread([partial(mean_job, r) for r in range(0, SUB, 16)], t0, t0 + 0.15 * work)
                + _spread([partial(var_job, r) for r in range(0, SUB, 8)],
                          t0 + 2 + 0.15 * work, t0 + 2 + 0.45 * work)
                + _spread([partial(out_job, r, k, which) for r in range(0, HS, 16) for k in range(4)
                           for which in ((2, 4, 6), (0, 1, 3, 5))], t0 + 4 + 0.45 * work, t1))

    def out_operands(dst, k, r, src, g0, g1, zero):
        o = [_swap_odd_heads(*[src[g + zero, pl.ds(rh * HS + r, 16), :] for rh in range(2)])
             for g in (g0, g1)]
        _put_left([dst], k, r, o[0][0], o[1][0], o[0][1], o[1][1])

    def first_norm(i, _):
        r = pl.multiple_of(i * 32, 32)
        rows = []
        for rh in range(2):
            x = xbuf[pl.ds(r + rh * HS, 32), :].astype(f32)
            d = x - _row_mean([x])
            rows.append(d * lax.rsqrt(_row_mean([d * d]) + 1e-5))
        for k in range(4):
            _put_left([xn, p0_l[0]], k, r,
                      *[y[:, 128 * g:128 * (g + 1)] for y in rows for g in (k, k + 4)])

    def value_weights(i, _):
        halves = [band(raw_vkq.at[0], i * 64 + rh * HALF, 64) for rh in range(2)]
        for t in range(4):
            _put_right(band(w_v, i * 64, 64), t, 0, *quads(*halves, 0, 64, t))

    def phase0(first, c):
        zero = c >> 4
        jobs = []
        if first:
            for i in range(4):
                @pl.when(c == i)
                def _():
                    for cp in ([], [x_copy(2)], [x_copy(3), w_copy(0)], [x_copy(4), w_copy(1)])[i]:
                        cp.wait()
                    for cp in ([x_copy(2), x_copy(3), x_copy(4)], [w_copy(0), w_copy(1)],
                               [w_copy(2), w_copy(3)] + bqkv_copies(0), [])[i]:
                        cp.start()

            def arrive(tick):
                pl.when(c == 0)(x_copy(1).wait)

            raw = raw_vkq.at[jnp.maximum(c - 1, 0) + zero]
            dst = w_kq.at[pl.ds(7 * jnp.maximum(c - 2, 0), 7)]

            def weights(r, t, tick):
                _fence(raw_vkq.at[0], tick)
                _put_right(dst, t, r, *quads(raw, raw.at[pl.ds(HALF, HALF)], r, 16, t))

            jobs += [(24, arrive)] + _spread(
                [partial(weights, r, t) for r in range(0, HALF, 16) for t in range(4)], 0, 110)

        def values(u):
            for t in range(4):
                def emit(rh, ch, val):
                    vbuf[t + 4 * ch, c * 4 + u, pl.ds(rh * HS, HS), :] = val.astype(bf16)
                yield from project(p0_l[u], 0, HS, w_v, t, emit, zero)

        def norm(u, t0, t1):
            unit = c * 4 + u + 1
            x = band(xbuf, (unit if u < 3 else jnp.minimum(unit, NSUB - 1)) * SUB, SUB)
            return norm_jobs(lambda g, r, n: x[pl.ds(r, n), pl.ds(128 * g, 128)].astype(f32), xbuf,
                             stat[(u + 1) % 4], [band(xn, unit * HS, HS), p0_l[(u + 1) % 4]],
                             zero, t0, t1)

        jobs += norm(0, 0, 24) + norm(1, 24, 52) + norm(2, 52, 80) + norm(3, 80, 110)
        jobs.sort(key=lambda j: j[0])
        for i in range(1, len(jobs)):
            jobs[i] = (max(jobs[i][0], jobs[i - 1][0] + 0.2), jobs[i][1])
        for _ in _paced([values(u) for u in range(4)], jobs):
            pass

    def phase1(layer, t):
        zero = t >> 4
        never = row8 < zero
        st = {}
        turns = []
        todo = []

        @pl.when(jnp.logical_and(layer == 0, t == 1))
        def _():
            for cp in bqkv_copies(1):
                cp.wait()

        def turn(buf, tick, read):
            if len(turns) >= 3:
                tick = pltpu.bitcast(pltpu.bitcast(tick, u32) | turns[-3], f32)
            _fence(buf, tick)
            y = read().T
            turns.append(pltpu.bitcast(y[:16 if y.dtype == bf16 else 8], u32))
            return y

        def plain_weights(r, k, tick):
            _fence(raw_o, tick)
            halves = [band(raw_o, t * 128 + rh * HALF, 128) for rh in range(2)]
            _put_right(band(w_o, t * 128, 128), k, r, *quads(*halves, r, 16, k))

        def column_weights(m, dst):
            turned, back = perm_c[m]

            def there(c, tick):
                w = turn(raw_bqkv, tick, lambda: _pair(*[
                    band(raw_bqkv, t * 128 + rh * HALF, 128)[:, pl.ds(m * D + 128 * c, 128)]
                    for rh in range(2)]))
                for j in range(4):
                    turned[0, pl.ds((4 * c + j) * (DH + 1), DH), :] = w[j * DH:(j + 1) * DH]

            def again(c, tick):
                back[c] = turn(turned, tick, lambda: jnp.concatenate(
                    [turned[zero, pl.ds(d, H, stride=DH + 1), :] for d in range(4 * c, 4 * c + 4)],
                    axis=0))

            def operands(r, k, tick):
                _fence(back, tick)
                w = [back[k + 4 * ch + zero, pl.ds(r, 16), :] for ch in range(2)]
                _put_right(band(dst, t * 128, 128), k, r,
                           *[_unpair(w[ch], rh) for rh in range(2) for ch in range(2)])
            return ([partial(there, c) for c in range(8)], [partial(again, c) for c in range(8)],
                    [partial(operands, r, k) for r in range(0, 128, 16) for k in range(4)])

        def pad_head(h, tick):
            _fence(raw_bo, tick)
            perm_r[0, pl.ds(h * (DH + 1), DH), :] = _pair(*[
                raw_bo[pl.ds(h * DH, DH), pl.ds(pl.multiple_of(t * 128 + ch * HALF, 128), 128)]
                for ch in range(2)])

        def row_weights(d, h, tick):
            _fence(perm_r, tick)
            w = [perm_r[zero, pl.ds(h * (DH + 1) + d + rh * (DH // 2), 16, stride=DH + 1), :]
                 for rh in range(2)]
            _put_right(w_bo, t, d * H + h, *[_unpair(w[rh], ch) for rh in range(2) for ch in range(2)])

        def turn_q(s, ch, blk, tick):
            def read():
                y = p1_f[blk // 2][2 * ch + blk % 2 + zero]
                return jnp.concatenate(_swap_odd_heads(y[:HS], y[HS:]), axis=0)
            y = turn(p1_f[blk // 2], tick, read)
            p1_q[2 * s + ch][blk][0] = (y * QK_SCALE).astype(bf16)
            if s > 0:
                p1_pq[2 * s + ch - 2][blk][0] = _phi(y).astype(bf16)
            st['q', s, ch, blk] = True

        def turn_v(s, blk, tick):
            y = turn(vbuf, tick, lambda: jnp.concatenate(
                [vbuf[t + 4 * ch, 4 * s + blk] for ch in range(2)], axis=1))
            for ch in range(2):
                p1_v[2 * s + ch][blk][0] = y[128 * ch:128 * (ch + 1)]

        def projection(is_q, s, half, extra):
            def emit(rh, ch, val):
                slot, rows = 2 * s + ch, pl.ds(rh * HS, HS)
                for u in range(2):
                    y = val[HS * u:HS * (u + 1)]
                    if is_q:
                        p1_f[half][2 * ch + u, rows, :] = y
                        continue
                    p1_k[slot][2 * half + u][0, rows, :] = y.astype(bf16)
                    if s < 3:
                        pk = _phi(y)
                        p1_pk[slot][2 * half + u][0, rows, :] = pk.astype(bf16)
                        z = jnp.sum(pk.reshape(HS // 8, 8, 128), axis=0)
                        st['dz', slot] = z + st['dz', slot] if ('dz', slot) in st else z
            jobs = (_spread(todo + [partial(turn_v, s, 2 * half + 1 - is_q)], 0, 7)
                    + _spread(extra, 0, 7))
            todo.clear()
            yield from _paced(
                [project(xn, (4 * s + 2 * half) * HS, SUB, w_kq, t, emit, zero, 7 * is_q)], jobs)
            if is_q:
                todo.extend(partial(turn_q, s, ch, 2 * half + u) for ch in range(2) for u in (1, 0))
            st['k', s, half, is_q] = True

        def scores(a, n, s, ch, i, kb):
            assert st['q', s, ch, i] and st['k', s, kb // 2, False]
            slot, buf, tops = 2 * s + ch, p1_s[a % len(p1_s)], p1_x[n % len(p1_x)]
            head = lambda at, j: _words(p1_q[slot][i], (at,), DH * j, DH)

            def queries(first, parts):
                pads = [[jnp.zeros((DH // 2 * k, 128), u32)] if k else []
                        for k in (first, 4 - first - len(parts))]
                return pltpu.bitcast(jnp.concatenate(pads[0] + parts + pads[1], axis=0), bf16)

            nk = HS if kb == i else 128
            k = _ld16(p1_k[slot][kb], (zero,), 0, nk)
            for j in range(4):
                sc = _mm(k, queries(j, [head(zero, j)]))
                if kb == i:
                    sc = sc + causal[j % 2 + zero, pl.ds(0, HS), :]
                buf[j, pl.ds(0, nk), :] = sc
                m = jnp.max(sc.reshape(nk // 8, 8, 128), axis=0)
                st['m', n, j] = jnp.maximum(m, st['m', n, j]) if kb > 0 else m
            if kb < i:
                return sc
            upper = _iota((DH // 2, 128), 1) >= HS
            for j in (0, 2):
                m = []
                for r in (HS, HS + 32):
                    at = zero if r == HS else t >> 5
                    q = [jnp.where(upper, head(at, j), 0), jnp.where(upper, 0, head(at, j + 1))]
                    up = _mm(_ld16(p1_k[slot][kb], (zero,), r, 32), queries(j, q))
                    up = up + causal[2 + zero, pl.ds(r, 32), :]
                    buf[j, pl.ds(r, 32), :] = up
                    m.append(jnp.max(up.reshape(4, 8, 128), axis=0))
                m, both = jnp.maximum(*m), []
                for jj, own in ((j, lane8 >= HS), (j + 1, lane8 < HS)):
                    top = jnp.where(own, jnp.maximum(st['m', n, jj], m), st['m', n, jj])
                    both.append(jnp.broadcast_to(jnp.max(top, axis=0, keepdims=True), (8, 128)))
                    tops[jj] = both[-1]
                tops[4 + j // 2] = jnp.where(lane8 >= HS, *both)
            st['top', n] = True
            return jnp.concatenate([sc, up], axis=0)

        def probs(a, n, s, ch, i, kb, ticks):
            assert st['top', n]
            buf, out, tot = p1_s[a % len(p1_s)], p1_p[a % len(p1_p)], p1_l[n % len(p1_l)]
            runs = [(j, 0, HS if kb == i else 128) for j in range(4)]
            if kb == i:
                runs += [(j, HS, 128) for j in (0, 2)]
            count, c = sum(hi - lo for _, lo, hi in runs) // 32, 0
            for j, lo, hi in runs:
                top, l = p1_x[n % len(p1_x)][(4 + j // 2 if lo else j) + zero], None
                for r in range(lo, hi, 32):
                    m = jnp.where(never, ticks[c * len(ticks) // count], top)
                    c += 1
                    p = jnp.exp2(buf[j + zero, pl.ds(r, 32), :] - jnp.concatenate([m] * 4, axis=0))
                    for x in range(0, 32, 8):
                        l = p[x:x + 8] if l is None else l + p[x:x + 8]
                    if lo:
                        upper = _iota((32, 128), 1) >= HS
                        out[j, pl.ds(r, 32), :] = jnp.where(upper, p, 0.0).astype(bf16)
                        out[j + 1, pl.ds(r, 32), :] = jnp.where(upper, 0.0, p).astype(bf16)
                    else:
                        out[j, pl.ds(r, 32), :] = p.astype(bf16)
                if lo:
                    for jj, own in ((j, lane8 >= HS), (j + 1, lane8 < HS)):
                        tot[jj][0] = jnp.broadcast_to(jnp.sum(
                            tot[jj][zero] + jnp.where(own, l, 0.0), axis=0, keepdims=True), (8, 128))
                else:
                    tot[j][0] = l + tot[j][zero] if kb > 0 else l

        def values(a, n, s, ch, i, kb):
            tot = [x[zero] for x in p1_l[n % len(p1_l)]]
            scale = (1.0 - gate[t + 4 * ch]) / jnp.where(
                row8 < 2, jnp.where(row8 == 0, tot[0], tot[1]), jnp.where(row8 == 2, tot[2], tot[3]))
            o, ticks = [None] * 4, []
            for b in range(i + 1):
                for j in range(4):
                    pv = _mm(_ld16(p1_v[2 * s + ch][b], (zero,), DH * j, DH),
                             _ld16(p1_p[(a - i + b) % len(p1_p)], (j + zero,), 0, 128))
                    o[j] = o[j] + pv if b else pv
                ticks.append(pv)
            for j in range(4):
                y = o[j] * scale[j:j + 1]
                if s > 0:
                    assert st['read', ch, i // 2] == s
                    y = y + p1_m[2 * ch + i // 2][i % 2 + zero, pl.ds(DH * j, DH), :]
                obuf[t + 4 * ch, pl.ds(SEG * s + 128 * i + DH * j, DH), :] = y
            return jnp.concatenate(ticks, axis=0)

        def mem_read(s, ch, half):
            assert st['memory', ch] == s
            z = jnp.sum(st['z', ch], axis=0, keepdims=True)
            lhs = jnp.concatenate(
                [jnp.where((lane8 >> 5) == row8, z, 0.0)]
                + [jnp.where((_iota((DH, 128), 1) >> 5) == j, p1_mt[ch][zero, pl.ds(DH * j, DH), :], 0.0)
                   for j in range(4)], axis=0)
            for b in (2 * half, 2 * half + 1):
                assert st['q', s, ch, b]
                nd = _mm(lhs, _ld16(p1_pq[2 * s + ch - 2][b], (zero,), 0, 128))
                inv = gate[t + 4 * ch] / (nd[0:8] + 1e-6)
                for j in range(4):
                    p1_m[2 * ch + half][b % 2, pl.ds(DH * j, DH), :] = (
                        nd[8 + DH * j:8 + DH * (j + 1)] * inv[j:j + 1])
            st['read', ch, half] = s
            return nd

        def mem_update(s, ch):
            assert st['k', s, 0, False] and st['k', s, 1, False]
            slot = 2 * s + ch
            v = jnp.concatenate([_ld16(p1_v[slot][b], (zero,), 0, 128) for b in range(4)], axis=1)
            pk = jnp.concatenate([_ld16(p1_pk[slot][b], (zero,), 0, 128) for b in range(4)], axis=0)
            mt = _mm(v, pk)
            p1_mt[ch][0] = mt + p1_mt[ch][zero] if s > 0 else mt
            st['z', ch] = st['dz', slot] + st['z', ch] if s > 0 else st['dz', slot]
            st['memory', ch] = s + 1
            return mt

        def first_turn(ch, tick):
            p2_t[0][ch] = turn(obuf, tick, lambda: obuf[t + 4 * ch, pl.ds(0, SUB), :])

        def first_operands(r, tick):
            _fence(p2_t[0], tick)
            out_operands(p2_l[0], t, r, p2_t[0], 0, 1, zero)

        tiles = []
        for s in range(4):
            for half in ((0, 1) if s == 0 else (1, 0)):
                for i in (2 * half + 1, 2 * half):
                    for ch in range(2):
                        n = tiles[-1][0] + 1 if tiles else 0
                        tiles += [(n, s, ch, i, kb) for kb in range(i + 1)]
        blocks = [(True, 0, 0), (False, 0, 0), (True, 0, 1), (False, 0, 1)]
        for s in range(1, 4):
            blocks += [(True, s, 1), (False, s, 0), (False, s, 1), (True, s, 0)]
        cq, ck, cv = (column_weights(m, dst) for m, dst in enumerate((w_bq, w_bk, w_bv)))
        ro = [partial(row_weights, d, h) for d in range(DH // 2) for h in (0, 16)]
        side = [cq[0], [partial(plain_weights, r, k) for r in range(0, 128, 16) for k in range(4)],
                ck[0][:4], ck[0][4:] + cv[0][:4],
                cq[1], [partial(pad_head, h) for h in range(H)], cv[0][4:], ck[1][:4],
                ck[1][4:] + cq[2][:16], cq[2][16:], cv[1][:4], cv[1][4:],
                [partial(first_turn, ch) for ch in range(2)] + ro[:16], ck[2],
                [partial(first_operands, r) for r in range(0, HS, 16)] + ro[16:], cv[2]]
        stream = (p for blk, jobs in zip(blocks, side) for p in projection(*blk, jobs))

        issued = exps = 0
        ready, owed = [0, 0, 0], []
        for a in range(len(tiles) + 3):
            s, pos = divmod(a, 20)
            prods = []
            if 0 < s < 4 and pos in ((2, 13) if s < 3 else (10, 14)):
                prods.append([mem_read(s, ch, int(pos < 13)) for ch in range(2)][1])
            if s < 3 and pos in (16, 18):
                prods.append(mem_update(s, (pos - 16) // 2))
            due = min(int(24 + 1.4 * a) if a < 59 else 47 + a, 7 * len(blocks))
            prods.extend(next(stream) for _ in range(issued, due))
            issued = due
            if a < len(tiles):
                assert a - exps < len(p1_s)
                prods.append(scores(a, *tiles[a]))
            owed += [b for b in range(ready[-3], ready[-2]) if tiles[b][3] == tiles[b][4]]
            for b in owed[:{77: 1, 79: 1, 80: 2}.get(a, 0) if 68 <= a <= 80 else None]:
                assert exps - (b - tiles[b][3]) <= len(p1_p)
                assert tiles[exps - 1][0] - tiles[b][0] < len(p1_l)
                owed.remove(b)
                prods.append(values(b, *tiles[b]))
            if due == 7 * len(blocks):
                next(stream, None)
                if todo:
                    todo.pop(0)(prods[0][0:8])
            upto = min(max(a - 3, exps, {77: 75, 78: 76, 79: 78, 80: 80}.get(a, 0)), len(tiles))
            ticks = [x[r:r + 8] for x in prods[-4:] for r in range(0, x.shape[0], 8)]
            if a == len(tiles):
                ticks = ticks[:16]
            for b in range(exps, upto):
                share = len(ticks) // (upto - exps)
                probs(b, *tiles[b], ticks[(b - exps) * share:(b + 1 - exps) * share])
            exps = upto
            ready.append(exps)
        assert not todo and not owed and ready[-3] == len(tiles)

    def phase2(layer, c):
        zero = c >> 4

        def rows(u, rh):
            return pl.ds(pl.multiple_of((2 * c + u) * SUB + rh * HS, HS), HS)

        def out_jobs(unit, u, t0, t1):
            def turn(g, tick):
                _fence(obuf, tick)
                p2_t[u][g] = obuf[g, pl.ds(pl.multiple_of(unit * SUB, SUB), SUB), :].T

            def operands(r, k, tick):
                _fence(p2_t[u], tick)
                out_operands(p2_l[u], k, r, p2_t[u], k, k + 4, zero)
            return (_spread([partial(turn, g) for g in range(8)], t0, t0 + 6)
                    + _spread([partial(operands, r, k) for r in range(0, HS, 16) for k in range(4)],
                              t0 + 10, t1))

        def infini_out(u):
            for t in range(4):
                def emit(rh, ch, val):
                    g = t + 4 * ch
                    x = xbuf[rows(u, rh), pl.ds(128 * g, 128)].astype(f32)
                    p2_x[u][g, pl.ds(rh * HS, HS), :] = x + val
                yield from project(p2_l[u], 0, HS, w_o, t, emit, zero)

        def norm(u, t0, t1):
            return norm_jobs(lambda g, r, n: p2_x[u][g + zero, pl.ds(r, n), :], p2_x[u], stat[u],
                             [p2_l[2 + u]], zero, t0, t1)

        def local_proj(u, w, dst, off):
            for t in range(4):
                def emit(rh, ch, val):
                    dst[u][t + 4 * ch, pl.ds(off + rh * HS, HS), :] = val
                    if off and rh == 1 and u == 0:
                        dst[1][t + 4 * ch, pl.ds(0, HALO), :] = val[HS - HALO:]
                yield from project(p2_l[2 + u], 0, HS, w, t, emit, zero)

        def attend(u, t0, t1, t2, t3):
            held = {}

            def taps(buf, g, r, w):
                x = buf[g + zero, pl.ds(HALO + r - DIL * w - 8, 24), :]
                return (w, x[8:]), (w + WIN // 2, x[:16])

            def logits(r, w0, g, tick):
                _fence(p2_q[u], tick)
                q = p2_q[u][g + zero, pl.ds(r, 16), :]
                for w, k in taps(p2_k[u], g, r, w0) + taps(p2_k[u], g, r, w0 + 1):
                    a = held[w] = q * k if g == 0 else held[w] + q * k
                    if g < 7:
                        continue
                    a = (a + pltpu.roll(a, 64, 1)) + (pltpu.roll(a, 32, 1) + pltpu.roll(a, 96, 1))
                    a = a * QK_SCALE
                    if u == 0 and r == 0 and w > 0:
                        a = jnp.where(2 * c * SUB + _iota((16, 128), 0) >= DIL * w, a, MASKED)
                    p2_a[u][r // 16][0][w] = a

            def softmax(r, tick):
                src, dst = p2_a[u][r // 16]
                _fence(src, tick)
                lg = [src[w + zero, pl.ds(r % 16, 8), :] for w in range(WIN)]
                top = reduce(jnp.maximum, lg)
                ex = [jnp.exp2(a - top) for a in lg]
                for w in range(WIN):
                    dst[w, pl.ds(r % 16, 8), :] = ex[w]
                dst[WIN, pl.ds(r % 16, 8), :] = 1.0 / reduce(jnp.add, ex)

            def mix(r, g, tick):
                _fence(p2_v[u], tick)
                if g % 2 == 0:
                    _fence(p2_a[u][r // 16][1], tick)
                    held['p'] = [p2_a[u][r // 16][1][w + zero] for w in range(WIN + 1)]
                acc = reduce(jnp.add, [held['p'][w] * v for w0 in range(WIN // 2)
                                       for w, v in taps(p2_v[u], g, r, w0)])
                p2_o[u][r % HS // 16][g, pl.ds(r // HS * 16, 16), :] = acc * held['p'][WIN]

            def operands(j, k, tick):
                _fence(p2_o[u][j], tick)
                _put_left([p2_l[4 + u]], k, 16 * j,
                          *[p2_o[u][j][g + zero, pl.ds(16 * rh, 16), :]
                            for rh in range(2) for g in (k, k + 4)])

            order = [rh * HS + r for r in range(0, HS, 16) for rh in range(2)]
            lag, step = (t1 - t0) / 8 + 3.06, (t3 - t2) / 4
            return (_spread([partial(logits, r, w, g) for r in order for w in (0, 2) for g in range(8)],
                            t0, t1)
                    + _spread([partial(softmax, r + i) for r in order for i in (0, 8)],
                              t0 + lag, t1 + lag)
                    + _spread([partial(mix, r, g) for r in order for g in range(8)], t2, t3)
                    + [(t2 + step * (j + 1) + (step / 4 if j < 3 else 0.3) * k + 0.2,
                        partial(operands, j, k)) for j in range(4) for k in range(4)])

        def local_out(u):
            for t in range(4):
                def emit(rh, ch, val):
                    g = t + 4 * ch
                    y = p2_x[u][g + zero, pl.ds(rh * HS, HS), :] + val
                    xbuf[rows(u, rh), pl.ds(128 * g, 128)] = y.astype(bf16)
                yield from project(p2_l[4 + u], 0, HS, w_bo, t, emit, zero)

        def send(u, tick=None):
            pl.when(layer == 1)(out_copy(2 * c + u).start)

        stages = [infini_out(0), infini_out(1)]
        for u in range(2):
            stages += [local_proj(u, w_bk, p2_k, HALO), local_proj(u, w_bq, p2_q, 0),
                       local_proj(u, w_bv, p2_v, HALO)]
        stages += [local_out(0), local_out(1)]
        jobs = (out_jobs(2 * c + 1, 1, 0, 24) + out_jobs(jnp.minimum(2 * c + 2, NSUB - 1), 0, 250, 279)
                + norm(0, 28, 52) + norm(1, 58, 110) + [(252, partial(send, 0))]
                + attend(0, 112, 150, 156, 194) + attend(1, 196, 221, 224, 247))
        for _ in _paced(stages, jobs):
            pass
        for buf in (p2_k, p2_v):
            for g in range(8):
                buf[0][g, pl.ds(0, HALO), :] = buf[1][g + zero, pl.ds(SUB, HALO), :]
        send(1)

    def layer_pair(layer, _):
        lax.fori_loop(0, HS // 32, first_norm, None)

        @pl.when(layer == 0)
        def _():
            for i in range(4):
                for cp in wv_copies(i):
                    cp.wait()
                for cp in (wv_copies(3), [], [x_copy(1)], [])[i]:
                    cp.start()
                lax.fori_loop(2 * i, 2 * i + 2, value_weights, None)
            lax.fori_loop(0, 4, lambda c, _: phase0(True, c), None)
            for cp in [w_copy(2), w_copy(3)] + bqkv_copies(0):
                cp.wait()
            for cp in bqkv_copies(1):
                cp.start()

        @pl.when(layer == 1)
        def _():
            lax.fori_loop(0, 4, lambda c, _: phase0(False, c), None)

        lax.fori_loop(0, 4, lambda t, _: phase1(layer, t), None)
        for buf in (p2_k, p2_v):
            buf[0][pl.ds(0, 8), pl.ds(0, HALO), :] = jnp.zeros((8, HALO, 128), f32)
        lax.fori_loop(0, NSUB // 2, lambda c, _: phase2(layer, c), None)

    lax.fori_loop(0, 2, layer_pair, None)
    for unit in range(NSUB):
        out_copy(unit).wait()


@jax.jit
def pallas_interleave_layers__memory_aug_infini_attn__sliding_local_dilated__prompt_kernel(
    A_x: jax.Array,
    A_wq: jax.Array,
    A_wk: jax.Array,
    A_wv: jax.Array,
    A_wo: jax.Array,
    A_beta: jax.Array,
    B_x: jax.Array,
    B_wqkv: jax.Array,
    B_wo: jax.Array,
):
    del B_x
    vmem = pltpu.VMEM
    hbm = pl.BlockSpec(memory_space=pl.ANY)
    block = [vmem((2, 128, 128), bf16)] * 4
    scratch = [
        vmem((S + 16, D), bf16),
        vmem((3, D + 16, D), bf16),
        vmem((D + 16, D), bf16),
        vmem((D + 16, 3 * D), bf16),
        vmem((D + 16, D), bf16),
        vmem((14, 4, HALF, 128), bf16),
        *[vmem((7, 4, HALF, 128), bf16)] * 6,
        vmem((7, 4, (NSUB + 1) * HS, 128), bf16),
        vmem((9, NSUB, 128, 128), bf16),
        vmem((9, S, 128), f32),
        vmem((8, 8, 128), f32),
        vmem((3, 128, 128), f32),
        [[vmem((2, H * (DH + 1), 128), u32), vmem((9, 128, 128), u32)]] * 3,
        vmem((2, H * (DH + 1), 128), u32),
        [vmem((7, 4, HS, 128), bf16)] * 4,
        [block] * 8, [block] * 6,
        [block] * 8, [block] * 6,
        [block] * 8,
        [vmem((5, 128, 128), f32)] * 2,
        [vmem((2, 128, 128), f32)] * 4,
        [vmem((2, 128, 128), f32)] * 2,
        [vmem((8, 8, 128), f32)] * 8,
        [[vmem((2, 8, 128), f32)] * 4] * 8,
        [vmem((4, 128, 128), bf16)] * 20,
        [vmem((5, 128, 128), f32)] * 8,
        [vmem((10, SUB, 128), f32)] * 2,
        [vmem((10, SUB, 128), f32)] * 2,
        [vmem((8, 4, HS, 128), bf16)] * 6,
        [vmem((10, SUB, 128), f32)] * 2,
        [vmem((10, HALO + SUB, 128), f32)] * 2,
        [vmem((10, HALO + SUB, 128), f32)] * 2,
        [[vmem((9, 32, 128), f32)] * 4] * 2,
        [[[vmem((WIN + 2, 16, 128), f32)] * 2] * 8] * 2,
        [[vmem((2, SUB, 128), f32)] * 2] * 4,
        [vmem((2, SUB, 128), f32)] * 7,
        vmem((1, H), bf16),
        pltpu.SemaphoreType.DMA((5,)),
        pltpu.SemaphoreType.DMA((8,)),
        pltpu.SemaphoreType.DMA((9,)),
        pltpu.SemaphoreType.DMA((NSUB,)),
    ]
    out = pl.pallas_call(
        _kernel,
        out_shape=jax.ShapeDtypeStruct((S, D), bf16),
        in_specs=[hbm] * 8,
        out_specs=hbm,
        scratch_shapes=scratch,
        compiler_params=pltpu.CompilerParams(
            vmem_limit_bytes=112 * 1024 * 1024, flags={"XLA_TPU_FORCE_LP_LLO_SCHEDULER": True}),
        name="interleaved_layers",
    )(A_x.reshape(S, D), A_wq, A_wk, A_wv, A_wo, A_beta.reshape(1, H), B_wqkv, B_wo)
    return out.reshape(1, S, D)
```

```python
import math
from functools import partial, reduce

import jax
import jax.numpy as jnp
import numpy as np
from jax import lax
from jax.experimental import pallas as pl
from jax.experimental.pallas import tpu as pltpu

S = 2048
D = 1024
HALF = D // 2
H = 32
DH = 32
SEG = 512
WIN, DIL = 8, 2
HALO = 16
SUB = 128
HS = SUB // 2
NSUB = S // SUB
LOG2E = math.log2(math.e)
QK_SCALE = DH ** -0.5 * LOG2E
MASKED = -1e9 * LOG2E

f32 = jnp.float32
bf16 = jnp.bfloat16
u32 = jnp.uint32


def _mm(a, b):
    return lax.dot_general(a, b, (((1,), (0,)), ((), ())), preferred_element_type=f32)


def _iota(shape, axis):
    return lax.broadcasted_iota(jnp.int32, shape, axis)


def _words(ref, lead, r, n):
    return ref.bitcast(u32)[(*lead, pl.ds(r // 2, n // 2), slice(None))]


def _ld16(ref, lead, r, n):
    return pltpu.bitcast(_words(ref, lead, r, n), bf16)


def _pair(lo, hi):
    return (pltpu.bitcast(lo.astype(f32), u32) >> 16) | pltpu.bitcast(hi.astype(f32), u32)


def _unpair(w, i):
    return pltpu.bitcast(w & np.uint32(0xFFFF0000) if i else w << 16, f32)


def _phi(t):
    return jnp.where(t > 0, t + 1.0, jnp.exp(t))


def _row_mean(tiles):
    return jnp.sum(reduce(jnp.add, tiles), axis=-1, keepdims=True) * (1.0 / D)


def _swap_odd_heads(lo, hi):
    odd = (_iota(lo.shape, 1) & DH) != 0
    return jnp.where(odd, hi, lo), jnp.where(odd, lo, hi)


def _put_left(dsts, k, r, a11, a12, a21, a22, which=range(7)):
    ops = (a11 + a22, a21 + a22, a11, a22, a11 + a12, a21 - a11, a12 - a22)
    for i in which:
        for dst in dsts:
            dst[i, k, pl.ds(r, a11.shape[0]), :] = ops[i].astype(bf16)


def _put_right(dst, t, r, b11, b12, b21, b22):
    for i, op in enumerate((b11 + b22, b11, b12 - b22, b21 - b11, b22, b11 + b12, b21 + b22)):
        dst[i, t, pl.ds(r, b11.shape[0]), :] = op.astype(bf16)


def _strassen(prod, emit, park, zero):
    m1 = prod(0)
    rows = pl.ds(0, m1.shape[0])
    yield m1
    m4 = prod(3)
    park[0][0, rows, :] = m1 + m4
    yield m4
    m2 = prod(1)
    emit(1, 0, m2 + m4)
    park[1][0, rows, :] = m1 - m2
    yield m2
    m6 = prod(5)
    yield m6
    m3 = prod(2)
    emit(1, 1, park[1][zero, rows, :] + (m6 + m3))
    yield m3
    m5 = prod(4)
    emit(0, 1, m3 + m5)
    yield m5
    m7 = prod(6)
    emit(0, 0, park[0][zero, rows, :] + (m7 - m5))
    yield m7


def _strassen_lean(prod, emit, park, zero):
    m = prod(0)
    park[0][0] = m
    yield m
    m = prod(3)
    park[1][0] = park[0][zero] + m
    park[2][0] = m
    yield m
    m = prod(1)
    emit(1, 0, park[2][zero] + m)
    park[3][0] = park[0][zero] - m
    yield m
    m = prod(5)
    park[4][0] = park[3][zero] + m
    yield m
    m = prod(2)
    emit(1, 1, park[4][zero] + m)
    park[5][0] = m
    yield m
    m = prod(4)
    emit(0, 1, park[5][zero] + m)
    park[6][0] = park[1][zero] - m
    yield m
    m = prod(6)
    emit(0, 0, park[6][zero] + m)
    yield m


def _fence(buf, tick):
    if buf.dtype == bf16:
        spare = (buf.shape[0] - 1, 0) if len(buf.shape) == 4 else (pl.ds(buf.shape[0] - 16, 16),)
        buf[(*spare, *[pl.ds(0, 16)] * (len(spare) - 1), pl.ds(0, 128))] = (
            jnp.concatenate([tick, tick], axis=0).astype(bf16))
    else:
        buf[buf.shape[0] - 1, pl.ds(0, 8), :] = pltpu.bitcast(tick, buf.dtype)


def _spread(jobs, first, last):
    return [(first + (last - first) * i / len(jobs), job) for i, job in enumerate(jobs)]


def _paced(stages, jobs):
    jobs = sorted(jobs, key=lambda j: j[0])
    n = 0
    for i, prod in enumerate(p for stage in stages for p in stage):
        while n < len(jobs) and jobs[n][0] < i + 1:
            r = 8 * int(max(jobs[n][0] - i, 0) * (prod.shape[0] // 8))
            jobs[n][1](prod[r:r + 8])
            n += 1
        yield prod
    assert n == len(jobs)


def _kernel(x_hbm, wq_hbm, wk_hbm, wv_hbm, wo_hbm, beta_hbm, bqkv_hbm, bo_hbm, out_hbm,
            xbuf, raw_a, raw_bqkv, raw_bo, w_kqo, w_v, w_bq, w_bk, w_bv, w_bo,
            xn, vbuf, obuf, gate, causal, perm_c, perm_r,
            p0_l, p1_q, p1_pq, p1_k, p1_pk, p1_v, p1_f, p1_m, p1_mt, p1_x, p1_l, p1_p, p1_s,
            p2_t, p2_x, p2_l, p2_q, p2_k, p2_v, p2_o, p2_a, stat, park, beta,
            x_sem, v_sem, w_sem, o_sem):
    lane8, row8 = _iota((8, 128), 1), _iota((8, 128), 0)

    x_edges = (0, 2 * SUB, SUB + SEG, SUB + 2 * SEG, SUB + 3 * SEG, S)

    def x_copy(i):
        rows = pl.ds(x_edges[i], x_edges[i + 1] - x_edges[i])
        return pltpu.make_async_copy(x_hbm.at[rows], xbuf.at[rows], x_sem.at[i])

    def wv_copies(i):
        rows = [pl.ds(128 * i + rh * HALF, 128) for rh in range(2)]
        return [pltpu.make_async_copy(wv_hbm.at[r], raw_a.at[0, r], v_sem.at[2 * i + rh])
                for rh, r in enumerate(rows)]

    def w_copy(i):
        src = (wk_hbm, wq_hbm, wo_hbm, bo_hbm)[i]
        dst = raw_a.at[i + 1] if i < 3 else raw_bo
        return pltpu.make_async_copy(src, dst.at[pl.ds(0, D)], w_sem.at[i])

    def bqkv_copies(i):
        rows = [pl.ds(128 * i + rh * HALF, 128 + 256 * i) for rh in range(2)]
        return [pltpu.make_async_copy(bqkv_hbm.at[r], raw_bqkv.at[r], w_sem.at[4 + 2 * i + rh])
                for rh, r in enumerate(rows)]

    def out_copy(unit):
        rows = pl.ds(pl.multiple_of(unit * SUB, SUB), SUB)
        return pltpu.make_async_copy(xbuf.at[rows], out_hbm.at[rows], o_sem.at[unit])

    beta_copy = pltpu.make_async_copy(beta_hbm, beta, w_sem.at[8])
    for cp in [x_copy(0), beta_copy] + wv_copies(0):
        cp.start()
    x_copy(0).wait()
    for cp in wv_copies(1) + wv_copies(2):
        cp.start()
    beta_copy.wait()

    sig = 1.0 / (1.0 + jnp.exp(-beta[...].astype(f32)))
    for g in range(8):
        pick = _iota((8, H), 0) + 4 * g == _iota((8, H), 1)
        gate[g] = jnp.broadcast_to(
            jnp.sum(jnp.where(pick, sig, 0.0), axis=1, keepdims=True), (8, 128))
    lane = _iota((128, 128), 1)
    for i, query in enumerate((lane, lane ^ HS, lane | HS)):
        causal[i] = jnp.where(_iota((128, 128), 0) <= query, 0.0, MASKED)

    def quads(upper, lower, r, n, t):
        return [half[pl.ds(r, n), pl.ds(128 * (t + 4 * ch), 128)].astype(f32)
                for half in (upper, lower) for ch in range(2)]

    def band(ref, start, n):
        rows = pl.ds(pl.multiple_of(start, n), n)
        return ref.at[(slice(None),) * (len(ref.shape) - 2) + (rows,)]

    def project(left, r, n, right, t, emit, zero, first=0):
        def prod(i):
            lhs = jnp.concatenate([_ld16(left, (i + zero, k), r, n) for k in range(4)], axis=1)
            return _mm(lhs, _ld16(right, (first + i, t), 0, HALF))
        return (_strassen_lean if n == SUB else _strassen)(prod, emit, park, zero)

    def norm_jobs(src, src_buf, st, dsts, zero, t0, t1):
        def mean_job(r, tick):
            _fence(src_buf, tick)
            st[0][0, pl.ds(r, 16), :] = jnp.broadcast_to(
                _row_mean([src(g, r, 16) for g in range(8)]), (16, 128))

        def var_job(r, tick):
            _fence(st[0], tick)
            mean = st[0][zero, pl.ds(r, 8), :]
            dev = [src(g, r, 8) - mean for g in range(8)]
            st[1][0, pl.ds(r, 8), :] = jnp.broadcast_to(
                lax.rsqrt(_row_mean([d * d for d in dev]) + 1e-5), (8, 128))

        def out_job(r, k, which, tick):
            for buf in (src_buf, *st):
                _fence(buf, tick)
            mean, rstd = ([b[zero, pl.ds(rh * HS + r, 16), :] for rh in range(2)] for b in st)
            _put_left(dsts, k, r, *[(src(k + 4 * ch, rh * HS + r, 16) - mean[rh]) * rstd[rh]
                                    for rh in range(2) for ch in range(2)], which=which)

        work = t1 - t0 - 4
        return (_spread([partial(mean_job, r) for r in range(0, SUB, 16)], t0, t0 + 0.15 * work)
                + _spread([partial(var_job, r) for r in range(0, SUB, 8)],
                          t0 + 2 + 0.15 * work, t0 + 2 + 0.45 * work)
                + _spread([partial(out_job, r, k, which) for r in range(0, HS, 16) for k in range(4)
                           for which in ((2, 4, 6), (0, 1, 3, 5))], t0 + 4 + 0.45 * work, t1))

    def out_operands(dst, k, r, src, g0, g1, zero):
        o = [_swap_odd_heads(*[src[g + zero, pl.ds(rh * HS + r, 16), :] for rh in range(2)])
             for g in (g0, g1)]
        _put_left([dst], k, r, o[0][0], o[1][0], o[0][1], o[1][1])

    def first_norm(i, _):
        r = pl.multiple_of(i * 32, 32)
        rows = []
        for rh in range(2):
            x = xbuf[pl.ds(r + rh * HS, 32), :].astype(f32)
            d = x - _row_mean([x])
            rows.append(d * lax.rsqrt(_row_mean([d * d]) + 1e-5))
        for k in range(4):
            _put_left([xn, p0_l[0]], k, r,
                      *[y[:, 128 * g:128 * (g + 1)] for y in rows for g in (k, k + 4)])

    def value_weights(i, _):
        halves = [band(raw_a.at[0], i * 64 + rh * HALF, 64) for rh in range(2)]
        for t in range(4):
            _put_right(band(w_v, i * 64, 64), t, 0, *quads(*halves, 0, 64, t))

    def phase0(first, c):
        zero = c >> 4
        jobs = []
        if first:
            for i in range(4):
                @pl.when(c == i)
                def _():
                    if i > 0:
                        x_copy(i + 1).wait()
                        w_copy(i - 1).wait()
                    for cp in [w_copy(i)] + ([x_copy(i + 2)] if i < 3 else bqkv_copies(0)):
                        cp.start()

            def arrive(tick):
                pl.when(c == 0)(x_copy(1).wait)

            raw = raw_a.at[c]
            dst = w_kqo.at[pl.ds(7 * jnp.maximum(c - 1, 0), 7)]

            def weights(r, t, tick):
                _fence(raw_a.at[0], tick)
                _put_right(dst, t, r, *quads(raw, raw.at[pl.ds(HALF, HALF)], r, 16, t))

            jobs += [(24, arrive)] + _spread(
                [partial(weights, r, t) for r in range(0, HALF, 16) for t in range(4)], 0, 110)

        def values(u):
            for t in range(4):
                def emit(rh, ch, val):
                    vbuf[t + 4 * ch, c * 4 + u, pl.ds(rh * HS, HS), :] = val.astype(bf16)
                yield from project(p0_l[u], 0, HS, w_v, t, emit, zero)

        def norm(u, t0, t1):
            unit = c * 4 + u + 1
            x = band(xbuf, (unit if u < 3 else jnp.minimum(unit, NSUB - 1)) * SUB, SUB)
            return norm_jobs(lambda g, r, n: x[pl.ds(r, n), pl.ds(128 * g, 128)].astype(f32), xbuf,
                             stat[(u + 1) % 4], [band(xn, unit * HS, HS), p0_l[(u + 1) % 4]],
                             zero, t0, t1)

        jobs += norm(0, 0, 24) + norm(1, 24, 52) + norm(2, 52, 80) + norm(3, 80, 110)
        jobs.sort(key=lambda j: j[0])
        for i in range(1, len(jobs)):
            jobs[i] = (max(jobs[i][0], jobs[i - 1][0] + 0.2), jobs[i][1])
        for _ in _paced([values(u) for u in range(4)], jobs):
            pass

    def phase1(layer, t):
        zero = t >> 4
        never = row8 < zero
        st = {}
        turns = []
        todo = []

        @pl.when(jnp.logical_and(layer == 0, t == 1))
        def _():
            for cp in bqkv_copies(1):
                cp.wait()

        def turn(buf, tick, read):
            if len(turns) >= 3:
                tick = pltpu.bitcast(pltpu.bitcast(tick, u32) | turns[-3], f32)
            _fence(buf, tick)
            y = read().T
            turns.append(pltpu.bitcast(y[:16 if y.dtype == bf16 else 8], u32))
            return y

        def column_weights(m, dst):
            turned, back = perm_c[m]

            def there(c, tick):
                w = turn(raw_bqkv, tick, lambda: _pair(*[
                    band(raw_bqkv, t * 128 + rh * HALF, 128)[:, pl.ds(m * D + 128 * c, 128)]
                    for rh in range(2)]))
                for j in range(4):
                    turned[0, pl.ds((4 * c + j) * (DH + 1), DH), :] = w[j * DH:(j + 1) * DH]

            def again(c, tick):
                back[c] = turn(turned, tick, lambda: jnp.concatenate(
                    [turned[zero, pl.ds(d, H, stride=DH + 1), :] for d in range(4 * c, 4 * c + 4)],
                    axis=0))

            def operands(r, k, tick):
                _fence(back, tick)
                w = [back[k + 4 * ch + zero, pl.ds(r, 16), :] for ch in range(2)]
                _put_right(band(dst, t * 128, 128), k, r,
                           *[_unpair(w[ch], rh) for rh in range(2) for ch in range(2)])
            return ([partial(there, c) for c in range(8)], [partial(again, c) for c in range(8)],
                    [partial(operands, r, k) for r in range(0, 128, 16) for k in range(4)])

        def pad_head(h, tick):
            _fence(raw_bo, tick)
            perm_r[0, pl.ds(h * (DH + 1), DH), :] = _pair(*[
                raw_bo[pl.ds(h * DH, DH), pl.ds(pl.multiple_of(t * 128 + ch * HALF, 128), 128)]
                for ch in range(2)])

        def row_weights(d, h, tick):
            _fence(perm_r, tick)
            w = [perm_r[zero, pl.ds(h * (DH + 1) + d + rh * (DH // 2), 16, stride=DH + 1), :]
                 for rh in range(2)]
            _put_right(w_bo, t, d * H + h, *[_unpair(w[rh], ch) for rh in range(2) for ch in range(2)])

        def turn_q(s, ch, blk, tick):
            def read():
                y = p1_f[blk // 2][2 * ch + blk % 2 + zero]
                return jnp.concatenate(_swap_odd_heads(y[:HS], y[HS:]), axis=0)
            y = turn(p1_f[blk // 2], tick, read)
            p1_q[2 * s + ch][blk][0] = (y * QK_SCALE).astype(bf16)
            if s > 0:
                p1_pq[2 * s + ch - 2][blk][0] = _phi(y).astype(bf16)
            st['q', s, ch, blk] = True

        def turn_v(s, blk, tick):
            y = turn(vbuf, tick, lambda: jnp.concatenate(
                [vbuf[t + 4 * ch, 4 * s + blk] for ch in range(2)], axis=1))
            for ch in range(2):
                p1_v[2 * s + ch][blk][0] = y[128 * ch:128 * (ch + 1)]

        def projection(is_q, s, half, extra):
            def emit(rh, ch, val):
                slot, rows = 2 * s + ch, pl.ds(rh * HS, HS)
                for u in range(2):
                    y = val[HS * u:HS * (u + 1)]
                    if is_q:
                        p1_f[half][2 * ch + u, rows, :] = y
                        continue
                    p1_k[slot][2 * half + u][0, rows, :] = y.astype(bf16)
                    if s < 3:
                        pk = _phi(y)
                        p1_pk[slot][2 * half + u][0, rows, :] = pk.astype(bf16)
                        z = jnp.sum(pk.reshape(HS // 8, 8, 128), axis=0)
                        st['dz', slot] = z + st['dz', slot] if ('dz', slot) in st else z
            jobs = (_spread(todo + [partial(turn_v, s, 2 * half + 1 - is_q)], 0, 7)
                    + _spread(extra, 0, 7))
            todo.clear()
            yield from _paced(
                [project(xn, (4 * s + 2 * half) * HS, SUB, w_kqo, t, emit, zero, 7 * is_q)], jobs)
            if is_q:
                todo.extend(partial(turn_q, s, ch, 2 * half + u) for ch in range(2) for u in (1, 0))
            st['k', s, half, is_q] = True

        def scores(a, n, s, ch, i, kb):
            assert st['q', s, ch, i] and st['k', s, kb // 2, False]
            slot, buf, tops = 2 * s + ch, p1_s[a % len(p1_s)], p1_x[n % len(p1_x)]
            head = lambda at, j: _words(p1_q[slot][i], (at,), DH * j, DH)

            def queries(first, parts):
                pads = [[jnp.zeros((DH // 2 * k, 128), u32)] if k else []
                        for k in (first, 4 - first - len(parts))]
                return pltpu.bitcast(jnp.concatenate(pads[0] + parts + pads[1], axis=0), bf16)

            nk = HS if kb == i else 128
            k = _ld16(p1_k[slot][kb], (zero,), 0, nk)
            for j in range(4):
                sc = _mm(k, queries(j, [head(zero, j)]))
                if kb == i:
                    sc = sc + causal[j % 2 + zero, pl.ds(0, HS), :]
                buf[j, pl.ds(0, nk), :] = sc
                m = jnp.max(sc.reshape(nk // 8, 8, 128), axis=0)
                st['m', n, j] = jnp.maximum(m, st['m', n, j]) if kb > 0 else m
            if kb < i:
                return sc
            upper = _iota((DH // 2, 128), 1) >= HS
            for j in (0, 2):
                m = []
                for r in (HS, HS + 32):
                    at = zero if r == HS else t >> 5
                    q = [jnp.where(upper, head(at, j), 0), jnp.where(upper, 0, head(at, j + 1))]
                    up = _mm(_ld16(p1_k[slot][kb], (zero,), r, 32), queries(j, q))
                    up = up + causal[2 + zero, pl.ds(r, 32), :]
                    buf[j, pl.ds(r, 32), :] = up
                    m.append(jnp.max(up.reshape(4, 8, 128), axis=0))
                m, both = jnp.maximum(*m), []
                for jj, own in ((j, lane8 >= HS), (j + 1, lane8 < HS)):
                    top = jnp.where(own, jnp.maximum(st['m', n, jj], m), st['m', n, jj])
                    both.append(jnp.broadcast_to(jnp.max(top, axis=0, keepdims=True), (8, 128)))
                    tops[jj] = both[-1]
                tops[4 + j // 2] = jnp.where(lane8 >= HS, *both)
            st['top', n] = True
            return jnp.concatenate([sc, up], axis=0)

        def probs(a, n, s, ch, i, kb, ticks):
            assert st['top', n]
            buf, out, tot = p1_s[a % len(p1_s)], p1_p[a % len(p1_p)], p1_l[n % len(p1_l)]
            runs = [(j, 0, HS if kb == i else 128) for j in range(4)]
            if kb == i:
                runs += [(j, HS, 128) for j in (0, 2)]
            count, c = sum(hi - lo for _, lo, hi in runs) // 32, 0
            for j, lo, hi in runs:
                top, l = p1_x[n % len(p1_x)][(4 + j // 2 if lo else j) + zero], None
                for r in range(lo, hi, 32):
                    m = jnp.where(never, ticks[c * len(ticks) // count], top)
                    c += 1
                    p = jnp.exp2(buf[j + zero, pl.ds(r, 32), :] - jnp.concatenate([m] * 4, axis=0))
                    for x in range(0, 32, 8):
                        l = p[x:x + 8] if l is None else l + p[x:x + 8]
                    if lo:
                        upper = _iota((32, 128), 1) >= HS
                        out[j, pl.ds(r, 32), :] = jnp.where(upper, p, 0.0).astype(bf16)
                        out[j + 1, pl.ds(r, 32), :] = jnp.where(upper, 0.0, p).astype(bf16)
                    else:
                        out[j, pl.ds(r, 32), :] = p.astype(bf16)
                if lo:
                    for jj, own in ((j, lane8 >= HS), (j + 1, lane8 < HS)):
                        tot[jj][0] = jnp.broadcast_to(jnp.sum(
                            tot[jj][zero] + jnp.where(own, l, 0.0), axis=0, keepdims=True), (8, 128))
                else:
                    tot[j][0] = l + tot[j][zero] if kb > 0 else l

        def values(a, n, s, ch, i, kb):
            tot = [x[zero] for x in p1_l[n % len(p1_l)]]
            scale = (1.0 - gate[t + 4 * ch]) / jnp.where(
                row8 < 2, jnp.where(row8 == 0, tot[0], tot[1]), jnp.where(row8 == 2, tot[2], tot[3]))
            o, ticks = [None] * 4, []
            for b in range(i + 1):
                for j in range(4):
                    pv = _mm(_ld16(p1_v[2 * s + ch][b], (zero,), DH * j, DH),
                             _ld16(p1_p[(a - i + b) % len(p1_p)], (j + zero,), 0, 128))
                    o[j] = o[j] + pv if b else pv
                ticks.append(pv)
            for j in range(4):
                y = o[j] * scale[j:j + 1]
                if s > 0:
                    assert st['read', ch, i // 2] == s
                    y = y + p1_m[2 * ch + i // 2][i % 2 + zero, pl.ds(DH * j, DH), :]
                obuf[t + 4 * ch, pl.ds(SEG * s + 128 * i + DH * j, DH), :] = y
            return jnp.concatenate(ticks, axis=0)

        def mem_read(s, ch, half):
            assert st['memory', ch] == s
            z = jnp.sum(st['z', ch], axis=0, keepdims=True)
            lhs = jnp.concatenate(
                [jnp.where((lane8 >> 5) == row8, z, 0.0)]
                + [jnp.where((_iota((DH, 128), 1) >> 5) == j, p1_mt[ch][zero, pl.ds(DH * j, DH), :], 0.0)
                   for j in range(4)], axis=0)
            for b in (2 * half, 2 * half + 1):
                assert st['q', s, ch, b]
                nd = _mm(lhs, _ld16(p1_pq[2 * s + ch - 2][b], (zero,), 0, 128))
                inv = gate[t + 4 * ch] / (nd[0:8] + 1e-6)
                for j in range(4):
                    p1_m[2 * ch + half][b % 2, pl.ds(DH * j, DH), :] = (
                        nd[8 + DH * j:8 + DH * (j + 1)] * inv[j:j + 1])
            st['read', ch, half] = s
            return nd

        def mem_update(s, ch):
            assert st['k', s, 0, False] and st['k', s, 1, False]
            slot = 2 * s + ch
            v = jnp.concatenate([_ld16(p1_v[slot][b], (zero,), 0, 128) for b in range(4)], axis=1)
            pk = jnp.concatenate([_ld16(p1_pk[slot][b], (zero,), 0, 128) for b in range(4)], axis=0)
            mt = _mm(v, pk)
            p1_mt[ch][0] = mt + p1_mt[ch][zero] if s > 0 else mt
            st['z', ch] = st['dz', slot] + st['z', ch] if s > 0 else st['dz', slot]
            st['memory', ch] = s + 1
            return mt

        def first_turn(ch, tick):
            p2_t[0][ch] = turn(obuf, tick, lambda: obuf[t + 4 * ch, pl.ds(0, SUB), :])

        def first_operands(r, tick):
            _fence(p2_t[0], tick)
            out_operands(p2_l[0], t, r, p2_t[0], 0, 1, zero)

        tiles = []
        for s in range(4):
            for half in ((0, 1) if s == 0 else (1, 0)):
                for i in (2 * half + 1, 2 * half):
                    for ch in range(2):
                        n = tiles[-1][0] + 1 if tiles else 0
                        tiles += [(n, s, ch, i, kb) for kb in range(i + 1)]
        blocks = [(True, 0, 0), (False, 0, 0), (True, 0, 1), (False, 0, 1)]
        for s in range(1, 4):
            blocks += [(True, s, 1), (False, s, 0), (False, s, 1), (True, s, 0)]
        cq, ck, cv = (column_weights(m, dst) for m, dst in enumerate((w_bq, w_bk, w_bv)))
        ro = [partial(row_weights, d, h) for d in range(DH // 2) for h in (0, 16)]
        ph = [partial(pad_head, h) for h in range(H)]
        side = [cq[0], ph[:16], ck[0][:4] + ph[16:], ck[0][4:] + cv[0][:4],
                cq[1], [], cv[0][4:], ck[1][:4] + ro[:16],
                ck[1][4:] + cq[2][:16], [], cv[1][:4], cv[1][4:] + ro[16:],
                [partial(first_turn, ch) for ch in range(2)] + cq[2][16:], ck[2][:16],
                [partial(first_operands, r) for r in range(0, HS, 16)] + ck[2][16:] + cv[2][:8], cv[2][8:]]
        stream = (p for blk, jobs in zip(blocks, side) for p in projection(*blk, jobs))

        issued = exps = 0
        ready, owed = [0, 0, 0], []
        for a in range(len(tiles) + 3):
            s, pos = divmod(a, 20)
            prods = []
            if 0 < s < 4 and pos in ((2, 13) if s < 3 else (10, 14)):
                prods.append([mem_read(s, ch, int(pos < 13)) for ch in range(2)][1])
            if s < 3 and pos in (16, 18):
                prods.append(mem_update(s, (pos - 16) // 2))
            due = min(int(24 + 1.4 * a) if a < 59 else 47 + a, 7 * len(blocks))
            prods.extend(next(stream) for _ in range(issued, due))
            issued = due
            if a < len(tiles):
                assert a - exps < len(p1_s)
                prods.append(scores(a, *tiles[a]))
            owed += [b for b in range(ready[-3], ready[-2]) if tiles[b][3] == tiles[b][4]]
            for b in owed[:{77: 1, 79: 1, 80: 2}.get(a, 0) if 68 <= a <= 80 else None]:
                assert exps - (b - tiles[b][3]) <= len(p1_p)
                assert tiles[exps - 1][0] - tiles[b][0] < len(p1_l)
                owed.remove(b)
                prods.append(values(b, *tiles[b]))
            if due == 7 * len(blocks):
                next(stream, None)
                if todo:
                    todo.pop(0)(prods[0][0:8])
            upto = min(max(a - 3, exps, {77: 75, 78: 76, 79: 78, 80: 80}.get(a, 0)), len(tiles))
            ticks = [x[r:r + 8] for x in prods[-4:] for r in range(0, x.shape[0], 8)]
            if a == len(tiles):
                ticks = ticks[:16]
            for b in range(exps, upto):
                share = len(ticks) // (upto - exps)
                probs(b, *tiles[b], ticks[(b - exps) * share:(b + 1 - exps) * share])
            exps = upto
            ready.append(exps)
        assert not todo and not owed and ready[-3] == len(tiles)

    def phase2(layer, c):
        zero = c >> 4

        def rows(u, rh):
            return pl.ds(pl.multiple_of((2 * c + u) * SUB + rh * HS, HS), HS)

        def out_jobs(unit, u, t0, t1):
            def turn(g, tick):
                _fence(obuf, tick)
                p2_t[u][g] = obuf[g, pl.ds(pl.multiple_of(unit * SUB, SUB), SUB), :].T

            def operands(r, k, tick):
                _fence(p2_t[u], tick)
                out_operands(p2_l[u], k, r, p2_t[u], k, k + 4, zero)
            return (_spread([partial(turn, g) for g in range(8)], t0, t0 + 6)
                    + _spread([partial(operands, r, k) for r in range(0, HS, 16) for k in range(4)],
                              t0 + 10, t1))

        def infini_out(u):
            for t in range(4):
                def emit(rh, ch, val):
                    g = t + 4 * ch
                    x = xbuf[rows(u, rh), pl.ds(128 * g, 128)].astype(f32)
                    p2_x[u][g, pl.ds(rh * HS, HS), :] = x + val
                yield from project(p2_l[u], 0, HS, w_kqo, t, emit, zero, 14)

        def norm(u, t0, t1):
            return norm_jobs(lambda g, r, n: p2_x[u][g + zero, pl.ds(r, n), :], p2_x[u], stat[u],
                             [p2_l[2 + u]], zero, t0, t1)

        def local_proj(u, w, dst, off):
            for t in range(4):
                def emit(rh, ch, val):
                    dst[u][t + 4 * ch, pl.ds(off + rh * HS, HS), :] = val
                    if off and rh == 1 and u == 0:
                        dst[1][t + 4 * ch, pl.ds(0, HALO), :] = val[HS - HALO:]
                yield from project(p2_l[2 + u], 0, HS, w, t, emit, zero)

        def attend(u, t0, t1, t2, t3):
            held = {}

            def taps(buf, g, r, w):
                x = buf[g + zero, pl.ds(HALO + r - DIL * w - 8, 24), :]
                return (w, x[8:]), (w + WIN // 2, x[:16])

            def logits(r, w0, g, tick):
                _fence(p2_q[u], tick)
                q = p2_q[u][g + zero, pl.ds(r, 16), :]
                for w, k in taps(p2_k[u], g, r, w0) + taps(p2_k[u], g, r, w0 + 1):
                    a = held[w] = q * k if g == 0 else held[w] + q * k
                    if g < 7:
                        continue
                    a = (a + pltpu.roll(a, 64, 1)) + (pltpu.roll(a, 32, 1) + pltpu.roll(a, 96, 1))
                    a = a * QK_SCALE
                    if u == 0 and r == 0 and w > 0:
                        a = jnp.where(2 * c * SUB + _iota((16, 128), 0) >= DIL * w, a, MASKED)
                    p2_a[u][r // 16][0][w] = a

            def softmax(r, tick):
                src, dst = p2_a[u][r // 16]
                _fence(src, tick)
                lg = [src[w + zero, pl.ds(r % 16, 8), :] for w in range(WIN)]
                top = reduce(jnp.maximum, lg)
                ex = [jnp.exp2(a - top) for a in lg]
                for w in range(WIN):
                    dst[w, pl.ds(r % 16, 8), :] = ex[w]
                dst[WIN, pl.ds(r % 16, 8), :] = 1.0 / reduce(jnp.add, ex)

            def mix(r, g, tick):
                _fence(p2_v[u], tick)
                if g % 2 == 0:
                    _fence(p2_a[u][r // 16][1], tick)
                    held['p'] = [p2_a[u][r // 16][1][w + zero] for w in range(WIN + 1)]
                acc = reduce(jnp.add, [held['p'][w] * v for w0 in range(WIN // 2)
                                       for w, v in taps(p2_v[u], g, r, w0)])
                p2_o[u][r % HS // 16][g, pl.ds(r // HS * 16, 16), :] = acc * held['p'][WIN]

            def operands(j, k, tick):
                _fence(p2_o[u][j], tick)
                _put_left([p2_l[4 + u]], k, 16 * j,
                          *[p2_o[u][j][g + zero, pl.ds(16 * rh, 16), :]
                            for rh in range(2) for g in (k, k + 4)])

            order = [rh * HS + r for r in range(0, HS, 16) for rh in range(2)]
            lag, step = (t1 - t0) / 8 + 2.85, (t3 - t2) / 4
            return (_spread([partial(logits, r, w, g) for r in order for w in (0, 2) for g in range(8)],
                            t0, t1)
                    + _spread([partial(softmax, r + i) for r in order for i in (0, 8)],
                              t0 + lag, t1 + lag)
                    + _spread([partial(mix, r, g) for r in order for g in range(8)], t2, t3)
                    + [(t2 + step * (j + 1) + (step / 4 if j < 3 else 0.3) * k + 0.2,
                        partial(operands, j, k)) for j in range(4) for k in range(4)])

        def local_out(u):
            for t in range(4):
                def emit(rh, ch, val):
                    g = t + 4 * ch
                    y = p2_x[u][g + zero, pl.ds(rh * HS, HS), :] + val
                    xbuf[rows(u, rh), pl.ds(128 * g, 128)] = y.astype(bf16)
                yield from project(p2_l[4 + u], 0, HS, w_bo, t, emit, zero)

        def send(u, tick=None):
            pl.when(layer == 1)(out_copy(2 * c + u).start)

        stages = [infini_out(0), infini_out(1)]
        for u in range(2):
            stages += [local_proj(u, w_bk, p2_k, HALO), local_proj(u, w_bq, p2_q, 0),
                       local_proj(u, w_bv, p2_v, HALO)]
        stages += [local_out(0), local_out(1)]
        jobs = (out_jobs(2 * c + 1, 1, 0, 25) + out_jobs(jnp.minimum(2 * c + 2, NSUB - 1), 0, 250, 279)
                + norm(0, 28, 53) + norm(1, 56, 112) + [(252, partial(send, 0))]
                + attend(0, 112, 148, 154, 194) + attend(1, 196, 220, 225, 247))
        for _ in _paced(stages, jobs):
            pass
        for buf in (p2_k, p2_v):
            for g in range(8):
                buf[0][g, pl.ds(0, HALO), :] = buf[1][g + zero, pl.ds(SUB, HALO), :]
        send(1)

    def layer_pair(layer, _):
        lax.fori_loop(0, HS // 32, first_norm, None)

        @pl.when(layer == 0)
        def _():
            for i in range(4):
                for cp in wv_copies(i):
                    cp.wait()
                for cp in (wv_copies(3), [], [x_copy(1)], [])[i]:
                    cp.start()
                lax.fori_loop(2 * i, 2 * i + 2, value_weights, None)
            lax.fori_loop(0, 4, lambda c, _: phase0(True, c), None)
            for cp in [w_copy(3)] + bqkv_copies(0):
                cp.wait()
            for cp in bqkv_copies(1):
                cp.start()

        @pl.when(layer == 1)
        def _():
            lax.fori_loop(0, 4, lambda c, _: phase0(False, c), None)

        lax.fori_loop(0, 4, lambda t, _: phase1(layer, t), None)
        for buf in (p2_k, p2_v):
            buf[0][pl.ds(0, 8), pl.ds(0, HALO), :] = jnp.zeros((8, HALO, 128), f32)
        lax.fori_loop(0, NSUB // 2, lambda c, _: phase2(layer, c), None)

    lax.fori_loop(0, 2, layer_pair, None)
    for unit in range(NSUB):
        out_copy(unit).wait()


@jax.jit
def pallas_interleave_layers__memory_aug_infini_attn__sliding_local_dilated__prompt_kernel(
    A_x: jax.Array,
    A_wq: jax.Array,
    A_wk: jax.Array,
    A_wv: jax.Array,
    A_wo: jax.Array,
    A_beta: jax.Array,
    B_x: jax.Array,
    B_wqkv: jax.Array,
    B_wo: jax.Array,
):
    del B_x
    vmem = pltpu.VMEM
    hbm = pl.BlockSpec(memory_space=pl.ANY)
    block = [vmem((2, 128, 128), bf16)] * 4
    scratch = [
        vmem((S + 16, D), bf16),
        vmem((4, D + 16, D), bf16),
        vmem((D + 16, 3 * D), bf16),
        vmem((D + 16, D), bf16),
        vmem((21, 4, HALF, 128), bf16),
        *[vmem((7, 4, HALF, 128), bf16)] * 5,
        vmem((7, 4, (NSUB + 1) * HS, 128), bf16),
        vmem((9, NSUB, 128, 128), bf16),
        vmem((9, S, 128), f32),
        vmem((8, 8, 128), f32),
        vmem((3, 128, 128), f32),
        [[vmem((2, H * (DH + 1), 128), u32), vmem((9, 128, 128), u32)]] * 3,
        vmem((2, H * (DH + 1), 128), u32),
        [vmem((7, 4, HS, 128), bf16)] * 4,
        [block] * 8, [block] * 6,
        [block] * 8, [block] * 6,
        [block] * 8,
        [vmem((5, 128, 128), f32)] * 2,
        [vmem((2, 128, 128), f32)] * 4,
        [vmem((2, 128, 128), f32)] * 2,
        [vmem((8, 8, 128), f32)] * 8,
        [[vmem((2, 8, 128), f32)] * 4] * 8,
        [vmem((4, 128, 128), bf16)] * 20,
        [vmem((5, 128, 128), f32)] * 8,
        [vmem((10, SUB, 128), f32)] * 2,
        [vmem((10, SUB, 128), f32)] * 2,
        [vmem((8, 4, HS, 128), bf16)] * 6,
        [vmem((10, SUB, 128), f32)] * 2,
        [vmem((10, HALO + SUB, 128), f32)] * 2,
        [vmem((10, HALO + SUB, 128), f32)] * 2,
        [[vmem((9, 32, 128), f32)] * 4] * 2,
        [[[vmem((WIN + 2, 16, 128), f32)] * 2] * 8] * 2,
        [[vmem((2, SUB, 128), f32)] * 2] * 4,
        [vmem((2, SUB, 128), f32)] * 7,
        vmem((1, H), bf16),
        pltpu.SemaphoreType.DMA((5,)),
        pltpu.SemaphoreType.DMA((8,)),
        pltpu.SemaphoreType.DMA((9,)),
        pltpu.SemaphoreType.DMA((NSUB,)),
    ]
    out = pl.pallas_call(
        _kernel,
        out_shape=jax.ShapeDtypeStruct((S, D), bf16),
        in_specs=[hbm] * 8,
        out_specs=hbm,
        scratch_shapes=scratch,
        compiler_params=pltpu.CompilerParams(
            vmem_limit_bytes=112 * 1024 * 1024, flags={"XLA_TPU_FORCE_LP_LLO_SCHEDULER": True}),
        name="interleaved_layers",
    )(A_x.reshape(S, D), A_wq, A_wk, A_wv, A_wo, A_beta.reshape(1, H), B_wqkv, B_wo)
    return out.reshape(1, S, D)
```
